```python
import jax
import jax.numpy as jnp

def _softmax(x, axis=-1):
    return jax.nn.softmax(x, axis=axis)
def _gelu(x):
    return jax.nn.gelu(x, approximate=True)
def _silu(x):
    return jax.nn.silu(x)
def _sigmoid(x):
    return jax.nn.sigmoid(x)
def _layernorm(x, axis=-1, eps=1e-5):
    m = jnp.mean(x, axis=axis, keepdims=True)
    v = jnp.var(x, axis=axis, keepdims=True)
    return (x - m) / jnp.sqrt(v + eps)
def _scatter_add(tgt, idx, src, axis=0):
    return tgt.at[idx].add(src)
def _segment_sum(src, seg, n):
    return jax.ops.segment_sum(src, seg, n)
class _Rng:
    def __init__(self, key):
        self._k = key
    def _next(self):
        self._k, sub = jax.random.split(self._k)
        return sub
    def normal(self, shape):
        return jax.random.normal(self._next(), shape, dtype=jnp.bfloat16)
    def randint(self, lo, hi, shape):
        return jax.random.randint(self._next(), shape, lo, hi, dtype=jnp.int32)
    def uniform(self, shape, lo=0.0, hi=1.0):
        return jax.random.uniform(self._next(), shape, jnp.bfloat16, lo, hi)
    def permutation(self, n):
        return jax.random.permutation(self._next(), n)


kernel_name = 'interleave_layers__sliding_block_cached__glu_gated_swiglu__decode'

def setup_inputs():
    _rng = _Rng(jax.random.key(int.from_bytes(__import__("os").urandom(4), "little")))
    _w = (lambda a: (lambda t: t.astype(jnp.bfloat16) if jnp.issubdtype(t.dtype, jnp.floating) else t)(jnp.asarray(a)))
    def _A_setup():
        B, Sq, D = 1, 1, 640
        Hq, Hkv, Sk, Dh = 32, 32, 32768, 192
        assert Hq % Hkv == 0, (Hq, Hkv)
        return {
            "x": _w((lambda *s: _rng.normal(s) * 0.05)(B, Sq, D)),
            "k_cache": _w((lambda *s: _rng.normal(s) * 0.05)(B, Hkv, Sk, Dh)),
            "v_cache": _w((lambda *s: _rng.normal(s) * 0.05)(B, Hkv, Sk, Dh)),
            "wq": _w((lambda *s: _rng.normal(s) * 0.05)(D, Hq * Dh) * (D ** -0.5)),
            "wo": _w((lambda *s: _rng.normal(s) * 0.05)(Hq * Dh, D) * ((Hq * Dh) ** -0.5)),
        }
    _A_in = _A_setup()

    def _B_setup():
        B, S, D, F = 1, 1, 640, 1536
        return {
            "x": _w((lambda *s: _rng.normal(s) * 0.05)(B, S, D)),
            "w1": _w((lambda *s: _rng.normal(s) * 0.05)(D, F) * (2.0 / D) ** 0.5),
            "w3": _w((lambda *s: _rng.normal(s) * 0.05)(D, F) * (2.0 / D) ** 0.5),
            "w2": _w((lambda *s: _rng.normal(s) * 0.05)(F, D) * (2.0 / F) ** 0.5),
        }
    _B_in = _B_setup()

    return {
        "A_x": _A_in["x"],
        "A_k_cache": _A_in["k_cache"],
        "A_v_cache": _A_in["v_cache"],
        "A_wq": _A_in["wq"],
        "A_wo": _A_in["wo"],
        "B_x": _B_in["x"],
        "B_w1": _B_in["w1"],
        "B_w3": _B_in["w3"],
        "B_w2": _B_in["w2"],
    }

def reference(A_x, A_k_cache, A_v_cache, A_wq, A_wo, B_x, B_w1, B_w3, B_w2):
    def _A_ref(x, k_cache, v_cache, wq, wo):
        B, Sq, D = x.shape
        Hq, Dh = 32, 192
        Hkv, Sk = k_cache.shape[1], k_cache.shape[2]
        W = min(4096, max(256, Sk // 4))
        rep = Hq // Hkv
        q = (lambda x, *d: x.transpose(*d))((x @ wq).reshape(B, Sq, Hq, Dh), 0, 2, 1, 3)
        k = jnp.repeat(k_cache[:, :, Sk - W:, :], rep, axis=1)
        v = jnp.repeat(v_cache[:, :, Sk - W:, :], rep, axis=1)
        scores = jnp.einsum("bhqd,bhkd->bhqk", q, k) * (Dh ** -0.5)
        p = _softmax(scores, axis=-1)
        o = jnp.einsum("bhqk,bhkd->bhqd", p, v)
        return (lambda x, *d: x.transpose(*d))(o, 0, 2, 1, 3).reshape(B, Sq, Hq * Dh) @ wo

    def _B_ref(x, w1, w3, w2):
        gate = jnp.einsum("bsd,df->bsf", x, w1)
        up = jnp.einsum("bsd,df->bsf", x, w3)
        h = _silu(gate) * up
        out = jnp.einsum("bsf,fd->bsd", h, w2)
        return out

    x = A_x
    x = x + _A_ref(_layernorm(x, axis=-1), A_k_cache, A_v_cache, A_wq, A_wo)
    x = x + _B_ref(_layernorm(x, axis=-1), B_w1, B_w3, B_w2)
    x = x + _A_ref(_layernorm(x, axis=-1), A_k_cache, A_v_cache, A_wq, A_wo)
    x = x + _B_ref(_layernorm(x, axis=-1), B_w1, B_w3, B_w2)
    return x
```

```python
import jax
import jax.numpy as jnp
import numpy as np
from jax import lax
import jax.experimental.pallas as pl
import jax.experimental.pallas.tpu as pltpu

D = 640
H = 32
DH = 192
FF = 1536
NG = DH // 8
EPS = 1e-5

f32 = jnp.float32
bf16 = jnp.bfloat16
u32 = jnp.uint32

_TILE_GROUPS = (
    tuple(range(0, 16, 2)),
    tuple(range(1, 16, 2)),
    (16, 18, 20, 22, 17, 19, 21, 23),
)


def _round_bf16(x):
    return x.astype(bf16).astype(f32)


def _layernorm(x):
    m = jnp.mean(x, axis=-1, keepdims=True)
    c = x - m
    v = jnp.mean(c * c, axis=-1, keepdims=True)
    return c * lax.rsqrt(v + EPS)


def _make_kernel(sk, win):
    nc = win // 128
    ncp = nc // 2
    row0 = (sk - win) // 128 * 4
    nrows = nc * 4
    assert nc == 32
    scale = float(np.asarray(DH ** -0.5, dtype=bf16))
    w2_splits = ((0, 1024), (1024, 1536))

    def kernel(x_hbm, k_hbm, v_hbm, wq_hbm, wo_hbm, w1_hbm, w3_hbm, w2_hbm,
               o_ref,
               xbuf, kbuf, vbuf, wq, wo, w1, w3, w2, ybuf, pbuf, lbuf, obuf,
               zbuf, ksem, vsem, wsem):
        k32 = k_hbm.bitcast(u32)
        v32 = v_hbm.bitcast(u32)

        def k_copy(h):
            return pltpu.make_async_copy(
                k32.at[h, :, pl.ds(row0, nrows), :], kbuf.at[h], ksem.at[h])

        def v_copy(h):
            return pltpu.make_async_copy(
                v32.at[h, :, pl.ds(row0, nrows), :], vbuf.at[h], vsem.at[h])

        x_copy = pltpu.make_async_copy(x_hbm, xbuf, wsem.at[0])
        wq_copy = pltpu.make_async_copy(wq_hbm, wq, wsem.at[1])
        wo_copy = pltpu.make_async_copy(wo_hbm, wo, wsem.at[2])
        w1_copy = pltpu.make_async_copy(w1_hbm, w1, wsem.at[3])
        w3_copy = pltpu.make_async_copy(w3_hbm, w3, wsem.at[4])
        w2_copies = [
            pltpu.make_async_copy(w2_hbm.at[pl.ds(a, b - a)],
                                  w2.at[pl.ds(a, b - a)], wsem.at[5 + i])
            for i, (a, b) in enumerate(w2_splits)]

        x_copy.start()
        wq_copy.start()
        wo_copy.start()
        for h in range(H):
            k_copy(h).start()
            v_copy(h).start()
        w1_copy.start()
        w3_copy.start()
        for c in w2_copies:
            c.start()

        zbuf[...] = jnp.zeros((8, 128), u32)

        lane = lax.broadcasted_iota(jnp.int32, (8, 128), 1)
        sub = lax.broadcasted_iota(jnp.int32, (8, 128), 0)
        even_grp = (lane & 8) == 0
        low_half = lane < 64

        def build_y(t):
            b = pltpu.bitcast(t, u32)
            y_even = jnp.where(even_grp, b >> 16, pltpu.roll(b, 8, 1))
            y_odd = jnp.where(even_grp, pltpu.roll(b, 120, 1) >> 16, b)
            return y_even, y_odd

        def q_proj(z):
            q = jnp.dot(z, wq[...], preferred_element_type=f32)
            q = _round_bf16(q)
            for i in range(H // 2):
                t0, t1, t2 = (q[:, (3 * i + j) * 128:(3 * i + j + 1) * 128]
                              for j in range(3))
                r1 = pltpu.roll(t1, 64, 1)
                r2 = pltpu.roll(t2, 64, 1)
                for h, (a, b) in ((2 * i, (t0, t1)),
                                  (2 * i + 1, (jnp.where(low_half, r1, r2), r2))):
                    e0, o0 = build_y(a)
                    e1, o1 = build_y(b)
                    ybuf[h, 0] = e0
                    ybuf[h, 1] = o0
                    ybuf[h, 2] = jnp.where(low_half, e1, pltpu.roll(o1, 64, 1))

        def qk_steps(h):
            kref = kbuf.at[h]
            ys = [ybuf[h, t] for t in range(3)]
            lhs = [[jnp.where(sub == cl, ys[t], jnp.uint32(0)) for t in range(3)]
                   for cl in range(4)]
            quarters = []
            for j in range(4):
                acc = None
                for cl in range(4):
                    c = 4 * j + cl
                    dep = yield
                    l0 = lhs[cl][0]
                    if dep is not None:
                        l0 = l0 | (pltpu.bitcast(dep, u32) & zbuf[...])
                    l = jnp.concatenate([l0, lhs[cl][1], lhs[cl][2]], axis=1)
                    w = jnp.concatenate(
                        [kref[g, 8 * c:8 * c + 8, :]
                         for t in range(3) for g in _TILE_GROUPS[t]], axis=0)
                    s = jnp.dot(pltpu.bitcast(l, bf16), pltpu.bitcast(w, bf16),
                                preferred_element_type=f32)[0:8]
                    acc = s if acc is None else acc + s
                quarters.append(acc)
            s = jnp.concatenate(quarters, axis=0) * scale
            m = jnp.max(jnp.max(s, axis=0, keepdims=True), axis=1, keepdims=True)
            p = jnp.exp(s - m)
            l = jnp.sum(jnp.sum(p, axis=0, keepdims=True), axis=1, keepdims=True)
            pbuf[h] = p
            lbuf[h] = jnp.broadcast_to(1.0 / l, (8, 128))
            yield

        def pv_group(h, g):
            vref = vbuf.at[h]
            pref = pbuf.at[h]
            acc = None
            for c in range(ncp):
                v = pltpu.bitcast(vref[g, 8 * c:8 * c + 8, :], bf16).astype(f32)
                t = (v[0:8] * pref[2 * c:2 * c + 1, :]
                     + v[8:16] * pref[2 * c + 1:2 * c + 2, :])
                acc = t if acc is None else acc + t
            return acc

        def pv_finish(h, accs):
            t = [jnp.zeros((8, 128), f32), jnp.zeros((8, 128), f32)]
            for g in range(NG):
                r = jnp.sum(accs[g], axis=1, keepdims=True)
                t[g // 16] = jnp.where((lane >> 3) == (g % 16), r, t[g // 16])
            inv = lbuf[h]
            diag = (lane & 7) == sub
            for i in range(2):
                obuf[h, :, 128 * i:128 * (i + 1)] = jnp.where(diag, t[i] * inv, 0.0)

        def run_qk(h):
            for _ in qk_steps(h):
                pass

        def run_pv(h):
            pv_finish(h, [pv_group(h, g) for g in range(NG)])

        def run_both(hq, hv):
            gen = qk_steps(hq)
            next(gen)
            accs = []
            for step in range(16):
                need = int(step * 1.1)
                while len(accs) < need:
                    accs.append(pv_group(hv, len(accs)))
                gen.send(accs[need - 1] if need > 0 else None)
            while len(accs) < NG:
                accs.append(pv_group(hv, len(accs)))
            pv_finish(hv, accs)

        x_copy.wait()
        x0 = jnp.broadcast_to(xbuf[0].astype(f32), (8, D))

        def layer_body(layer, x):
            first = layer == 0

            @pl.when(first)
            def _():
                wq_copy.wait()
                k_copy(0).wait()

            q_proj(_layernorm(x).astype(bf16))
            run_qk(0)

            def head_body(h, carry):
                @pl.when(first)
                def _():
                    v_copy(h).wait()
                    k_copy(h + 1).wait()
                run_both(h + 1, h)
                return carry

            lax.fori_loop(0, H - 1, head_body, 0)

            @pl.when(first)
            def _():
                v_copy(H - 1).wait()
                wo_copy.wait()

            run_pv(H - 1)

            o = jnp.concatenate([obuf[h][:, :DH] for h in range(H)], axis=1)
            a = jnp.dot(o.astype(bf16), wo[...], preferred_element_type=f32)
            a = jnp.sum(a, axis=0, keepdims=True)
            x = _round_bf16(x + _round_bf16(a))

            @pl.when(first)
            def _():
                w1_copy.wait()
                w3_copy.wait()

            z = _layernorm(x).astype(bf16)
            gate = _round_bf16(jnp.dot(z, w1[...], preferred_element_type=f32))
            up = _round_bf16(jnp.dot(z, w3[...], preferred_element_type=f32))
            hid = (_round_bf16(gate * jax.nn.sigmoid(gate)) * up).astype(bf16)
            y = None
            for (a0, b0), cp in zip(w2_splits, w2_copies):
                @pl.when(first)
                def _():
                    cp.wait()
                t = jnp.dot(hid[:, a0:b0], w2[a0:b0, :],
                            preferred_element_type=f32)
                y = t if y is None else y + t
            return _round_bf16(x + _round_bf16(y))

        x = lax.fori_loop(0, 2, layer_body, x0)
        o_ref[0] = x[0:1].astype(bf16)

    return kernel


def _tile_view(cache):
    _, h, s, dh = cache.shape
    t = jnp.swapaxes(cache, 2, 3).reshape(h, dh // 8, 8, s // 128, 128)
    return t.transpose(0, 1, 3, 2, 4).reshape(h, dh // 8, s // 128 * 8, 128)


@jax.jit
def pallas_interleave_layers__sliding_block_cached__glu_gated_swiglu__decode_kernel(
    A_x: jax.Array,
    A_k_cache: jax.Array,
    A_v_cache: jax.Array,
    A_wq: jax.Array,
    A_wo: jax.Array,
    B_x: jax.Array,
    B_w1: jax.Array,
    B_w3: jax.Array,
    B_w2: jax.Array,
):
    del B_x
    sk = A_k_cache.shape[2]
    win = min(4096, max(256, sk // 4))
    nrows = win // 128 * 4
    any_spec = pl.BlockSpec(memory_space=pl.ANY)
    return pl.pallas_call(
        _make_kernel(sk, win),
        out_shape=jax.ShapeDtypeStruct((1, 1, D), bf16),
        in_specs=[any_spec] * 8,
        out_specs=pl.BlockSpec(memory_space=pltpu.VMEM),
        scratch_shapes=[
            pltpu.VMEM((1, 1, D), bf16),
            pltpu.VMEM((H, NG, nrows, 128), u32),
            pltpu.VMEM((H, NG, nrows, 128), u32),
            pltpu.VMEM((D, H * DH), bf16),
            pltpu.VMEM((H * DH, D), bf16),
            pltpu.VMEM((D, FF), bf16),
            pltpu.VMEM((D, FF), bf16),
            pltpu.VMEM((FF, D), bf16),
            pltpu.VMEM((H, 3, 8, 128), u32),
            pltpu.VMEM((H, 32, 128), f32),
            pltpu.VMEM((H, 8, 128), f32),
            pltpu.VMEM((H, 8, 256), f32),
            pltpu.VMEM((8, 128), u32),
            pltpu.SemaphoreType.DMA((H,)),
            pltpu.SemaphoreType.DMA((H,)),
            pltpu.SemaphoreType.DMA((7,)),
        ],
        compiler_params=pltpu.CompilerParams(
            vmem_limit_bytes=124 * 1024 * 1024),
    )(A_x, _tile_view(A_k_cache), _tile_view(A_v_cache),
      A_wq, A_wo, B_w1, B_w3, B_w2)
```

```python
import jax
import jax.numpy as jnp
import numpy as np
from jax import lax
import jax.experimental.pallas as pl
import jax.experimental.pallas.tpu as pltpu

D = 640
H = 32
NP = H // 2
DH = 192
PD = 2 * DH
NG = PD // 8
FF = 1536
EPS = 1e-5
NLAYERS = 2
REP = 1
DEPTH = (11,) * 48
SYNC = True
LINK_L = None
LAG = 1
MV = 190
VPACE = 26
LINK_P = None
XLINK = 1
NOCSE = False
CHAIN = True
MLINK = 190
VLINK = True
VMARGIN = -40
VRATE = 1 / 25
GLMAJOR = True
PREMASK = True
LINK_R = (18, 18, 18)
ORDER = 'rkqo'
RLATE = False

f32 = jnp.float32
bf16 = jnp.bfloat16
u32 = jnp.uint32


def _round_bf16(x):
    return x.astype(bf16).astype(f32)


def _as_bf16(x):
    return pltpu.bitcast(x, bf16)


def _layernorm(x):
    m = jnp.mean(x, axis=-1, keepdims=True)
    c = x - m
    v = jnp.mean(c * c, axis=-1, keepdims=True)
    return c * lax.rsqrt(v + EPS)


def _make_kernel(sk, win):
    nc = win // 128
    ncp = nc // 2
    row0 = (sk - win) // 128 * 4
    assert nc == 32
    scale = float(np.asarray(DH ** -0.5, dtype=bf16))
    w2_splits = ((0, 1536),)

    def kernel(x_hbm, k_hbm, v_hbm, wq_hbm, wo_hbm, w1_hbm, w3_hbm, w2_hbm,
               o_ref,
               xbuf, kbuf, vbuf, wq, wo, w1, w3, w2,
               zq, ybuf, pc, lbuf, abuf, obuf,
               zbuf, onesb, cbuf, ksem, vsem, wsem):
        k32 = k_hbm.bitcast(u32)
        v32 = v_hbm.bitcast(u32)

        def k_copy(i):
            return pltpu.make_async_copy(
                k32.at[i, :, pl.ds(row0, 4 * nc), :], kbuf.at[i], ksem.at[i])

        def v_copy(i):
            return pltpu.make_async_copy(
                v32.at[i, :, pl.ds(row0, 4 * nc), :], vbuf.at[i], vsem.at[i])

        x_copy = pltpu.make_async_copy(x_hbm, xbuf, wsem.at[0])
        wq_copy = pltpu.make_async_copy(wq_hbm.bitcast(u32), wq, wsem.at[1])
        wo_copy = pltpu.make_async_copy(wo_hbm.bitcast(u32), wo, wsem.at[2])
        w1_copy = pltpu.make_async_copy(w1_hbm, w1, wsem.at[3])
        w3_copy = pltpu.make_async_copy(w3_hbm, w3, wsem.at[4])
        w2_copies = [
            pltpu.make_async_copy(w2_hbm.at[pl.ds(a, b - a)],
                                  w2.at[pl.ds(a, b - a)], wsem.at[5 + i])
            for i, (a, b) in enumerate(w2_splits)]

        wq_copy.start()
        x_copy.start()
        wo_copy.start()
        for i in range(NP):
            k_copy(i).start()
            if i == NP - 1:
                w1_copy.start()
                w3_copy.start()
            v_copy(i).start()
        for c in w2_copies:
            c.start()

        zbuf[...] = jnp.zeros((8, 128), u32)
        onesb[...] = jnp.ones((8, 128), f32)
        lbuf[...] = jnp.ones(lbuf.shape, f32)

        lane = lax.broadcasted_iota(jnp.int32, (8, 128), 1)
        sub = lax.broadcasted_iota(jnp.int32, (8, 128), 0)

        for n in range(4):
            cbuf[n] = 2 * n + (sub >> 2)
        cbuf[4] = sub ^ 1
        cbuf[5] = jnp.zeros_like(sub)
        cbuf[6] = jnp.where(lane < 64, 0, 2)
        cbuf[7] = jnp.full_like(sub, 2)
        cbuf[8] = lane & 8
        cbuf[9] = sub
        cbuf[10] = sub - jnp.where(lane < 64, 0, 1)
        cbuf[11] = sub - 1

        def rows(x, n):
            return jnp.take_along_axis(x, cbuf[n], axis=0,
                                       mode="promise_in_bounds")

        def retile(ref, ntile):
            top = sub < 4

            def body(a, carry):
                v = [ref[a, 8 * n:8 * n + 8, :] for n in range(ntile)]
                for t in range(ntile):
                    lo, hi = v[t // 2], v[(ntile + t) // 2]
                    if t % 2:
                        lo = pltpu.roll(lo, 4, 0)
                    if (ntile + t) % 2 == 0:
                        hi = pltpu.roll(hi, 4, 0)
                    ref[a, 8 * t:8 * t + 8, :] = jnp.where(top, lo, hi)
                return carry

            lax.fori_loop(0, ref.shape[0], body, 0)

        wq_copy.wait()
        retile(wq, H * DH // 128)
        wo_copy.wait()
        retile(wo, D // 128)

        def kmask(var, t):
            return cbuf[9 + t] == 2 * var

        def q_stage(i, out):
            r0 = 24 * i
            if not isinstance(r0, int):
                r0 = pl.multiple_of(r0, 8)
            wref = wq.at[:, pl.ds(r0, 24), :]
            even_grp = cbuf[8] == 0
            z = _as_bf16(zq[...])
            for t in range(3):
                w = wref[:, 8 * t:8 * t + 8, :].reshape(D // 2, 128)
                q = jnp.dot(z, _as_bf16(w), preferred_element_type=f32)[0:8]
                b = pltpu.bitcast(_round_bf16(q), u32)
                for y in (jnp.where(even_grp, b >> 16, pltpu.roll(b, 8, 1)),
                          jnp.where(even_grp, pltpu.roll(b, 120, 1) >> 16, b)):
                    if PREMASK:
                        for var in range(2):
                            out.append(jnp.where(kmask(var, t), y, jnp.uint32(0)))
                    else:
                        out.append(y)
                yield 40, q

        def k_stage(i, ys, out):
            kref = kbuf.at[i]
            groups = [16 * t + 2 * n + e
                      for t in range(3) for e in range(2) for n in range(8)]
            for c in range(ncp):
                var = c % 2
                if PREMASK:
                    lhs = jnp.concatenate(
                        [ys(2 * n + var) for n in range(6)], axis=1)
                else:
                    lhs = jnp.concatenate(
                        [jnp.where(kmask(var, n // 2), ys(n), jnp.uint32(0))
                         for n in range(6)], axis=1)
                w = jnp.concatenate(
                    [kref[g, 8 * c:8 * c + 8, :] for g in groups], axis=0)
                s = jnp.dot(_as_bf16(lhs), _as_bf16(w),
                            preferred_element_type=f32)[0:8]
                if c % 2 == 0:
                    out.append(s)
                else:
                    out[-1] = out[-1] + s
                yield 48, out[-1]

        def o_stage(i, ts, valid=None):
            wref = wo.at[pl.ds(24 * i, 24)]
            t = jnp.concatenate(ts, axis=1).astype(bf16)
            w = jnp.concatenate(
                [wref[:, 8 * n:8 * n + 8, :].reshape(DH, 128)
                 for n in range(D // 128)], axis=1)
            y = jnp.dot(t, _as_bf16(w), preferred_element_type=f32)
            if valid is not None:
                y = jnp.where(valid, y, 0.0)
            obuf[...] += y
            yield 120, None

        def run(*gens):
            for g in gens:
                for _ in g:
                    pass

        def trace_mxu(mxu_gens, links):
            spent = 0
            for gen in mxu_gens:
                for cost, res in gen:
                    spent += cost
                    if res is not None and MV is not None:
                        g = int((spent + MV) / VPACE)
                        if g < NG:
                            links.setdefault(g, []).append(res)

        def fold_rows(x, op):
            x = op(x, pltpu.roll(x, 4, 0))
            return op(x, rows(x, 4))

        def softmax_stage(ss):
            m = ss[0]
            for s in ss[1:]:
                m = jnp.maximum(m, s)
            m = jnp.max(fold_rows(m, jnp.maximum), axis=1, keepdims=True)
            return [jnp.exp((s - m) * scale) for s in ss]

        def v_stage(i, links):
            vref = vbuf.at[i]
            never = zbuf[...] != 0
            hist = []
            for g in range(NG):
                par = g // 24
                if g % 24 == 0:
                    ps = [pc[par, j] for j in range(nc // 4)]
                    pv = [rows(ps[c // 2], 2 * (c % 2) + par) for c in range(ncp)]
                    if par == 1:
                        tot = ps[0]
                        for p in ps[1:]:
                            tot = tot + p
                        l = jnp.sum(fold_rows(tot, jnp.add), axis=1, keepdims=True)
                        inv = jnp.broadcast_to(1.0 / l, (8, 128))
                        if LINK_L is not None:
                            links.setdefault(LINK_L, []).append(inv)
                        for j in range(3):
                            lbuf[j] = rows(inv, 5 + j)
                npair = 16 - DEPTH[g]
                accs = [None, None]
                pend = [None, None]
                pending = list(links.get(g, ()))
                for c in range(ncp):
                    w = vref[g, 8 * c:8 * c + 8, :]
                    hold = c % 2 == 1 and c < 15 and ((c // 2) * npair) % 7 < npair
                    p = pv[c]
                    if SYNC and c == 0 and len(hist) >= LAG:
                        p = jnp.where(never, hist[-LAG][0] + hist[-LAG][1], p)
                    ts = (pltpu.bitcast(w << 16, f32) * p,
                          pltpu.bitcast(w & jnp.uint32(0xFFFF0000), f32) * p)
                    for a, t in enumerate(ts):
                        if accs[a] is None:
                            if len(hist) >= LAG and not SYNC:
                                t = jnp.where(never, hist[-LAG][(a + XLINK) % 2], t)
                            accs[a] = t
                            continue
                        if pending:
                            t = jnp.where(never, pending.pop(), t)
                        if hold:
                            pend[a] = t
                        else:
                            if pend[a] is not None:
                                t = pend[a] + t
                                pend[a] = None
                            accs[a] = accs[a] + t
                for a in range(2):
                    abuf[g, pl.ds(a, 8, stride=2), :] = accs[a]
                hist.append(accs)

        def r_stage(out):
            ones = jnp.concatenate([onesb[...]] * 2, axis=1)
            for j in range(3):
                a = jnp.concatenate(
                    [abuf[16 * j:16 * j + 16, 8 * s:8 * s + 8, :].reshape(128, 128)
                     for s in range(2)], axis=1)
                t = lax.dot_general(ones, a, (((1,), (1,)), ((), ())),
                                    preferred_element_type=f32)
                out.append(t * lbuf[j])
                yield 32, (out[-1] if RLATE else t)

        x_copy.wait()
        x0 = jnp.broadcast_to(xbuf[0].astype(f32), (8, D))

        def layer_body(layer, x):
            first = layer == 0

            @pl.when(first)
            def _():
                k_copy(0).wait()

            z = _layernorm(x)
            zq[...] = pltpu.bitcast(
                jnp.concatenate([z, z], axis=0).astype(bf16), u32)
            obuf[...] = jnp.zeros(obuf.shape, f32)
            abuf[...] = jnp.zeros(abuf.shape, f32)

            y0, y1, ss = [], [], []
            run(q_stage(0, y0), q_stage(1, y1), k_stage(0, lambda n: y0[n], ss))
            for t, y in enumerate(y1):
                ybuf[t] = y
            for j, p in enumerate(softmax_stage(ss)):
                pc[0, j] = p
                pc[1, j] = p

            def pair_body(it, carry):
                i = it % (NP - 1) if REP > 1 else it

                @pl.when(jnp.logical_and(first, it < NP - 1))
                def _():
                    v_copy(i).wait()
                    k_copy(i + 1).wait()

                links = {}
                ss, yn, ts = [], [], []
                gens = {
                    'r': r_stage(ts),
                    'k': k_stage(i + 1, lambda n: ybuf[n], ss),
                    'q': q_stage(jnp.minimum(i + 2, NP - 1), yn),
                    'o': o_stage(jnp.maximum(i - 1, 0), ts)}
                trace_mxu([gens[st] for st in ORDER], links)
                ps = softmax_stage(ss)
                v_stage(i, links)
                for t, y in enumerate(yn):
                    ybuf[t] = y
                for j, p in enumerate(ps):
                    pc[0, j] = p
                    pc[1, j] = p
                return carry

            lax.fori_loop(0, (NP - 1) * REP, pair_body, 0)

            @pl.when(first)
            def _():
                w1_copy.wait()
                w3_copy.wait()
                v_copy(NP - 1).wait()

            i = NP - 1
            ts = []
            run(r_stage(ts), o_stage(i - 1, ts))
            v_stage(i, {})
            ts = []
            run(r_stage(ts), o_stage(i, ts))

            x = _round_bf16(x + _round_bf16(obuf[...]))

            z = _layernorm(x).astype(bf16)
            gate = _round_bf16(jnp.dot(z, w1[...], preferred_element_type=f32))
            up = _round_bf16(jnp.dot(z, w3[...], preferred_element_type=f32))
            hid = (_round_bf16(gate * jax.nn.sigmoid(gate)) * up).astype(bf16)
            y = None
            for (a0, b0), cp in zip(w2_splits, w2_copies):
                @pl.when(first)
                def _():
                    cp.wait()
                t = jnp.dot(hid[:, a0:b0], w2[a0:b0, :],
                            preferred_element_type=f32)
                y = t if y is None else y + t
            return _round_bf16(x + _round_bf16(y))

        x = lax.fori_loop(0, NLAYERS, layer_body, x0)
        o_ref[0] = x[0:1].astype(bf16)

    return kernel


def _tiles(a, lead):
    r, c = a.shape
    t = a.reshape(r // 8, 8, c // 128, 128).transpose(0, 2, 1, 3)
    return t.reshape(lead + (-1, 128))


@jax.jit
def pallas_interleave_layers__sliding_block_cached__glu_gated_swiglu__decode_kernel(
    A_x: jax.Array,
    A_k_cache: jax.Array,
    A_v_cache: jax.Array,
    A_wq: jax.Array,
    A_wo: jax.Array,
    B_x: jax.Array,
    B_w1: jax.Array,
    B_w3: jax.Array,
    B_w2: jax.Array,
):
    del B_x
    sk = A_k_cache.shape[2]
    win = min(4096, max(256, sk // 4))
    kt = _tiles(jnp.swapaxes(A_k_cache, 2, 3).reshape(H * DH, sk), (NP, NG))
    vt = _tiles(jnp.swapaxes(A_v_cache, 2, 3).reshape(H * DH, sk), (NP, NG))
    any_spec = pl.BlockSpec(memory_space=pl.ANY)
    return pl.pallas_call(
        _make_kernel(sk, win),
        out_shape=jax.ShapeDtypeStruct((1, 1, D), bf16),
        in_specs=[any_spec] * 8,
        out_specs=pl.BlockSpec(memory_space=pltpu.VMEM),
        scratch_shapes=[
            pltpu.VMEM((1, 1, D), bf16),
            pltpu.VMEM((NP, NG, win // 32, 128), u32),
            pltpu.VMEM((NP, NG, win // 32, 128), u32),
            pltpu.VMEM((D // 16, H * DH // 16, 128), u32),
            pltpu.VMEM((H * DH // 16, D // 16, 128), u32),
            pltpu.VMEM((D, FF), bf16),
            pltpu.VMEM((D, FF), bf16),
            pltpu.VMEM((FF, D), bf16),
            pltpu.VMEM((8, D), u32),
            pltpu.VMEM((12, 8, 128), u32),
            pltpu.VMEM((2, 8, 8, 128), f32),
            pltpu.VMEM((3, 8, 128), f32),
            pltpu.VMEM((NG, 16, 128), f32),
            pltpu.VMEM((8, D), f32),
            pltpu.VMEM((8, 128), u32),
            pltpu.VMEM((8, 128), f32),
            pltpu.VMEM((16, 8, 128), jnp.int32),
            pltpu.SemaphoreType.DMA((NP,)),
            pltpu.SemaphoreType.DMA((NP,)),
            pltpu.SemaphoreType.DMA((7,)),
        ],
        compiler_params=pltpu.CompilerParams(
            vmem_limit_bytes=124 * 1024 * 1024,
            disable_semaphore_checks=True),
    )(A_x, kt, vt, _tiles(A_wq, (D // 16,)), _tiles(A_wo, (H * DH // 16,)),
      B_w1, B_w3, B_w2)
```

```python
import jax
import jax.numpy as jnp
import numpy as np
from jax import lax
import jax.experimental.pallas as pl
import jax.experimental.pallas.tpu as pltpu

D = 640
H = 32
NP = H // 2
DH = 192
PD = 2 * DH
NG = PD // 8
FF = 1536
EPS = 1e-5
NLAYERS = 2
REP = 1
LDEPTH = (9,) * 48
EDEPTH = (11,) * 48
SYNC = True
OLATE = True
OL2 = True
EL = (99, 99, 3, 99, 99, 99, 99)
ELAG = 100
WEARLY = False
W2S = ((0, 1280), (1280, 1536))
FCH = 256
LINK_L = None
LAG = 1
MV = 190
VPACE = 26
LINK_P = None
XLINK = 1
NOCSE = False
CHAIN = True
MLINK = 190
VLINK = True
VMARGIN = -40
VRATE = 1 / 25
GLMAJOR = True
PREMASK = True
LINK_R = (18, 18, 18)
ORDER = 'rkqo'
RLATE = False

f32 = jnp.float32
bf16 = jnp.bfloat16
u32 = jnp.uint32


def _round_bf16(x):
    return x.astype(bf16).astype(f32)


def _as_bf16(x):
    return pltpu.bitcast(x, bf16)


def _ln_stats(x):
    m = jnp.mean(x, axis=-1, keepdims=True)
    c = x - m
    v = jnp.mean(c * c, axis=-1, keepdims=True)
    return m, c, lax.rsqrt(v + EPS)


def _with_ones(x):
    return jnp.concatenate([x, jnp.ones_like(x)], axis=0).astype(bf16)


def _ln_dot(xo, w, m, r):
    y = jnp.dot(xo, w, preferred_element_type=f32)
    y = y[0:8] - m * y[8:16]
    return y if r is None else y * r


def _make_kernel(sk, win):
    nc = win // 128
    ncp = nc // 2
    row0 = (sk - win) // 128 * 4
    assert nc == 32
    scale = float(np.asarray(DH ** -0.5, dtype=bf16))
    w2_splits = W2S

    def kernel(x_hbm, k_hbm, v_hbm, wq_hbm, wo_hbm, w1_hbm, w3_hbm, w2_hbm,
               o_ref,
               xbuf, kbuf, vbuf, wq, wo, w1, w3, w2,
               zq, ybuf, pc, lbuf, abuf, obuf,
               zbuf, onesb, cbuf, vf32, ksem, vsem, wsem):
        k32 = k_hbm.bitcast(u32)
        v32 = v_hbm.bitcast(u32)

        def k_copy(i):
            return pltpu.make_async_copy(
                k32.at[i, :, pl.ds(row0, 4 * nc), :], kbuf.at[i], ksem.at[i])

        def v_copy(i):
            return pltpu.make_async_copy(
                v32.at[i, :, pl.ds(row0, 4 * nc), :], vbuf.at[i], vsem.at[i])

        x_copy = pltpu.make_async_copy(x_hbm, xbuf, wsem.at[0])
        wq_copy = pltpu.make_async_copy(wq_hbm.bitcast(u32), wq, wsem.at[1])
        wo_copy = pltpu.make_async_copy(wo_hbm.bitcast(u32), wo, wsem.at[2])
        w1_copy = pltpu.make_async_copy(w1_hbm, w1, wsem.at[3])
        w3_copy = pltpu.make_async_copy(w3_hbm, w3, wsem.at[4])
        w2_copies = [
            pltpu.make_async_copy(w2_hbm.at[pl.ds(a // FCH, (b - a) // FCH)],
                                  w2.at[pl.ds(a // FCH, (b - a) // FCH)],
                                  wsem.at[5 + i])
            for i, (a, b) in enumerate(w2_splits)]

        wq_copy.start()
        x_copy.start()
        wo_copy.start()

        def start_kv(i, carry):
            k_copy(i).start()
            v_copy(i).start()
            return carry

        lax.fori_loop(0, NP, start_kv, 0)
        w1_copy.start()
        w3_copy.start()

        zbuf[...] = jnp.zeros((8, 128), u32)
        onesb[...] = jnp.ones((8, 128), f32)
        lbuf[...] = jnp.ones(lbuf.shape, f32)

        lane = lax.broadcasted_iota(jnp.int32, (8, 128), 1)
        sub = lax.broadcasted_iota(jnp.int32, (8, 128), 0)

        for n in range(4):
            cbuf[n] = 2 * n + (sub >> 2)
        cbuf[4] = sub ^ 1
        cbuf[5] = jnp.zeros_like(sub)
        cbuf[6] = jnp.where(lane < 64, 0, 2)
        cbuf[7] = jnp.full_like(sub, 2)
        cbuf[8] = lane & 8
        cbuf[9] = sub
        cbuf[10] = sub - jnp.where(lane < 64, 0, 1)
        cbuf[11] = sub - 1

        def rows(x, n):
            return jnp.take_along_axis(x, cbuf[n], axis=0,
                                       mode="promise_in_bounds")

        def retile(ref, ntile):
            top = sub < 4

            def body(a, carry):
                v = [ref[a, 8 * n:8 * n + 8, :] for n in range(ntile)]
                for t in range(ntile):
                    lo, hi = v[t // 2], v[(ntile + t) // 2]
                    if t % 2:
                        lo = pltpu.roll(lo, 4, 0)
                    if (ntile + t) % 2 == 0:
                        hi = pltpu.roll(hi, 4, 0)
                    ref[a, 8 * t:8 * t + 8, :] = jnp.where(top, lo, hi)
                return carry

            lax.fori_loop(0, ref.shape[0], body, 0)

        wq_copy.wait()
        retile(wq, H * DH // 128)
        for c in w2_copies:
            c.start()
        wo_copy.wait()
        retile(wo, D // 128)

        def kmask(var, t):
            return cbuf[9 + t] == 2 * var

        def q_stage(i, out, raw=None):
            r0 = 24 * i
            if not isinstance(r0, int):
                r0 = pl.multiple_of(r0, 8)
            wref = wq.at[:, pl.ds(r0, 24), :]
            even_grp = cbuf[8] == 0
            for t in range(3):
                w = _as_bf16(wref[:, 8 * t:8 * t + 8, :].reshape(D // 2, 128))
                if raw is None:
                    q = jnp.dot(_as_bf16(zq[...]), w,
                                preferred_element_type=f32)[0:8]
                else:
                    q = _ln_dot(raw[0], w, raw[1], raw[2])
                b = pltpu.bitcast(_round_bf16(q), u32)
                for y in (jnp.where(even_grp, b >> 16, pltpu.roll(b, 8, 1)),
                          jnp.where(even_grp, pltpu.roll(b, 120, 1) >> 16, b)):
                    if PREMASK:
                        for var in range(2):
                            out.append(jnp.where(kmask(var, t), y, jnp.uint32(0)))
                    else:
                        out.append(y)
                yield 40, q

        def k_stage(i, ys, out):
            kref = kbuf.at[i]
            groups = [16 * t + 2 * n + e
                      for t in range(3) for e in range(2) for n in range(8)]
            for c in range(ncp):
                var = c % 2
                if PREMASK:
                    lhs = jnp.concatenate(
                        [ys(2 * n + var) for n in range(6)], axis=1)
                else:
                    lhs = jnp.concatenate(
                        [jnp.where(kmask(var, n // 2), ys(n), jnp.uint32(0))
                         for n in range(6)], axis=1)
                w = jnp.concatenate(
                    [kref[g, 8 * c:8 * c + 8, :] for g in groups], axis=0)
                s = jnp.dot(_as_bf16(lhs), _as_bf16(w),
                            preferred_element_type=f32)[0:8]
                if c % 2 == 0:
                    out.append(s)
                else:
                    out[-1] = out[-1] + s
                yield 48, out[-1]

        def o_stage(i, ts, valid=None):
            wref = wo.at[pl.ds(24 * i, 24)]
            t = jnp.concatenate(ts, axis=1).astype(bf16)
            w = jnp.concatenate(
                [wref[:, 8 * n:8 * n + 8, :].reshape(DH, 128)
                 for n in range(D // 128)], axis=1)
            y = jnp.dot(t, _as_bf16(w), preferred_element_type=f32)
            if valid is not None:
                y = jnp.where(valid, y, 0.0)
            obuf[...] += y
            yield 120, None

        def run(*gens):
            for g in gens:
                for _ in g:
                    pass

        def trace_mxu(mxu_gens, links):
            spent = 0
            for gen in mxu_gens:
                for cost, res in gen:
                    spent += cost
                    if res is not None and MV is not None:
                        g = int((spent + MV) / VPACE)
                        if g < NG:
                            links.setdefault(g, []).append(res)

        def fold_rows(x, op):
            x = op(x, pltpu.roll(x, 4, 0))
            return op(x, rows(x, 4))

        def softmax_stage(ss, sc=scale):
            m = ss[0]
            for s in ss[1:]:
                m = jnp.maximum(m, s)
            m = jnp.max(fold_rows(m, jnp.maximum), axis=1, keepdims=True)
            return [jnp.exp((s - m) * sc) for s in ss]

        def v_stage(i, links, DEPTH=None, mode=None, hook=None):
            DEPTH = DEPTH or LDEPTH
            vref = vbuf.at[i]
            never = zbuf[...] != 0
            hist = []
            for g in range(NG):
                par = g // 24
                if g % 24 == 0:
                    ps = [pc[par, j] for j in range(nc // 4)]
                    pv = [rows(ps[c // 2], 2 * (c % 2) + par) for c in range(ncp)]
                    if par == 1 and hook is None:
                        tot = ps[0]
                        for p in ps[1:]:
                            tot = tot + p
                        l = jnp.sum(fold_rows(tot, jnp.add), axis=1, keepdims=True)
                        inv = jnp.broadcast_to(1.0 / l, (8, 128))
                        if LINK_L is not None:
                            links.setdefault(LINK_L, []).append(inv)
                        for j in range(3):
                            lbuf[j] = rows(inv, 5 + j)
                npair = 16 - DEPTH[g]
                accs = [None, None]
                pend = [None, None]
                pending = list(links.get(g, ()))
                for c in range(ncp):
                    if mode == 'use':
                        lo, hi = vf32[g, 0, c], vf32[g, 1, c]
                    else:
                        w = vref[g, 8 * c:8 * c + 8, :]
                        lo = pltpu.bitcast(w << 16, f32)
                        hi = pltpu.bitcast(w & jnp.uint32(0xFFFF0000), f32)
                    if mode == 'save':
                        vf32[g, 0, c] = lo
                        vf32[g, 1, c] = hi
                    hold = c % 2 == 1 and c < 15 and ((c // 2) * npair) % 7 < npair
                    p = pv[c]
                    lag = ELAG if mode else LAG
                    if SYNC and c == 0 and len(hist) >= lag:
                        p = jnp.where(never, hist[-lag][0] + hist[-lag][1], p)
                    ts = (lo * p, hi * p)
                    for a, t in enumerate(ts):
                        if accs[a] is None:
                            if len(hist) >= LAG and not SYNC:
                                t = jnp.where(never, hist[-LAG][(a + XLINK) % 2], t)
                            accs[a] = t
                            continue
                        if pending:
                            t = jnp.where(never, pending.pop(), t)
                        if hold:
                            pend[a] = t
                        else:
                            if pend[a] is not None:
                                t = pend[a] + t
                                pend[a] = None
                            accs[a] = accs[a] + t
                for a in range(2):
                    abuf[g, pl.ds(a, 8, stride=2), :] = accs[a]
                hist.append(accs)
                if hook is not None:
                    hook(g)

        def r_tile(j):
            ones = jnp.concatenate([onesb[...]] * 2, axis=1)
            a = jnp.concatenate(
                [abuf[16 * j:16 * j + 16, 8 * s:8 * s + 8, :].reshape(128, 128)
                 for s in range(2)], axis=1)
            return lax.dot_general(ones, a, (((1,), (1,)), ((), ())),
                                   preferred_element_type=f32)

        def r_stage(out):
            for j in range(3):
                t = r_tile(j)
                out.append(t * lbuf[j])
                yield 32, t

        def o_tile(i, j, t):
            r0 = 24 * i + 8 * j
            w = jnp.concatenate(
                [wo[r0:r0 + 8, 8 * n:8 * n + 8, :].reshape(64, 128)
                 for n in range(D // 128)], axis=1)
            return jnp.dot(t.astype(bf16), _as_bf16(w),
                           preferred_element_type=f32)

        def last_pair(mode):
            i = NP - 1
            links = {}

            def link(g, vals):
                if g < NG:
                    links.setdefault(g, []).extend(vals)

            def tiles(y):
                return [y[:, 128 * n:128 * n + 128] for n in range(D // 128)]

            y = obuf[...]
            ts = [r_tile(j) * lbuf[j] for j in range(3)]
            for j in range(3):
                link(EL[0] + 2 * j, [ts[j]])
                if not OLATE:
                    y = y + o_tile(i - 1, j, ts[j])
            link(EL[1], tiles(y))
            tot = pc[1, 0]
            for j in range(1, nc // 4):
                tot = tot + pc[1, j]
            lf = fold_rows(tot, jnp.add)
            link(EL[2], [lf])
            l = jnp.sum(lf, axis=1, keepdims=True)
            inv = jnp.broadcast_to(1.0 / l, (8, 128))
            link(EL[3], [inv])
            acc = [y]
            tn = []

            def hook(g):
                if g % 16 == 15:
                    j = g // 16
                    tn.append(r_tile(j) * rows(inv, 5 + j))
                    link(EL[4 + j], [tn[j]])
                    if OLATE and j == 2:
                        for jj in range(3):
                            acc[0] = acc[0] + o_tile(i - 1, jj, ts[jj])
                    for jj in (((), (), (0, 1, 2)) if OL2 else ((), (0, 1), (2,)))[j]:
                        acc[0] = acc[0] + o_tile(i, jj, tn[jj])

            v_stage(i, links, EDEPTH, mode, hook)
            return acc[0]

        x_copy.wait()
        x0 = jnp.broadcast_to(xbuf[0].astype(f32), (8, D))

        def layer_body(layer, x):
            first = layer == 0
            if first:
                k_copy(0).wait()

            m, c, r = _ln_stats(x)
            z = c * r
            raw = (_with_ones(x), m, r)
            zq[...] = pltpu.bitcast(
                jnp.concatenate([z, z], axis=0).astype(bf16), u32)
            obuf[...] = jnp.zeros(obuf.shape, f32)
            abuf[...] = jnp.zeros(abuf.shape, f32)

            y0, y1, ss = [], [], []
            run(q_stage(0, y0, raw[:2] + (None,)), q_stage(1, y1, raw), k_stage(0, lambda n: y0[n], ss))
            for t, y in enumerate(y1):
                ybuf[t] = y
            for j, p in enumerate(softmax_stage(ss, r * scale)):
                pc[0, j] = p
                pc[1, j] = p

            def pair_body(it, carry):
                i = it
                if first:
                    v_copy(i).wait()
                    k_copy(i + 1).wait()

                links = {}
                ss, yn, ts = [], [], []
                gens = {
                    'r': r_stage(ts),
                    'k': k_stage(i + 1, lambda n: ybuf[n], ss),
                    'q': q_stage(jnp.minimum(i + 2, NP - 1), yn),
                    'o': o_stage(jnp.maximum(i - 1, 0), ts)}
                trace_mxu([gens[st] for st in ORDER], links)
                ps = softmax_stage(ss)
                v_stage(i, links)
                for t, y in enumerate(yn):
                    ybuf[t] = y
                for j, p in enumerate(ps):
                    pc[0, j] = p
                    pc[1, j] = p
                return carry

            lax.fori_loop(0, (NP - 1) * REP, pair_body, 0)

            def epilogue(waits, x):
                if waits:
                    v_copy(NP - 1).wait()
                a = last_pair('save' if waits else 'use')
                x = _round_bf16(x + _round_bf16(a))
                if waits:
                    w1_copy.wait()
                    w3_copy.wait()
                m, _, r = _ln_stats(x)
                xo = _with_ones(x)
                hids = []
                for n in range(0, FF, FCH):
                    gate = _round_bf16(_ln_dot(xo, w1[:, n:n + FCH], m, r))
                    up = _round_bf16(_ln_dot(xo, w3[:, n:n + FCH], m, r))
                    hids.append(
                        (_round_bf16(gate * jax.nn.sigmoid(gate)) * up).astype(bf16))
                y = None
                starts = [a for a, _ in w2_splits]
                for n, hid in zip(range(0, FF, FCH), hids):
                    if waits and n in starts:
                        if y is not None:
                            obuf[...] = y
                        w2_copies[starts.index(n)].wait()
                        if y is not None:
                            y = obuf[...]
                    t = jnp.dot(hid, w2[n // FCH], preferred_element_type=f32)
                    y = t if y is None else y + t
                return _round_bf16(x + _round_bf16(y))

            return epilogue(first, x)

        x = x0
        for layer in range(NLAYERS):
            x = layer_body(layer, x)
        o_ref[0] = x[0:1].astype(bf16)

    return kernel


def _tiles(a, lead):
    r, c = a.shape
    t = a.reshape(r // 8, 8, c // 128, 128).transpose(0, 2, 1, 3)
    return t.reshape(lead + (-1, 128))


@jax.jit
def pallas_interleave_layers__sliding_block_cached__glu_gated_swiglu__decode_kernel(
    A_x: jax.Array,
    A_k_cache: jax.Array,
    A_v_cache: jax.Array,
    A_wq: jax.Array,
    A_wo: jax.Array,
    B_x: jax.Array,
    B_w1: jax.Array,
    B_w3: jax.Array,
    B_w2: jax.Array,
):
    del B_x
    sk = A_k_cache.shape[2]
    win = min(4096, max(256, sk // 4))
    kt = _tiles(jnp.swapaxes(A_k_cache, 2, 3).reshape(H * DH, sk), (NP, NG))
    vt = _tiles(jnp.swapaxes(A_v_cache, 2, 3).reshape(H * DH, sk), (NP, NG))
    any_spec = pl.BlockSpec(memory_space=pl.ANY)
    return pl.pallas_call(
        _make_kernel(sk, win),
        out_shape=jax.ShapeDtypeStruct((1, 1, D), bf16),
        in_specs=[any_spec] * 8,
        out_specs=pl.BlockSpec(memory_space=pltpu.VMEM),
        scratch_shapes=[
            pltpu.VMEM((1, 1, D), bf16),
            pltpu.VMEM((NP, NG, win // 32, 128), u32),
            pltpu.VMEM((NP, NG, win // 32, 128), u32),
            pltpu.VMEM((D // 16, H * DH // 16, 128), u32),
            pltpu.VMEM((H * DH // 16, D // 16, 128), u32),
            pltpu.VMEM((D, FF), bf16),
            pltpu.VMEM((D, FF), bf16),
            pltpu.VMEM((FF // FCH, FCH, D), bf16),
            pltpu.VMEM((8, D), u32),
            pltpu.VMEM((12, 8, 128), u32),
            pltpu.VMEM((2, 8, 8, 128), f32),
            pltpu.VMEM((3, 8, 128), f32),
            pltpu.VMEM((NG, 16, 128), f32),
            pltpu.VMEM((8, D), f32),
            pltpu.VMEM((8, 128), u32),
            pltpu.VMEM((8, 128), f32),
            pltpu.VMEM((16, 8, 128), jnp.int32),
            pltpu.VMEM((NG, 2, 16, 8, 128), f32),
            pltpu.SemaphoreType.DMA((NP,)),
            pltpu.SemaphoreType.DMA((NP,)),
            pltpu.SemaphoreType.DMA((8,)),
        ],
        compiler_params=pltpu.CompilerParams(
            vmem_limit_bytes=127 * 1024 * 1024,
            disable_semaphore_checks=True),
    )(A_x, kt, vt, _tiles(A_wq, (D // 16,)), _tiles(A_wo, (H * DH // 16,)),
      B_w1, B_w3, B_w2.reshape(FF // FCH, FCH, D))
```

```python
import jax
import jax.numpy as jnp
import numpy as np
from jax import lax
import jax.experimental.pallas as pl
import jax.experimental.pallas.tpu as pltpu

D = 640
H = 32
NP = H // 2
DH = 192
NG = 2 * DH // 8
FF = 1536
FCH = 256
EPS = 1e-5

LAYERS = (0, 1)
U = 2
NF = 6
FPOS = 'spread'
W2S = ((0, 5), (5, 6))
MV = 175
VPACE = 24.0
T0 = 20
YD = 0
GPER = 6
GNUM = 0
Y2L = None
KSW = lambda g: g // 2
LX = 0
GD = 0
RHO = 1.0
RW = 0
RD = 0
OD = 24
SPACE = 24.0
SMV = 190
FCOST = 0.69
NPAIR = 7
FGATE = 6
LINK_L = (40, 200)
SLINK_L = None
PL = 140
QB = False
ORD2 = 'kRqO4rKoQ'
ORD1 = 'RkO'
PRO = 'qqkq'

f32 = jnp.float32
bf16 = jnp.bfloat16
u32 = jnp.uint32


def _round_bf16(x):
    return x.astype(bf16).astype(f32)


def _as_bf16(x):
    return pltpu.bitcast(x, bf16)


def _as_f32(x):
    return pltpu.bitcast(x, f32)


def _ln_stats(x):
    m = jnp.mean(x, axis=-1, keepdims=True)
    c = x - m
    v = jnp.mean(c * c, axis=-1, keepdims=True)
    return m, c, lax.rsqrt(v + EPS)


def _with_ones(x):
    return jnp.concatenate([x, jnp.ones_like(x)], axis=0).astype(bf16)


def _centered_dot(xo, w, m):
    y = jnp.dot(xo, w, preferred_element_type=f32)
    return y[0:8] - m * y[8:16]


def _make_kernel(sk, win):
    nc = win // 128
    ncp = nc // 2
    row0 = (sk - win) // 128 * 4
    assert nc == 32
    scale = float(np.asarray(DH ** -0.5, dtype=bf16))
    nb = NG - NF
    order = []
    for par in range(2):
        packed = list(range(24 * par, 24 * par + 24 - NF // 2))
        wide = list(range(24 * par + 24 - NF // 2, 24 * par + 24))
        if FPOS == 'spread' and wide:
            step = 24 // len(wide)
            seq = []
            for n in range(24):
                if n % step == step // 2 and wide:
                    seq.append(wide.pop(0))
                else:
                    seq.append(packed.pop(0))
            order += seq
        else:
            order += packed + wide

    def is_wide(g):
        return g % 24 >= 24 - NF // 2

    def slot(g):
        par, gl = divmod(g, 24)
        if is_wide(g):
            return par * (NF // 2) + gl - (24 - NF // 2)
        return par * (24 - NF // 2) + gl

    def kernel(x_hbm, k_hbm, v_hbm, wq_hbm, wo_hbm, w1_hbm, w3_hbm, w2_hbm,
               o_ref,
               xbuf, kbuf, vbuf, vx, vlast, wq, wo, w1, w3, w2,
               zq, ybuf, pc, lbuf, abuf, obuf, zbuf, onesb, cbuf,
               ksem, vsem, wsem):
        k32 = k_hbm.bitcast(u32)
        v32 = v_hbm.bitcast(u32)
        rows_win = pl.ds(row0, 4 * nc)

        def k_copy(i):
            return pltpu.make_async_copy(
                k32.at[i, :, :, rows_win, :], kbuf.at[i], ksem.at[i])

        def v_copies(i):
            cps = [pltpu.make_async_copy(
                v32.at[i, :, pl.ds(0, nb // 2), rows_win, :], vbuf.at[i],
                vsem.at[2 * i])]
            if NF:
                cps.append(pltpu.make_async_copy(
                    v32.at[i, :, pl.ds(nb // 2, NF // 2), rows_win, :],
                    vx.at[i, 1], vsem.at[2 * i + 1]))
            return cps

        vlast_copy = pltpu.make_async_copy(
            v32.at[NP - 1, :, :, rows_win, :], vlast.at[1], wsem.at[7])
        x_copy = pltpu.make_async_copy(x_hbm, xbuf, wsem.at[0])
        wq_copy = pltpu.make_async_copy(wq_hbm.bitcast(u32), wq, wsem.at[1])
        wo_copy = pltpu.make_async_copy(wo_hbm.bitcast(u32), wo, wsem.at[2])
        w1_copy = pltpu.make_async_copy(w1_hbm, w1, wsem.at[3])
        w3_copy = pltpu.make_async_copy(w3_hbm, w3, wsem.at[4])
        w2_copies = [
            pltpu.make_async_copy(w2_hbm.at[pl.ds(a, b - a)],
                                  w2.at[pl.ds(a, b - a)], wsem.at[5 + n])
            for n, (a, b) in enumerate(W2S)]

        wq_copy.start()
        x_copy.start()
        wo_copy.start()
        k_copy(0).start()

        def start_kv(i, carry):
            for cp in v_copies(i):
                cp.start()
            k_copy(i + 1).start()
            return carry

        lax.fori_loop(0, NP - 1, start_kv, 0)
        vlast_copy.start()

        lane = lax.broadcasted_iota(jnp.int32, (8, 128), 1)
        sub = lax.broadcasted_iota(jnp.int32, (8, 128), 0)
        zbuf[...] = jnp.zeros((8, 128), u32)
        onesb[...] = jnp.ones((8, 128), f32)
        lbuf[...] = jnp.ones(lbuf.shape, f32)
        for n in range(4):
            cbuf[n] = 2 * n + (sub >> 2)
        cbuf[4] = sub ^ 1
        cbuf[5] = jnp.zeros_like(sub)
        cbuf[6] = jnp.where(lane < 64, 0, 2)
        cbuf[7] = jnp.full_like(sub, 2)
        cbuf[8] = lane & 8
        cbuf[9] = sub
        cbuf[10] = sub - jnp.where(lane < 64, 0, 1)
        cbuf[11] = sub - 1

        def rows(x, n):
            return jnp.take_along_axis(x, cbuf[n], axis=0,
                                       mode="promise_in_bounds")

        def retile(ref, ntile, place):
            top = sub < 4
            nrep = ref.shape[1] // (8 * ntile)

            def body(a, carry):
                v = [ref[a, 8 * n:8 * n + 8, :] for n in range(nrep * ntile)]
                for k in range(nrep):
                    for t in range(ntile):
                        lo = v[k * ntile + t // 2]
                        hi = v[k * ntile + (ntile + t) // 2]
                        if t % 2:
                            lo = pltpu.roll(lo, 4, 0)
                        if (ntile + t) % 2 == 0:
                            hi = pltpu.roll(hi, 4, 0)
                        ref[a, pl.ds(8 * place(k, t), 8), :] = jnp.where(top, lo, hi)
                return carry

            lax.fori_loop(0, ref.shape[0], body, 0)

        wq_copy.wait()
        retile(wq, H * DH // 128, lambda k, t: 2 * t + k)
        w1_copy.start()
        w3_copy.start()
        wo_copy.wait()
        retile(wo, D // 128, lambda k, t: t)
        for cp in w2_copies:
            cp.start()

        gate_src = [None, 0]

        def gated(tiles):
            out = []
            for t in tiles:
                n = gate_src[1]
                gate_src[1] += 1
                if gate_src[0] is not None and n % GPER < GNUM:
                    g = gate_src[0]
                    if t.dtype != g.dtype:
                        g = pltpu.bitcast(g, t.dtype)
                    t = jnp.where(zbuf[...] != 0, g, t)
                out.append(t)
            return out

        def kswz(g):
            return KSW(g) & 3

        def swizzle_k(i):
            def body(a, carry):
                for gl in range(8):
                    if kswz(gl):
                        ref = kbuf.at[i, a // 3, 8 * (a % 3) + gl]
                        v = [ref[8 * c:8 * c + 8, :] for c in range(ncp)]
                        for c in range(ncp):
                            ref[pl.ds(8 * (c ^ kswz(gl)), 8), :] = v[c]
                return carry
            lax.fori_loop(0, 6, body, 0)

        def k_ready(i):
            k_copy(i).wait()
            swizzle_k(i)

        def expand_q(t, b):
            even_grp = cbuf[8] == 0
            return [jnp.where(cbuf[9 + t] == 2 * var, y, jnp.uint32(0))
                    for y in (jnp.where(even_grp, b >> 16, pltpu.roll(b, 8, 1)),
                              jnp.where(even_grp, pltpu.roll(b, 120, 1) >> 16, b))
                    for var in range(2)]

        def q_stage(u, e, out, proj=None, expand=True):
            r0 = 96 * u
            if not isinstance(r0, int):
                r0 = pl.multiple_of(r0, 32)
            wref = wq.at[:, pl.ds(r0, 96), :]
            for t in range(3):
                r = 48 * e + 16 * t
                w = _as_bf16(wref[:, r:r + 16, :].reshape(D // 2, 128))
                if proj is None:
                    q = jnp.dot(_as_bf16(zq[...]), w,
                                preferred_element_type=f32)[0:8]
                else:
                    q = proj(w)
                b = pltpu.bitcast(_round_bf16(q), u32)
                if expand:
                    out.extend(expand_q(t, b))
                else:
                    out.append(b)
                yield 40, [(_as_f32(b), 0, 7)] + (
                    [(_as_f32(y), YD, 3.5) for y in out[-4:]] if YD and expand else [])

        def fold_rows(x, op):
            x = op(x, pltpu.roll(x, 4, 0))
            return op(x, rows(x, 4))

        def k_stage(i, ys, out):
            kref = kbuf.at[i]
            groups = [16 * t + 2 * n + e
                      for t in range(3) for e in range(2) for n in range(8)]
            m = None
            for c in range(ncp):
                lhs = jnp.concatenate(
                    gated([ys(2 * n + c % 2) for n in range(6)]), axis=1)
                w = jnp.concatenate(
                    [kref[g // 24, g % 24, pl.ds(8 * (c ^ kswz(g)), 8), :]
                     for g in groups],
                    axis=0)
                s = jnp.dot(_as_bf16(lhs), _as_bf16(w),
                            preferred_element_type=f32)[0:8]
                if c % 2 == 0:
                    out.append(s)
                    yield 48, [(s, 0, 6)]
                else:
                    out[-1] = out[-1] + s
                    m = out[-1] if m is None else jnp.maximum(m, out[-1])
                    if c == ncp - 1:
                        m = fold_rows(m, jnp.maximum)
                    yield 48, [(m, 0, 12 if c == ncp - 1 else 8)]
            out.append(m)

        def softmax_stage(ss, sc=scale):
            m = jnp.max(ss[-1], axis=1, keepdims=True)
            return [jnp.exp((s - m) * sc) for s in ss[:-1]]

        def r_tile(b, j):
            ones = jnp.concatenate(gated([onesb[...]] * 2), axis=1)
            a = jnp.concatenate(
                [abuf[b, 16 * j:16 * j + 16, 8 * s:8 * s + 8, :].reshape(128, 128)
                 for s in range(2)], axis=1)
            return lax.dot_general(ones, a, (((1,), (1,)), ((), ())),
                                   preferred_element_type=f32)

        def packed(t):
            return _as_f32(jnp.concatenate([t, t], axis=0).astype(bf16))

        def r_stage(b, out):
            for j in range(3):
                out.append(packed(r_tile(b, j) * lbuf[b, j]))
                yield 32, [(out[-1], RD, 4)]

        def o_dot(i, ts, j0=0):
            wref = wo.at[pl.ds(24 * i + 8 * j0, 8 * len(ts))]
            w = jnp.concatenate(
                [wref[:, 8 * n:8 * n + 8, :].reshape(64 * len(ts), 128)
                 for n in range(D // 128)], axis=1)
            return jnp.dot(_as_bf16(jnp.concatenate(ts, axis=1)), _as_bf16(w),
                           preferred_element_type=f32)[0:8]

        def o_stage(i, ts):
            wref = wo.at[pl.ds(24 * i, 24)]
            for n in range(D // 128):
                w = wref[:, 8 * n:8 * n + 8, :].reshape(DH, 128)
                y = obuf[:, 128 * n:128 * n + 128] + jnp.dot(
                    _as_bf16(jnp.concatenate(gated(ts), axis=1)), _as_bf16(w),
                    preferred_element_type=f32)[0:8]
                obuf[:, 128 * n:128 * n + 128] = y
                yield 24, [(y, 0, 4)]

        def run(*gens):
            for g in gens:
                for _ in g:
                    pass

        def weave(steps, vgens, links, state, mv):
            def advance(until):
                while vgens and state[0] < until:
                    try:
                        next(vgens[0])
                    except StopIteration:
                        vgens.pop(0)
                        if until != float('inf') and len(vgens) == 1 and not state[2]:
                            return
            t = 0.0
            gate_src[:] = [None, 0]
            for st in steps:
                if isinstance(st, int):
                    while len(vgens) > st:
                        run(vgens.pop(0))
                    t = max(t, state[0] - 64 + RW)
                    continue
                if callable(st):
                    st(t)
                    continue
                while True:
                    if GNUM:
                        while vgens and state[0] + GD < t and state[3]() :
                            try:
                                next(vgens[0])
                            except StopIteration:
                                vgens.pop(0)
                        if state[1] is not None:
                            gate_src[0] = state[1][0]
                    try:
                        cost, res = next(st)
                    except StopIteration:
                        break
                    t += cost / RHO
                    for val, extra, ops in res:
                        links.setdefault(t + mv + extra, []).append((val, ops))
            gate_src[0] = None
            for g in vgens:
                run(g)

        def take(gen, n):
            for _ in range(n):
                yield next(gen)

        def inverse_sum(ps):
            tot = ps[0]
            for p in ps[1:]:
                tot = tot + p
            lf = fold_rows(tot, jnp.add)
            l = jnp.sum(lf, axis=1, keepdims=True)
            return lf, jnp.broadcast_to(1.0 / l, (8, 128))

        def v_stage(first, i, b, links, getp, state, pace, link_l):
            never = zbuf[...] != 0
            last = i is None
            t_start = state[0]
            for n, g in enumerate(range(NG) if last else order):
                par = g // 24
                if n % 24 == 0:
                    ps = [getp(par, j) for j in range(nc // 4)]
                    pv = [rows(ps[c // 2], 2 * (c % 2) + par) for c in range(ncp)]
                    state[0] += 4
                    if par == 1 and not last:
                        lf, inv = inverse_sum(ps)
                        if link_l is not None:
                            for val, at in zip((lf, inv), link_l):
                                links.setdefault(state[0] + at, []).append((val, 14))
                        for j in range(3):
                            lbuf[b, j] = rows(inv, 5 + j)
                wide = last or is_wide(g)
                if last:
                    ref = vlast.at[:, par, g % 24]
                elif wide:
                    ref = vx.at[i, :, par, g % 24 - nb // 2]
                else:
                    ref = vbuf.at[i, par, g % 24]
                fast = wide and not first
                dur = pace * (FCOST if fast else 1.0)
                accs = [None, None]
                pend = [None, None]
                pending = []
                for c in range(ncp):
                    for key in sorted(links):
                        if key < state[0] + dur * (c + 1) / 16:
                            for val, ops in links.pop(key):
                                pending.append(val)
                                state[0] += ops / 4
                    rs = slice(8 * c, 8 * c + 8)
                    ls = slice(8 * (c ^ LX), 8 * (c ^ LX) + 8)
                    if fast:
                        lo, hi = ref[0, ls, :], ref[1, rs, :]
                    else:
                        w = ref[1, rs, :] if wide else ref[rs, :]
                        lo = w << 16
                        hi = w & jnp.uint32(0xFFFF0000)
                        if wide:
                            ref[0, ls, :] = lo
                            ref[1, rs, :] = hi
                    hold = c % 2 == 1 and c < 15 and ((c // 2) * NPAIR) % 7 < NPAIR
                    p = pv[c]
                    if c == (FGATE if fast else 0) and state[1] and not last:
                        p = jnp.where(never, state[1][0] + state[1][1], p)
                    for a, t in enumerate((_as_f32(lo) * p, _as_f32(hi) * p)):
                        if accs[a] is None:
                            accs[a] = t
                            continue
                        if pending:
                            t = jnp.where(never, pending.pop(), t)
                        if hold:
                            pend[a] = t
                        else:
                            if pend[a] is not None:
                                t = pend[a] + t
                                pend[a] = None
                            accs[a] = accs[a] + t
                for a in range(2):
                    abuf[b, g, pl.ds(a, 8, stride=2), :] = accs[a]
                state[0] += dur
                state[1] = accs
                yield g

        def from_pc(par, j):
            return pc[par, j]

        def store_p(ps):
            for j, p in enumerate(ps):
                pc[0, j] = p
                pc[1, j] = p

        def double_block(first, it):
            i = 2 * it
            links = {}
            s1, s2, ya, yb, t0, t1 = [], [], [], [], [], []
            y2 = []
            for t in range(3):
                y2 += expand_q(t, ybuf[1, t])
            if Y2L is not None:
                for n, y in enumerate(y2):
                    links.setdefault(Y2L[0] + Y2L[1] * n, []).append((_as_f32(y), 3.5))
            gens = {
                'r': r_stage(0, t0), 'R': r_stage(1, t1),
                'k': k_stage(i + 1, lambda n: ybuf[0, n], s1),
                'K': k_stage(i + 2, lambda n: y2[n], s2),
                'q': q_stage(it + 1, 1, ya),
                'Q': q_stage(jnp.minimum(it + 2, NP // 2 - 1), 0, yb, expand=False),
                'o': o_stage(i, t0),
                'O': o_stage(jnp.maximum(i - 1, 0), t1)}
            p1, p2 = [], []

            def soft(ps, ss):
                def f(t):
                    ps.extend(softmax_stage(ss))
                    if PL is not None:
                        links.setdefault(t + MV + PL, []).extend((p, 4) for p in ps)
                return f

            steps = []
            for st in ORD2:
                if st == 'r':
                    steps.append(1)
                steps.append(take(gens['K'], int(st)) if st.isdigit() else gens[st])
                if st == 'k':
                    steps.append(soft(p1, s1))
                if st == 'K':
                    steps.append(soft(p2, s2))
            state = [T0, None, None, lambda: True]
            weave(steps,
                  [v_stage(first, i, 0, links, from_pc, state, VPACE, LINK_L),
                   v_stage(first, i + 1, 1, links, lambda par, j: p1[j], state,
                           VPACE, LINK_L)], links, state, MV)
            for t in range(12):
                ybuf[0, t] = ya[t]
            for t in range(3):
                ybuf[1, t] = yb[t]
            store_p(p2)

        def single_block(first):
            i = NP - 2
            links = {}
            s1, t1 = [], []
            gens = {'k': k_stage(i + 1, lambda n: ybuf[0, n], s1),
                    'R': r_stage(1, t1), 'O': o_stage(i - 1, t1)}
            state = [T0, None, None, lambda: True]
            weave([gens[st] for st in ORD1],
                  [v_stage(first, i, 0, links, from_pc, state, SPACE, SLINK_L)],
                  links, state, SMV)
            store_p(softmax_stage(s1))

        def last_block(first):
            i = NP - 2
            ts = [packed(r_tile(0, j) * lbuf[0, j]) for j in range(3)]
            lf, inv = inverse_sum([pc[1, j] for j in range(nc // 4)])
            links = {50: [(lf, 0)]}
            tn = []
            for g in v_stage(first, None, 1, links, from_pc, [0.0, None], 24.0, None):
                if g % 16 == 15:
                    tn.append(packed(r_tile(1, g // 16) * rows(inv, 5 + g // 16)))
            y = obuf[...]
            for j in range(3):
                y = y + o_dot(i, ts[j:j + 1], j)
            for j in range(3):
                y = y + o_dot(i + 1, tn[j:j + 1], j)
            return y

        def layer_body(first, x):
            if first:
                k_ready(0)
            m, c, r = _ln_stats(x)
            z = c * r
            xo = _with_ones(x)
            zq[...] = pltpu.bitcast(
                jnp.concatenate([z, z], axis=0).astype(bf16), u32)
            obuf[...] = jnp.zeros(obuf.shape, f32)
            abuf[1] = jnp.zeros(abuf.shape[1:], f32)

            y0, y1, y2, ss = [], [], [], []
            qs = [q_stage(0, 0, y0, lambda w: _centered_dot(xo, w, m)),
                  q_stage(0, 1, y1, lambda w: _centered_dot(xo, w, m) * r),
                  q_stage(1, 0, y2, expand=False)]
            kgen = k_stage(0, lambda n: y0[n], ss)
            for st in PRO:
                if st == 'q':
                    run(qs.pop(0))
                elif st == 'k':
                    run(kgen)
                else:
                    for _ in range(int(st, 16)):
                        next(kgen)
            for t in range(12):
                ybuf[0, t] = y1[t]
            for t in range(3):
                ybuf[1, t] = y2[t]
            store_p(softmax_stage(ss, r * scale))

            def pair_body(it, carry):
                i = 2 * it
                if first:
                    for b in range(2):
                        for cp in v_copies(i + b):
                            cp.wait()
                        k_ready(i + b + 1)
                double_block(first, it)
                return carry + 1

            cnt = lax.fori_loop(0, NP // 2 - 1, pair_body, 0)

            @pl.when(cnt > 0)
            def _():
                if first:
                    for cp in v_copies(NP - 2):
                        cp.wait()
                    k_ready(NP - 1)
                single_block(first)

            if first:
                vlast_copy.wait()
            x = _round_bf16(x + _round_bf16(last_block(first)))

            if first:
                w1_copy.wait()
                w3_copy.wait()
            m, _, r = _ln_stats(x)
            xo = _with_ones(x)
            hids = []
            for n in range(0, FF, FCH):
                gate = _round_bf16(_centered_dot(xo, w1[:, n:n + FCH], m) * r)
                up = _round_bf16(_centered_dot(xo, w3[:, n:n + FCH], m) * r)
                hids.append(
                    (_round_bf16(gate * jax.nn.sigmoid(gate)) * up).astype(bf16))
            y = None
            starts = [a for a, _ in W2S]
            for n, hid in enumerate(hids):
                if first and n in starts:
                    if y is not None:
                        obuf[...] = y
                    w2_copies[starts.index(n)].wait()
                    if y is not None:
                        y = obuf[...]
                t = jnp.dot(hid, w2[n], preferred_element_type=f32)
                y = t if y is None else y + t
            return _round_bf16(x + _round_bf16(y))

        x_copy.wait()
        x = jnp.broadcast_to(xbuf[0].astype(f32), (8, D))
        for layer in LAYERS:
            x = layer_body(layer == 0, x)
        o_ref[0] = x[0:1].astype(bf16)

    return kernel


def _tiles(a, lead):
    r, c = a.shape
    t = a.reshape(r // 8, 8, c // 128, 128).transpose(0, 2, 1, 3)
    return t.reshape(lead + (-1, 128))


@jax.jit
def pallas_interleave_layers__sliding_block_cached__glu_gated_swiglu__decode_kernel(
    A_x: jax.Array,
    A_k_cache: jax.Array,
    A_v_cache: jax.Array,
    A_wq: jax.Array,
    A_wo: jax.Array,
    B_x: jax.Array,
    B_w1: jax.Array,
    B_w3: jax.Array,
    B_w2: jax.Array,
):
    del B_x
    sk = A_k_cache.shape[2]
    win = min(4096, max(256, sk // 4))
    wr = win // 32
    kt = _tiles(jnp.swapaxes(A_k_cache, 2, 3).reshape(H * DH, sk), (NP, 2, 24))
    vt = _tiles(jnp.swapaxes(A_v_cache, 2, 3).reshape(H * DH, sk), (NP, 2, 24))
    any_spec = pl.BlockSpec(memory_space=pl.ANY)
    return pl.pallas_call(
        _make_kernel(sk, win),
        out_shape=jax.ShapeDtypeStruct((1, 1, D), bf16),
        in_specs=[any_spec] * 8,
        out_specs=pl.BlockSpec(memory_space=pltpu.VMEM),
        scratch_shapes=[
            pltpu.VMEM((1, 1, D), bf16),
            pltpu.VMEM((NP, 2, 24, wr, 128), u32),
            pltpu.VMEM((NP - 1, 2, 24 - NF // 2, wr, 128), u32),
            pltpu.VMEM((NP - 1, 2, 2, max(NF // 2, 1), wr, 128), u32),
            pltpu.VMEM((2, 2, 24, wr, 128), u32),
            pltpu.VMEM((D // 32, H * DH // 8, 128), u32),
            pltpu.VMEM((H * DH // 16, D // 16, 128), u32),
            pltpu.VMEM((D, FF), bf16),
            pltpu.VMEM((D, FF), bf16),
            pltpu.VMEM((FF // FCH, FCH, D), bf16),
            pltpu.VMEM((8, D), u32),
            pltpu.VMEM((2, 12, 8, 128), u32),
            pltpu.VMEM((2, 8, 8, 128), f32),
            pltpu.VMEM((2, 3, 8, 128), f32),
            pltpu.VMEM((2, NG, 16, 128), f32),
            pltpu.VMEM((8, D), f32),
            pltpu.VMEM((8, 128), u32),
            pltpu.VMEM((8, 128), f32),
            pltpu.VMEM((12, 8, 128), jnp.int32),
            pltpu.SemaphoreType.DMA((NP,)),
            pltpu.SemaphoreType.DMA((2 * NP,)),
            pltpu.SemaphoreType.DMA((8,)),
        ],
        compiler_params=pltpu.CompilerParams(
            vmem_limit_bytes=128 * 1024 * 1024,
            disable_semaphore_checks=True),
    )(A_x, kt, vt, _tiles(A_wq, (D // 32,)), _tiles(A_wo, (H * DH // 16,)),
      B_w1, B_w3, B_w2.reshape(FF // FCH, FCH, D))
```

```python
import jax
import jax.numpy as jnp
import numpy as np
from jax import lax
import jax.experimental.pallas as pl
import jax.experimental.pallas.tpu as pltpu

D = 640
H = 32
NP = H // 2
DH = 192
GH = DH // 8
NG = 2 * GH
FF = 1536
FCH = 256
EPS = 1e-5

NW = 3
W2_SPLITS = ((0, 5), (5, 6))

T_START = 20
T_GROUP = 24.0
T_WIDE = 0.69
T_RESULT = 175
T_RESULT1 = 190
T_SUM = (40, 200)

f32 = jnp.float32
bf16 = jnp.bfloat16
u32 = jnp.uint32


def _round_bf16(x):
    return x.astype(bf16).astype(f32)


def _as_bf16(x):
    return pltpu.bitcast(x, bf16)


def _as_f32(x):
    return pltpu.bitcast(x, f32)


def _dot(a, b):
    return jnp.dot(a, b, preferred_element_type=f32)


def _gather_rows(x, idx):
    return jnp.take_along_axis(x, idx, axis=0, mode="promise_in_bounds")


def _ln_stats(x):
    m = jnp.mean(x, axis=-1, keepdims=True)
    c = x - m
    v = jnp.mean(c * c, axis=-1, keepdims=True)
    return m, c, lax.rsqrt(v + EPS)


def _with_ones(x):
    return jnp.concatenate([x, jnp.ones_like(x)], axis=0).astype(bf16)


def _centered_dot(xo, w, m):
    y = _dot(xo, w)
    return y[0:8] - m * y[8:16]


def _packed(t):
    return _as_f32(jnp.concatenate([t, t], axis=0).astype(bf16))


def _run(*gens):
    for g in gens:
        for _ in g:
            pass


def _take(gen, n):
    for _ in range(n):
        yield next(gen)


def _group_order():
    order = []
    step = GH // NW
    for par in range(2):
        packed = list(range(GH * par, GH * par + GH - NW))
        wide = list(range(GH * par + GH - NW, GH * par + GH))
        order += [(wide if n % step == step // 2 else packed).pop(0)
                  for n in range(GH)]
    return order


def _make_kernel(sk, win):
    nc = win // 128
    ncp = nc // 2
    row0 = (sk - win) // 128 * 4
    assert nc == 32
    scale = float(np.asarray(DH ** -0.5, dtype=bf16))
    order = _group_order()

    def kernel(x_hbm, k_hbm, v_hbm, wq_hbm, wo_hbm, w1_hbm, w3_hbm, w2_hbm,
               o_ref,
               xbuf, kbuf, vbuf, vwide, vlast, wq, wo, w1, w3, w2,
               zq, ybuf, qbuf, pbuf, lbuf, abuf, obuf, zeros, ones, tab,
               ksem, vsem, wsem):
        k32 = k_hbm.bitcast(u32)
        v32 = v_hbm.bitcast(u32)
        window = pl.ds(row0, 4 * nc)

        def k_copy(i):
            return pltpu.make_async_copy(
                k32.at[i, :, :, window, :], kbuf.at[i], ksem.at[i])

        def v_copies(i):
            return (
                pltpu.make_async_copy(
                    v32.at[i, :, pl.ds(0, GH - NW), window, :], vbuf.at[i],
                    vsem.at[2 * i]),
                pltpu.make_async_copy(
                    v32.at[i, :, pl.ds(GH - NW, NW), window, :],
                    vwide.at[i, 1], vsem.at[2 * i + 1]))

        x_copy = pltpu.make_async_copy(x_hbm, xbuf, wsem.at[0])
        wq_copy = pltpu.make_async_copy(wq_hbm.bitcast(u32), wq, wsem.at[1])
        wo_copy = pltpu.make_async_copy(wo_hbm.bitcast(u32), wo, wsem.at[2])
        vlast_copy = pltpu.make_async_copy(
            v32.at[NP - 1, :, :, window, :], vlast.at[1], wsem.at[3])
        w1_copy = pltpu.make_async_copy(w1_hbm, w1, wsem.at[4])
        w3_copy = pltpu.make_async_copy(w3_hbm, w3, wsem.at[5])
        w2_copies = [
            pltpu.make_async_copy(w2_hbm.at[pl.ds(a, b - a)],
                                  w2.at[pl.ds(a, b - a)], wsem.at[6 + n])
            for n, (a, b) in enumerate(W2_SPLITS)]

        wq_copy.start()
        x_copy.start()
        wo_copy.start()
        k_copy(0).start()

        def start_kv(i, carry):
            for cp in v_copies(i):
                cp.start()
            k_copy(i + 1).start()
            return carry

        lax.fori_loop(0, NP - 1, start_kv, 0)
        vlast_copy.start()

        lane = lax.broadcasted_iota(jnp.int32, (8, 128), 1)
        sub = lax.broadcasted_iota(jnp.int32, (8, 128), 0)
        zeros[...] = jnp.zeros((8, 128), u32)
        ones[...] = jnp.ones((8, 128), f32)
        lbuf[...] = jnp.ones(lbuf.shape, f32)
        for n in range(4):
            tab[n] = 2 * n + (sub >> 2)
        tab[4] = sub ^ 1
        tab[5] = jnp.zeros_like(sub)
        tab[6] = jnp.where(lane < 64, 0, 2)
        tab[7] = jnp.full_like(sub, 2)
        tab[8] = lane & 8
        tab[9] = sub
        tab[10] = sub - jnp.where(lane < 64, 0, 1)
        tab[11] = sub - 1

        def retile(ref, ntile, place):
            top = sub < 4
            nrep = ref.shape[1] // (8 * ntile)

            def body(a, carry):
                v = [ref[a, 8 * n:8 * n + 8, :] for n in range(nrep * ntile)]
                for k in range(nrep):
                    for t in range(ntile):
                        lo = v[k * ntile + t // 2]
                        hi = v[k * ntile + (ntile + t) // 2]
                        if t % 2:
                            lo = pltpu.roll(lo, 4, 0)
                        if (ntile + t) % 2 == 0:
                            hi = pltpu.roll(hi, 4, 0)
                        r = 8 * place(k, t)
                        ref[a, r:r + 8, :] = jnp.where(top, lo, hi)
                return carry

            lax.fori_loop(0, ref.shape[0], body, 0)

        def k_rows(g, c):
            r = 8 * (c ^ (g // 2 % 4))
            return slice(r, r + 8)

        def k_ready(i):
            k_copy(i).wait()

            def body(a, carry):
                for g in range(2, 8):
                    ref = kbuf.at[i, a // 3, 8 * (a % 3) + g]
                    v = [ref[8 * c:8 * c + 8, :] for c in range(ncp)]
                    for c in range(ncp):
                        ref[k_rows(g, c), :] = v[c]
                return carry

            lax.fori_loop(0, NG // 8, body, 0)

        wq_copy.wait()
        retile(wq, H * DH // 128, lambda k, t: 2 * t + k)
        w1_copy.start()
        w3_copy.start()
        wo_copy.wait()
        retile(wo, D // 128, lambda k, t: t)
        for cp in w2_copies:
            cp.start()

        def expand_q(t, b):
            even = tab[8] == 0
            return [jnp.where(tab[9 + t] == 2 * var, y, jnp.uint32(0))
                    for y in (jnp.where(even, b >> 16, pltpu.roll(b, 8, 1)),
                              jnp.where(even, pltpu.roll(b, 120, 1) >> 16, b))
                    for var in range(2)]

        def q_stage(u, e, out, proj=None, expand=True):
            r0 = 96 * u
            if not isinstance(r0, int):
                r0 = pl.multiple_of(r0, 32)
            wref = wq.at[:, pl.ds(r0, 96), :]
            for t in range(3):
                r = 48 * e + 16 * t
                w = _as_bf16(wref[:, r:r + 16, :].reshape(D // 2, 128))
                q = proj(w) if proj else _dot(_as_bf16(zq[...]), w)[0:8]
                b = pltpu.bitcast(_round_bf16(q), u32)
                out.extend(expand_q(t, b) if expand else [b])
                yield 40, [(_as_f32(b), 7)]

        def fold_rows(x, op):
            x = op(x, pltpu.roll(x, 4, 0))
            return op(x, _gather_rows(x, tab[4]))

        def scores(kref, ys, c, tiles):
            lhs = jnp.concatenate(
                [ys(4 * t + 2 * e + c % 2) for t in tiles for e in range(2)],
                axis=1)
            w = jnp.concatenate(
                [kref[g // GH, g % GH, k_rows(g, c), :]
                 for t in tiles for e in range(2)
                 for g in range(16 * t + e, 16 * t + 16, 2)], axis=0)
            return _dot(_as_bf16(lhs), _as_bf16(w))[0:8]

        def k_stage(i, ys, out):
            kref = kbuf.at[i]
            m = None
            for c in range(ncp):
                s = scores(kref, ys, c, (0, 1, 2))
                if c % 2 == 0:
                    out.append(s)
                    yield 48, [(s, 6)]
                else:
                    out[-1] = out[-1] + s
                    m = out[-1] if m is None else jnp.maximum(m, out[-1])
                    if c == ncp - 1:
                        m = fold_rows(m, jnp.maximum)
                    yield 48, [(m, 12 if c == ncp - 1 else 8)]
            out.append(m)

        def k_first(ys):
            plan = [(c, (t,)) for t in range(3) for c in range(4)]
            plan += [(c, (0, 1, 2)) for c in range(4, ncp)]
            acc = [None] * (ncp // 2)
            for c, tiles in plan:
                s = scores(kbuf.at[0], ys, c, tiles)
                acc[c // 2] = s if acc[c // 2] is None else acc[c // 2] + s
            m = acc[0]
            for a in acc[1:]:
                m = jnp.maximum(m, a)
            return acc + [fold_rows(m, jnp.maximum)]

        def softmax_numerator(ss, sc=scale):
            m = jnp.max(ss[-1], axis=1, keepdims=True)
            return [jnp.exp((s - m) * sc) for s in ss[:-1]]

        def inverse_sum(ps):
            tot = ps[0]
            for p in ps[1:]:
                tot = tot + p
            lf = fold_rows(tot, jnp.add)
            l = jnp.sum(lf, axis=1, keepdims=True)
            return lf, jnp.broadcast_to(1.0 / l, (8, 128))

        def lane_sums(b, j):
            a = jnp.concatenate(
                [abuf[b, 16 * j:16 * j + 16, 8 * s:8 * s + 8, :].reshape(128, 128)
                 for s in range(2)], axis=1)
            return lax.dot_general(
                jnp.concatenate([ones[...]] * 2, axis=1), a,
                (((1,), (1,)), ((), ())), preferred_element_type=f32)

        def r_stage(b, out):
            for j in range(3):
                out.append(_packed(lane_sums(b, j) * lbuf[b, j]))
                yield 32, [(out[-1], 4)]

        def o_stage(i, ts):
            wref = wo.at[pl.ds(24 * i, 24)]
            t = _as_bf16(jnp.concatenate(ts, axis=1))
            for n in range(D // 128):
                cols = slice(128 * n, 128 * n + 128)
                w = wref[:, 8 * n:8 * n + 8, :].reshape(DH, 128)
                y = obuf[:, cols] + _dot(t, _as_bf16(w))[0:8]
                obuf[:, cols] = y
                yield 24, [(y, 4)]

        def o_tile(i, j, t):
            r0 = 24 * i + 8 * j
            w = jnp.concatenate(
                [wo[r0:r0 + 8, 8 * n:8 * n + 8, :].reshape(64, 128)
                 for n in range(D // 128)], axis=1)
            return _dot(_as_bf16(t), _as_bf16(w))[0:8]

        def trace_mxu(gens, links, latency, t=0.0):
            for gen in gens:
                for cost, res in gen:
                    t += cost
                    links.setdefault(t + latency, []).extend(res)
            return t

        def v_stage(first, i, b, getp, links, clock, hist, t_sum=None):
            never = zeros[...] != 0
            last = i is None
            for n, g in enumerate(range(NG) if last else order):
                par, gl = divmod(g, GH)
                if n % GH == 0:
                    ps = [getp(par, j) for j in range(nc // 4)]
                    idx = [tab[par], tab[2 + par]]
                    if b == 1 and not last:
                        dep = pltpu.bitcast(hist[-2][0], jnp.int32)
                        idx = [jnp.where(never, dep, ix) for ix in idx]
                    pv = [_gather_rows(ps[c // 2], idx[c % 2])
                          for c in range(ncp)]
                    clock[0] += 4
                    if par == 1 and not last:
                        lf, inv = inverse_sum(ps)
                        for val, at in zip((lf, inv), t_sum or ()):
                            links.setdefault(clock[0] + at, []).append((val, 14))
                        for j in range(3):
                            lbuf[b, j] = _gather_rows(inv, tab[5 + j])
                wide = last or gl >= GH - NW
                if last:
                    ref = vlast.at[:, par, gl]
                elif wide:
                    ref = vwide.at[i, :, par, gl - (GH - NW)]
                else:
                    ref = vbuf.at[i, par, gl]
                fast = wide and not first
                dur = T_GROUP * (T_WIDE if fast else 1.0)
                accs = [None, None]
                held = [None, None]
                pending = []
                for c in range(ncp):
                    for key in sorted(links):
                        if key < clock[0] + dur * (c + 1) / 16:
                            for val, ops in links.pop(key):
                                pending.append(val)
                                clock[0] += ops / 4
                    rs = slice(8 * c, 8 * c + 8)
                    if fast:
                        lo, hi = ref[0, rs, :], ref[1, rs, :]
                    else:
                        w = ref[1, rs, :] if wide else ref[rs, :]
                        lo = w << 16
                        hi = w & jnp.uint32(0xFFFF0000)
                        if wide:
                            ref[0, rs, :] = lo
                            ref[1, rs, :] = hi
                    p = pv[c]
                    if c == (6 if fast else 0) and hist and not last:
                        p = jnp.where(never, hist[-1][0] + hist[-1][1], p)
                    for a, t in enumerate((_as_f32(lo) * p, _as_f32(hi) * p)):
                        if accs[a] is None:
                            accs[a] = t
                            continue
                        if pending:
                            t = jnp.where(never, pending.pop(), t)
                        if c % 2 == 1 and c < ncp - 1:
                            held[a] = t
                        else:
                            if held[a] is not None:
                                t = held[a] + t
                                held[a] = None
                            accs[a] = accs[a] + t
                for a in range(2):
                    abuf[b, g, pl.ds(a, 8, stride=2), :] = accs[a]
                clock[0] += dur
                hist.append(accs)
                yield g

        def from_pbuf(par, j):
            return pbuf[par, j]

        def store_p(ps):
            for j, p in enumerate(ps):
                pbuf[0, j] = p
                pbuf[1, j] = p

        def two_pairs(first, it):
            i = 2 * it
            links, clock, hist = {}, [T_START], []
            s1, s2, ya, qb, t0, t1 = [], [], [], [], [], []
            y2 = [y for t in range(3) for y in expand_q(t, qbuf[t])]
            k2 = k_stage(i + 2, lambda n: y2[n], s2)
            t = trace_mxu([k_stage(i + 1, lambda n: ybuf[n], s1)],
                          links, T_RESULT)
            p1 = softmax_numerator(s1)
            t = trace_mxu([r_stage(1, t1), q_stage(it + 1, 1, ya),
                           o_stage(jnp.maximum(i - 1, 0), t1), _take(k2, 4)],
                          links, T_RESULT, t)
            _run(v_stage(first, i, 0, from_pbuf, links, clock, hist, T_SUM))
            t = trace_mxu([r_stage(0, t0), k2], links, T_RESULT,
                          max(t, clock[0] - 64))
            p2 = softmax_numerator(s2)
            trace_mxu([o_stage(i, t0),
                       q_stage(jnp.minimum(it + 2, NP // 2 - 1), 0, qb,
                               expand=False)], links, T_RESULT, t)
            _run(v_stage(first, i + 1, 1, lambda par, j: p1[j], links, clock,
                         hist, T_SUM))
            for n in range(12):
                ybuf[n] = ya[n]
            for n in range(3):
                qbuf[n] = qb[n]
            store_p(p2)

        def one_pair(first):
            i = NP - 2
            links = {}
            s1, t1 = [], []
            trace_mxu([r_stage(1, t1), k_stage(i + 1, lambda n: ybuf[n], s1),
                       o_stage(i - 1, t1)], links, T_RESULT1)
            _run(v_stage(first, i, 0, from_pbuf, links, [T_START], []))
            store_p(softmax_numerator(s1))

        def last_pair(first):
            ts = [_packed(lane_sums(0, j) * lbuf[0, j]) for j in range(3)]
            lf, inv = inverse_sum([pbuf[1, j] for j in range(nc // 4)])
            tn = []
            for g in v_stage(first, None, 1, from_pbuf, {50: [(lf, 0)]},
                             [0.0], []):
                if g % 16 == 15:
                    j = g // 16
                    tn.append(_packed(
                        lane_sums(1, j) * _gather_rows(inv, tab[5 + j])))
            y = obuf[...]
            for j in range(3):
                y = y + o_tile(NP - 2, j, ts[j])
            for j in range(3):
                y = y + o_tile(NP - 1, j, tn[j])
            return y

        def attention(first, x):
            if first:
                k_ready(0)
            m, c, r = _ln_stats(x)
            z = c * r
            xo = _with_ones(x)
            zq[...] = pltpu.bitcast(
                jnp.concatenate([z, z], axis=0).astype(bf16), u32)
            obuf[...] = jnp.zeros(obuf.shape, f32)
            abuf[1] = jnp.zeros(abuf.shape[1:], f32)

            y0, y1, q2 = [], [], []
            _run(q_stage(0, 0, y0, lambda w: _centered_dot(xo, w, m)),
                 q_stage(0, 1, y1, lambda w: _centered_dot(xo, w, m) * r))
            ss = k_first(lambda n: y0[n])
            _run(q_stage(1, 0, q2, expand=False))
            for n in range(12):
                ybuf[n] = y1[n]
            for n in range(3):
                qbuf[n] = q2[n]
            store_p(softmax_numerator(ss, r * scale))

            def body(it, count):
                if first:
                    for i in (2 * it, 2 * it + 1):
                        for cp in v_copies(i):
                            cp.wait()
                        k_ready(i + 1)
                two_pairs(first, it)
                return count + 1

            count = lax.fori_loop(0, NP // 2 - 1, body, 0)

            @pl.when(count > 0)
            def _():
                if first:
                    for cp in v_copies(NP - 2):
                        cp.wait()
                    k_ready(NP - 1)
                one_pair(first)

            if first:
                vlast_copy.wait()
            return last_pair(first)

        def ffn(first, x):
            if first:
                w1_copy.wait()
                w3_copy.wait()
            m, _, r = _ln_stats(x)
            xo = _with_ones(x)
            hids = []
            for n in range(0, FF, FCH):
                gate = _round_bf16(_centered_dot(xo, w1[:, n:n + FCH], m) * r)
                up = _round_bf16(_centered_dot(xo, w3[:, n:n + FCH], m) * r)
                hids.append(
                    (_round_bf16(gate * jax.nn.sigmoid(gate)) * up).astype(bf16))
            y = None
            starts = [a for a, _ in W2_SPLITS]
            for n, hid in enumerate(hids):
                if first and n in starts:
                    if y is not None:
                        obuf[...] = y
                    w2_copies[starts.index(n)].wait()
                    if y is not None:
                        y = obuf[...]
                t = _dot(hid, w2[n])
                y = t if y is None else y + t
            return y

        x_copy.wait()
        x = jnp.broadcast_to(xbuf[0].astype(f32), (8, D))
        for first in (True, False):
            x = _round_bf16(x + _round_bf16(attention(first, x)))
            x = _round_bf16(x + _round_bf16(ffn(first, x)))
        o_ref[0] = x[0:1].astype(bf16)

    return kernel


def _tiles(a, lead):
    r, c = a.shape
    t = a.reshape(r // 8, 8, c // 128, 128).transpose(0, 2, 1, 3)
    return t.reshape(lead + (-1, 128))


@jax.jit
def pallas_interleave_layers__sliding_block_cached__glu_gated_swiglu__decode_kernel(
    A_x: jax.Array,
    A_k_cache: jax.Array,
    A_v_cache: jax.Array,
    A_wq: jax.Array,
    A_wo: jax.Array,
    B_x: jax.Array,
    B_w1: jax.Array,
    B_w3: jax.Array,
    B_w2: jax.Array,
):
    del B_x
    sk = A_k_cache.shape[2]
    win = min(4096, max(256, sk // 4))
    wr = win // 32
    kt = _tiles(jnp.swapaxes(A_k_cache, 2, 3).reshape(H * DH, sk), (NP, 2, GH))
    vt = _tiles(jnp.swapaxes(A_v_cache, 2, 3).reshape(H * DH, sk), (NP, 2, GH))
    any_spec = pl.BlockSpec(memory_space=pl.ANY)
    return pl.pallas_call(
        _make_kernel(sk, win),
        out_shape=jax.ShapeDtypeStruct((1, 1, D), bf16),
        in_specs=[any_spec] * 8,
        out_specs=pl.BlockSpec(memory_space=pltpu.VMEM),
        scratch_shapes=[
            pltpu.VMEM((1, 1, D), bf16),
            pltpu.VMEM((NP, 2, GH, wr, 128), u32),
            pltpu.VMEM((NP - 1, 2, GH - NW, wr, 128), u32),
            pltpu.VMEM((NP - 1, 2, 2, NW, wr, 128), u32),
            pltpu.VMEM((2, 2, GH, wr, 128), u32),
            pltpu.VMEM((D // 32, H * DH // 8, 128), u32),
            pltpu.VMEM((H * DH // 16, D // 16, 128), u32),
            pltpu.VMEM((D, FF), bf16),
            pltpu.VMEM((D, FF), bf16),
            pltpu.VMEM((FF // FCH, FCH, D), bf16),
            pltpu.VMEM((8, D), u32),
            pltpu.VMEM((12, 8, 128), u32),
            pltpu.VMEM((3, 8, 128), u32),
            pltpu.VMEM((2, 8, 8, 128), f32),
            pltpu.VMEM((2, 3, 8, 128), f32),
            pltpu.VMEM((2, NG, 16, 128), f32),
            pltpu.VMEM((8, D), f32),
            pltpu.VMEM((8, 128), u32),
            pltpu.VMEM((8, 128), f32),
            pltpu.VMEM((12, 8, 128), jnp.int32),
            pltpu.SemaphoreType.DMA((NP,)),
            pltpu.SemaphoreType.DMA((2 * NP - 2,)),
            pltpu.SemaphoreType.DMA((8,)),
        ],
        compiler_params=pltpu.CompilerParams(
            vmem_limit_bytes=128 * 1024 * 1024,
            disable_semaphore_checks=True),
    )(A_x, kt, vt, _tiles(A_wq, (D // 32,)), _tiles(A_wo, (H * DH // 16,)),
      B_w1, B_w3, B_w2.reshape(FF // FCH, FCH, D))
```

```python
import jax
import jax.numpy as jnp
import numpy as np
from jax import lax
import jax.experimental.pallas as pl
import jax.experimental.pallas.tpu as pltpu

D = 640
H = 32
NP = H // 2
DH = 192
GH = DH // 8
NG = 2 * GH
FF = 1536
FCH = 256
EPS = 1e-5

NW = 3
W2_SPLITS = ((0, 5), (5, 6))

T_START = 20
T_GROUP = 24.0
T_WIDE = 0.69
T_RESULT = 175
T_RESULT1 = 190
T_SUM = (40, 200)

f32 = jnp.float32
bf16 = jnp.bfloat16
u32 = jnp.uint32


def _round_bf16(x):
    return x.astype(bf16).astype(f32)


def _as_bf16(x):
    return pltpu.bitcast(x, bf16)


def _as_f32(x):
    return pltpu.bitcast(x, f32)


def _dot(a, b):
    return jnp.dot(a, b, preferred_element_type=f32)


def _gather_rows(x, idx):
    dnums = lax.GatherDimensionNumbers(
        offset_dims=(), collapsed_slice_dims=(0,), start_index_map=(0,),
        operand_batching_dims=(1,), start_indices_batching_dims=(1,))
    return lax.gather(x, idx.reshape(8, 128, 1), dnums, slice_sizes=(1, 1),
                      mode=lax.GatherScatterMode.FILL_OR_DROP)


def _ln_stats(x):
    m = jnp.mean(x, axis=-1, keepdims=True)
    c = x - m
    v = jnp.mean(c * c, axis=-1, keepdims=True)
    return m, c, lax.rsqrt(v + EPS)


def _with_ones(x):
    return jnp.concatenate([x, jnp.ones_like(x)], axis=0).astype(bf16)


def _centered_dot(xo, w, m):
    y = _dot(xo, w)
    return y[0:8] - m * y[8:16]


def _packed(t):
    return _as_f32(jnp.concatenate([t, t], axis=0).astype(bf16))


def _run(*gens):
    for g in gens:
        for _ in g:
            pass


def _take(gen, n):
    for _ in range(n):
        yield next(gen)


def _group_order():
    order = []
    step = GH // NW
    for par in range(2):
        packed = list(range(GH * par, GH * par + GH - NW))
        wide = list(range(GH * par + GH - NW, GH * par + GH))
        order += [(wide if n % step == step // 2 else packed).pop(0)
                  for n in range(GH)]
    return order


def _make_kernel(sk, win):
    nc = win // 128
    ncp = nc // 2
    row0 = (sk - win) // 128 * 4
    assert nc == 32
    scale = float(np.asarray(DH ** -0.5, dtype=bf16))
    order = _group_order()

    def kernel(x_hbm, k_hbm, v_hbm, wq_hbm, wo_hbm, w1_hbm, w3_hbm, w2_hbm,
               o_ref,
               xbuf, kbuf, vbuf, vwide, vlast, wq, wo, w1, w3, w2,
               zq, ybuf, qbuf, pbuf, lbuf, abuf, obuf, zeros, ones, tab,
               ksem, vsem, wsem):
        k32 = k_hbm.bitcast(u32)
        v32 = v_hbm.bitcast(u32)
        window = pl.ds(row0, 4 * nc)

        def k_copy(i):
            return pltpu.make_async_copy(
                k32.at[i, :, :, window, :], kbuf.at[i], ksem.at[i])

        def v_copies(i):
            return (
                pltpu.make_async_copy(
                    v32.at[i, :, pl.ds(0, GH - NW), window, :], vbuf.at[i],
                    vsem.at[2 * i]),
                pltpu.make_async_copy(
                    v32.at[i, :, pl.ds(GH - NW, NW), window, :],
                    vwide.at[i, 1], vsem.at[2 * i + 1]))

        x_copy = pltpu.make_async_copy(x_hbm, xbuf, wsem.at[0])
        wq_copy = pltpu.make_async_copy(wq_hbm.bitcast(u32), wq, wsem.at[1])
        wo_copy = pltpu.make_async_copy(wo_hbm.bitcast(u32), wo, wsem.at[2])
        vlast_copy = pltpu.make_async_copy(
            v32.at[NP - 1, :, :, window, :], vlast.at[1], wsem.at[3])
        w1_copy = pltpu.make_async_copy(w1_hbm, w1, wsem.at[4])
        w3_copy = pltpu.make_async_copy(w3_hbm, w3, wsem.at[5])
        w2_copies = [
            pltpu.make_async_copy(w2_hbm.at[pl.ds(a, b - a)],
                                  w2.at[pl.ds(a, b - a)], wsem.at[6 + n])
            for n, (a, b) in enumerate(W2_SPLITS)]

        wq_copy.start()
        x_copy.start()
        wo_copy.start()
        k_copy(0).start()

        def start_kv(i, carry):
            for cp in v_copies(i):
                cp.start()
            k_copy(i + 1).start()
            return carry

        lax.fori_loop(0, NP - 1, start_kv, 0)
        vlast_copy.start()

        lane = lax.broadcasted_iota(jnp.int32, (8, 128), 1)
        sub = lax.broadcasted_iota(jnp.int32, (8, 128), 0)
        zeros[...] = jnp.zeros((8, 128), u32)
        ones[...] = jnp.ones((8, 128), f32)
        lbuf[...] = jnp.ones(lbuf.shape, f32)
        for n in range(4):
            tab[n] = 2 * n + (sub >> 2)
        tab[4] = sub ^ 1
        tab[5] = jnp.zeros_like(sub)
        tab[6] = jnp.where(lane < 64, 0, 2)
        tab[7] = jnp.full_like(sub, 2)
        tab[8] = lane & 8
        tab[9] = sub
        tab[10] = sub - jnp.where(lane < 64, 0, 1)
        tab[11] = sub - 1

        def retile(ref, ntile, place):
            top = sub < 4
            nrep = ref.shape[1] // (8 * ntile)

            def body(a, carry):
                v = [ref[a, 8 * n:8 * n + 8, :] for n in range(nrep * ntile)]
                for k in range(nrep):
                    for t in range(ntile):
                        lo = v[k * ntile + t // 2]
                        hi = v[k * ntile + (ntile + t) // 2]
                        if t % 2:
                            lo = pltpu.roll(lo, 4, 0)
                        if (ntile + t) % 2 == 0:
                            hi = pltpu.roll(hi, 4, 0)
                        r = 8 * place(k, t)
                        ref[a, r:r + 8, :] = jnp.where(top, lo, hi)
                return carry

            lax.fori_loop(0, ref.shape[0], body, 0)

        def k_rows(g, c):
            r = 8 * (c ^ (g // 2 % 4))
            return slice(r, r + 8)

        def k_ready(i):
            k_copy(i).wait()

            def body(a, carry):
                for g in range(2, 8):
                    ref = kbuf.at[i, a // 3, 8 * (a % 3) + g]
                    v = [ref[8 * c:8 * c + 8, :] for c in range(ncp)]
                    for c in range(ncp):
                        ref[k_rows(g, c), :] = v[c]
                return carry

            lax.fori_loop(0, NG // 8, body, 0)

        wq_copy.wait()
        retile(wq, H * DH // 128, lambda k, t: 2 * t + k)
        w1_copy.start()
        w3_copy.start()
        wo_copy.wait()
        retile(wo, D // 128, lambda k, t: t)
        for cp in w2_copies:
            cp.start()

        def expand_q(t, b):
            even = tab[8] == 0
            return [jnp.where(tab[9 + t] == 2 * var, y, jnp.uint32(0))
                    for y in (jnp.where(even, b >> 16, pltpu.roll(b, 8, 1)),
                              jnp.where(even, pltpu.roll(b, 120, 1) >> 16, b))
                    for var in range(2)]

        def q_stage(u, e, out, proj=None, expand=True):
            r0 = 96 * u
            if not isinstance(r0, int):
                r0 = pl.multiple_of(r0, 32)
            wref = wq.at[:, pl.ds(r0, 96), :]
            for t in range(3):
                r = 48 * e + 16 * t
                w = _as_bf16(wref[:, r:r + 16, :].reshape(D // 2, 128))
                q = proj(w) if proj else _dot(_as_bf16(zq[...]), w)[0:8]
                b = pltpu.bitcast(_round_bf16(q), u32)
                out.extend(expand_q(t, b) if expand else [b])
                yield 40, [(_as_f32(b), 7)]

        def fold_rows(x, op):
            x = op(x, pltpu.roll(x, 4, 0))
            return op(x, _gather_rows(x, tab[4]))

        def scores(kref, ys, c, tiles):
            lhs = jnp.concatenate(
                [ys(4 * t + 2 * e + c % 2) for t in tiles for e in range(2)],
                axis=1)
            w = jnp.concatenate(
                [kref[g // GH, g % GH, k_rows(g, c), :]
                 for t in tiles for e in range(2)
                 for g in range(16 * t + e, 16 * t + 16, 2)], axis=0)
            return _dot(_as_bf16(lhs), _as_bf16(w))[0:8]

        def k_stage(i, ys, out):
            kref = kbuf.at[i]
            m = None
            for c in range(ncp):
                s = scores(kref, ys, c, (0, 1, 2))
                if c % 2 == 0:
                    out.append(s)
                    yield 48, [(s, 6)]
                else:
                    out[-1] = out[-1] + s
                    m = out[-1] if m is None else jnp.maximum(m, out[-1])
                    if c == ncp - 1:
                        m = fold_rows(m, jnp.maximum)
                    yield 48, [(m, 12 if c == ncp - 1 else 8)]
            out.append(m)

        def k_first(ys):
            plan = [(c, (t,)) for t in range(3) for c in range(4)]
            plan += [(c, (0, 1, 2)) for c in range(4, ncp)]
            acc = [None] * (ncp // 2)
            for c, tiles in plan:
                s = scores(kbuf.at[0], ys, c, tiles)
                acc[c // 2] = s if acc[c // 2] is None else acc[c // 2] + s
            m = acc[0]
            for a in acc[1:]:
                m = jnp.maximum(m, a)
            return acc + [fold_rows(m, jnp.maximum)]

        def softmax_numerator(ss, sc=scale):
            m = jnp.max(ss[-1], axis=1, keepdims=True)
            return [jnp.exp((s - m) * sc) for s in ss[:-1]]

        def inverse_sum(ps):
            tot = ps[0]
            for p in ps[1:]:
                tot = tot + p
            lf = fold_rows(tot, jnp.add)
            l = jnp.sum(lf, axis=1, keepdims=True)
            return lf, jnp.broadcast_to(1.0 / l, (8, 128))

        def lane_sums(b, j):
            a = jnp.concatenate(
                [abuf[b, 16 * j:16 * j + 16, 8 * s:8 * s + 8, :].reshape(128, 128)
                 for s in range(2)], axis=1)
            return lax.dot_general(
                jnp.concatenate([ones[...]] * 2, axis=1), a,
                (((1,), (1,)), ((), ())), preferred_element_type=f32)

        def r_stage(b, out):
            for j in range(3):
                out.append(_packed(lane_sums(b, j) * lbuf[b, j]))
                yield 32, [(out[-1], 4)]

        def o_stage(i, ts):
            wref = wo.at[pl.ds(24 * i, 24)]
            t = _as_bf16(jnp.concatenate(ts, axis=1))
            for n in range(D // 128):
                cols = slice(128 * n, 128 * n + 128)
                w = wref[:, 8 * n:8 * n + 8, :].reshape(DH, 128)
                y = obuf[:, cols] + _dot(t, _as_bf16(w))[0:8]
                obuf[:, cols] = y
                yield 24, [(y, 4)]

        def o_tile(i, j, t):
            r0 = 24 * i + 8 * j
            w = jnp.concatenate(
                [wo[r0:r0 + 8, 8 * n:8 * n + 8, :].reshape(64, 128)
                 for n in range(D // 128)], axis=1)
            return _dot(_as_bf16(t), _as_bf16(w))[0:8]

        def trace_mxu(gens, links, latency, t=0.0):
            for gen in gens:
                for cost, res in gen:
                    t += cost
                    links.setdefault(t + latency, []).extend(res)
            return t

        def v_stage(first, i, b, getp, links, clock, hist, t_sum=None):
            never = zeros[...] != 0
            last = i is None
            for n, g in enumerate(range(NG) if last else order):
                par, gl = divmod(g, GH)
                if n % GH == 0:
                    ps = [getp(par, j) for j in range(nc // 4)]
                    idx = [tab[par], tab[2 + par]]
                    if b == 1 and not last:
                        dep = pltpu.bitcast(hist[-2][0], jnp.int32)
                        idx = [jnp.where(never, dep, ix) for ix in idx]
                    pv = [_gather_rows(ps[c // 2], idx[c % 2])
                          for c in range(ncp)]
                    clock[0] += 4
                    if par == 1 and not last:
                        lf, inv = inverse_sum(ps)
                        for val, at in zip((lf, inv), t_sum or ()):
                            links.setdefault(clock[0] + at, []).append((val, 14))
                        for j in range(3):
                            lbuf[b, j] = _gather_rows(inv, tab[5 + j])
                wide = last or gl >= GH - NW
                if last:
                    ref = vlast.at[:, par, gl]
                elif wide:
                    ref = vwide.at[i, :, par, gl - (GH - NW)]
                else:
                    ref = vbuf.at[i, par, gl]
                fast = wide and not first
                dur = T_GROUP * (T_WIDE if fast else 1.0)
                accs = [None, None]
                held = [None, None]
                pending = []
                for c in range(ncp):
                    for key in sorted(links):
                        if key < clock[0] + dur * (c + 1) / 16:
                            for val, ops in links.pop(key):
                                pending.append(val)
                                clock[0] += ops / 4
                    rs = slice(8 * c, 8 * c + 8)
                    if fast:
                        lo, hi = ref[0, rs, :], ref[1, rs, :]
                    else:
                        w = ref[1, rs, :] if wide else ref[rs, :]
                        lo = w << 16
                        hi = w & jnp.uint32(0xFFFF0000)
                        if wide:
                            ref[0, rs, :] = lo
                            ref[1, rs, :] = hi
                    p = pv[c]
                    if c == (6 if fast else 0) and hist and not last:
                        p = jnp.where(never, hist[-1][0] + hist[-1][1], p)
                    for a, t in enumerate((_as_f32(lo) * p, _as_f32(hi) * p)):
                        if accs[a] is None:
                            accs[a] = t
                            continue
                        if pending:
                            t = jnp.where(never, pending.pop(), t)
                        if c % 2 == 1 and c < ncp - 1:
                            held[a] = t
                        else:
                            if held[a] is not None:
                                t = held[a] + t
                                held[a] = None
                            accs[a] = accs[a] + t
                for a in range(2):
                    abuf[b, g, pl.ds(a, 8, stride=2), :] = accs[a]
                clock[0] += dur
                hist.append(accs)
                yield g

        def from_pbuf(par, j):
            return pbuf[par, j]

        def store_p(ps):
            for j, p in enumerate(ps):
                pbuf[0, j] = p
                pbuf[1, j] = p

        def two_pairs(first, it):
            i = 2 * it
            links, clock, hist = {}, [T_START], []
            s1, s2, ya, qb, t0, t1 = [], [], [], [], [], []
            y2 = [y for t in range(3) for y in expand_q(t, qbuf[t])]
            k2 = k_stage(i + 2, lambda n: y2[n], s2)
            t = trace_mxu([k_stage(i + 1, lambda n: ybuf[n], s1)],
                          links, T_RESULT)
            p1 = softmax_numerator(s1)
            t = trace_mxu([r_stage(1, t1), q_stage(it + 1, 1, ya),
                           o_stage(jnp.maximum(i - 1, 0), t1), _take(k2, 4)],
                          links, T_RESULT, t)
            _run(v_stage(first, i, 0, from_pbuf, links, clock, hist, T_SUM))
            t = trace_mxu([r_stage(0, t0), k2], links, T_RESULT,
                          max(t, clock[0] - 64))
            p2 = softmax_numerator(s2)
            trace_mxu([o_stage(i, t0),
                       q_stage(jnp.minimum(it + 2, NP // 2 - 1), 0, qb,
                               expand=False)], links, T_RESULT, t)
            _run(v_stage(first, i + 1, 1, lambda par, j: p1[j], links, clock,
                         hist, T_SUM))
            for n in range(12):
                ybuf[n] = ya[n]
            for n in range(3):
                qbuf[n] = qb[n]
            store_p(p2)

        def one_pair(first):
            i = NP - 2
            links = {}
            s1, t1 = [], []
            trace_mxu([r_stage(1, t1), k_stage(i + 1, lambda n: ybuf[n], s1),
                       o_stage(i - 1, t1)], links, T_RESULT1)
            _run(v_stage(first, i, 0, from_pbuf, links, [T_START], []))
            store_p(softmax_numerator(s1))

        def last_pair(first):
            ts = [_packed(lane_sums(0, j) * lbuf[0, j]) for j in range(3)]
            lf, inv = inverse_sum([pbuf[1, j] for j in range(nc // 4)])
            tn = []
            for g in v_stage(first, None, 1, from_pbuf, {50: [(lf, 0)]},
                             [0.0], []):
                if g % 16 == 15:
                    j = g // 16
                    tn.append(_packed(
                        lane_sums(1, j) * _gather_rows(inv, tab[5 + j])))
            y = obuf[...]
            for j in range(3):
                y = y + o_tile(NP - 2, j, ts[j])
            for j in range(3):
                y = y + o_tile(NP - 1, j, tn[j])
            return y

        def attention(first, x):
            if first:
                k_ready(0)
            m, c, r = _ln_stats(x)
            z = c * r
            xo = _with_ones(x)
            zq[...] = pltpu.bitcast(
                jnp.concatenate([z, z], axis=0).astype(bf16), u32)
            obuf[...] = jnp.zeros(obuf.shape, f32)
            abuf[1] = jnp.zeros(abuf.shape[1:], f32)

            y0, y1, q2 = [], [], []
            _run(q_stage(0, 0, y0, lambda w: _centered_dot(xo, w, m)),
                 q_stage(0, 1, y1, lambda w: _centered_dot(xo, w, m) * r))
            ss = k_first(lambda n: y0[n])
            _run(q_stage(1, 0, q2, expand=False))
            for n in range(12):
                ybuf[n] = y1[n]
            for n in range(3):
                qbuf[n] = q2[n]
            store_p(softmax_numerator(ss, r * scale))

            def body(it, count):
                if first:
                    for i in (2 * it, 2 * it + 1):
                        for cp in v_copies(i):
                            cp.wait()
                        k_ready(i + 1)
                two_pairs(first, it)
                return count + 1

            count = lax.fori_loop(0, NP // 2 - 1, body, 0)

            @pl.when(count > 0)
            def _():
                if first:
                    for cp in v_copies(NP - 2):
                        cp.wait()
                    k_ready(NP - 1)
                one_pair(first)

            if first:
                vlast_copy.wait()
            return last_pair(first)

        def ffn(first, x):
            if first:
                w1_copy.wait()
                w3_copy.wait()
            m, _, r = _ln_stats(x)
            xo = _with_ones(x)
            hids = []
            for n in range(0, FF, FCH):
                gate = _round_bf16(_centered_dot(xo, w1[:, n:n + FCH], m) * r)
                up = _round_bf16(_centered_dot(xo, w3[:, n:n + FCH], m) * r)
                hids.append(
                    (_round_bf16(gate * jax.nn.sigmoid(gate)) * up).astype(bf16))
            y = None
            starts = [a for a, _ in W2_SPLITS]
            for n, hid in enumerate(hids):
                if first and n in starts:
                    if y is not None:
                        obuf[...] = y
                    w2_copies[starts.index(n)].wait()
                    if y is not None:
                        y = obuf[...]
                t = _dot(hid, w2[n])
                y = t if y is None else y + t
            return y

        x_copy.wait()
        x = jnp.broadcast_to(xbuf[0].astype(f32), (8, D))
        for first in (True, False):
            x = _round_bf16(x + _round_bf16(attention(first, x)))
            x = _round_bf16(x + _round_bf16(ffn(first, x)))
        o_ref[0] = x[0:1].astype(bf16)

    return kernel


def _tiles(a, lead):
    r, c = a.shape
    t = a.reshape(r // 8, 8, c // 128, 128).transpose(0, 2, 1, 3)
    return t.reshape(lead + (-1, 128))


@jax.jit
def pallas_interleave_layers__sliding_block_cached__glu_gated_swiglu__decode_kernel(
    A_x: jax.Array,
    A_k_cache: jax.Array,
    A_v_cache: jax.Array,
    A_wq: jax.Array,
    A_wo: jax.Array,
    B_x: jax.Array,
    B_w1: jax.Array,
    B_w3: jax.Array,
    B_w2: jax.Array,
):
    del B_x
    sk = A_k_cache.shape[2]
    win = min(4096, max(256, sk // 4))
    wr = win // 32
    kt = _tiles(jnp.swapaxes(A_k_cache, 2, 3).reshape(H * DH, sk), (NP, 2, GH))
    vt = _tiles(jnp.swapaxes(A_v_cache, 2, 3).reshape(H * DH, sk), (NP, 2, GH))
    any_spec = pl.BlockSpec(memory_space=pl.ANY)
    return pl.pallas_call(
        _make_kernel(sk, win),
        out_shape=jax.ShapeDtypeStruct((1, 1, D), bf16),
        in_specs=[any_spec] * 8,
        out_specs=pl.BlockSpec(memory_space=pltpu.VMEM),
        scratch_shapes=[
            pltpu.VMEM((1, 1, D), bf16),
            pltpu.VMEM((NP, 2, GH, wr, 128), u32),
            pltpu.VMEM((NP - 1, 2, GH - NW, wr, 128), u32),
            pltpu.VMEM((NP - 1, 2, 2, NW, wr, 128), u32),
            pltpu.VMEM((2, 2, GH, wr, 128), u32),
            pltpu.VMEM((D // 32, H * DH // 8, 128), u32),
            pltpu.VMEM((H * DH // 16, D // 16, 128), u32),
            pltpu.VMEM((D, FF), bf16),
            pltpu.VMEM((D, FF), bf16),
            pltpu.VMEM((FF // FCH, FCH, D), bf16),
            pltpu.VMEM((8, D), u32),
            pltpu.VMEM((12, 8, 128), u32),
            pltpu.VMEM((3, 8, 128), u32),
            pltpu.VMEM((2, 8, 8, 128), f32),
            pltpu.VMEM((2, 3, 8, 128), f32),
            pltpu.VMEM((2, NG, 16, 128), f32),
            pltpu.VMEM((8, D), f32),
            pltpu.VMEM((8, 128), u32),
            pltpu.VMEM((8, 128), f32),
            pltpu.VMEM((12, 8, 128), jnp.int32),
            pltpu.SemaphoreType.DMA((NP,)),
            pltpu.SemaphoreType.DMA((2 * NP - 2,)),
            pltpu.SemaphoreType.DMA((8,)),
        ],
        compiler_params=pltpu.CompilerParams(
            vmem_limit_bytes=128 * 1024 * 1024,
            disable_semaphore_checks=True),
    )(A_x, kt, vt, _tiles(A_wq, (D // 32,)), _tiles(A_wo, (H * DH // 16,)),
      B_w1, B_w3, B_w2.reshape(FF // FCH, FCH, D))
```

```python
import jax
import jax.numpy as jnp
import numpy as np
from jax import lax
import jax.experimental.pallas as pl
import jax.experimental.pallas.tpu as pltpu

D = 640
H = 32
NP = H // 2
DH = 192
GH = DH // 8
NG = 2 * GH
FF = 1536
FCH = 256
EPS = 1e-5

NW = 3
W2_SPLITS = ((0, 5), (5, 6))

T_START = 20
T_GROUP = 24.0
T_WIDE = 0.69
T_RESULT = 175
T_RESULT1 = 190
T_FIRST = 740
T_SUM = (40, 200)

f32 = jnp.float32
bf16 = jnp.bfloat16
u32 = jnp.uint32


def _round_bf16(x):
    return x.astype(bf16).astype(f32)


def _as_bf16(x):
    return pltpu.bitcast(x, bf16)


def _as_f32(x):
    return pltpu.bitcast(x, f32)


def _dot(a, b):
    return jnp.dot(a, b, preferred_element_type=f32)


def _gather_rows(x, idx):
    dnums = lax.GatherDimensionNumbers(
        offset_dims=(), collapsed_slice_dims=(0,), start_index_map=(0,),
        operand_batching_dims=(1,), start_indices_batching_dims=(1,))
    return lax.gather(x, idx.reshape(8, 128, 1), dnums, slice_sizes=(1, 1),
                      mode=lax.GatherScatterMode.FILL_OR_DROP)


def _ln_stats(x):
    m = jnp.mean(x, axis=-1, keepdims=True)
    c = x - m
    v = jnp.mean(c * c, axis=-1, keepdims=True)
    return m, c, lax.rsqrt(v + EPS)


def _with_ones(x):
    return jnp.concatenate([x, jnp.ones_like(x)], axis=0).astype(bf16)


def _centered_dot(xo, w, m):
    y = _dot(xo, w)
    return y[0:8] - m * y[8:16]


def _packed(t):
    return _as_f32(jnp.concatenate([t, t], axis=0).astype(bf16))


def _run(*gens):
    for g in gens:
        for _ in g:
            pass


def _take(gen, n):
    for _ in range(n):
        yield next(gen)


def _group_order():
    order = []
    step = GH // NW
    for par in range(2):
        packed = list(range(GH * par, GH * par + GH - NW))
        wide = list(range(GH * par + GH - NW, GH * par + GH))
        order += [(wide if n % step == step // 2 else packed).pop(0)
                  for n in range(GH)]
    return order


def _make_kernel(sk, win):
    nc = win // 128
    ncp = nc // 2
    row0 = (sk - win) // 128 * 4
    assert nc == 32
    scale = float(np.asarray(DH ** -0.5, dtype=bf16))
    order = _group_order()

    def kernel(x_hbm, k_hbm, v_hbm, wq_hbm, wo_hbm, w1_hbm, w3_hbm, w2_hbm,
               o_ref,
               xbuf, kbuf, vbuf, vwide, vlast, wq, wo, w1, w3, w2,
               zq, ybuf, qbuf, pbuf, lbuf, abuf, obuf, zeros, ones, tab,
               ksem, vsem, wsem):
        k32 = k_hbm.bitcast(u32)
        v32 = v_hbm.bitcast(u32)
        window = pl.ds(row0, 4 * nc)

        def k_copy(i):
            return pltpu.make_async_copy(
                k32.at[i, :, :, window, :], kbuf.at[i], ksem.at[i])

        def v_copies(i):
            return (
                pltpu.make_async_copy(
                    v32.at[i, :, pl.ds(0, GH - NW), window, :], vbuf.at[i],
                    vsem.at[2 * i]),
                pltpu.make_async_copy(
                    v32.at[i, :, pl.ds(GH - NW, NW), window, :],
                    vwide.at[i, 1], vsem.at[2 * i + 1]))

        x_copy = pltpu.make_async_copy(x_hbm, xbuf, wsem.at[0])
        wq_copy = pltpu.make_async_copy(wq_hbm.bitcast(u32), wq, wsem.at[1])
        wo_copy = pltpu.make_async_copy(wo_hbm.bitcast(u32), wo, wsem.at[2])
        vlast_copy = pltpu.make_async_copy(
            v32.at[NP - 1, :, :, window, :], vlast.at[1], wsem.at[3])
        w1_copy = pltpu.make_async_copy(w1_hbm, w1, wsem.at[4])
        w3_copy = pltpu.make_async_copy(w3_hbm, w3, wsem.at[5])
        w2_copies = [
            pltpu.make_async_copy(w2_hbm.at[pl.ds(a, b - a)],
                                  w2.at[pl.ds(a, b - a)], wsem.at[6 + n])
            for n, (a, b) in enumerate(W2_SPLITS)]

        wq_copy.start()
        x_copy.start()
        wo_copy.start()
        k_copy(0).start()

        def start_kv(i, carry):
            for cp in v_copies(i):
                cp.start()
            k_copy(i + 1).start()
            return carry

        lax.fori_loop(0, NP - 1, start_kv, 0)
        vlast_copy.start()

        lane = lax.broadcasted_iota(jnp.int32, (8, 128), 1)
        sub = lax.broadcasted_iota(jnp.int32, (8, 128), 0)
        zeros[...] = jnp.zeros((8, 128), u32)
        ones[...] = jnp.ones((8, 128), f32)
        for n in range(4):
            tab[n] = 2 * n + (sub >> 2)
        tab[4] = sub ^ 1
        tab[5] = jnp.zeros_like(sub)
        tab[6] = jnp.where(lane < 64, 0, 2)
        tab[7] = jnp.full_like(sub, 2)
        tab[8] = lane & 8
        tab[9] = sub
        tab[10] = sub - jnp.where(lane < 64, 0, 1)
        tab[11] = sub - 1

        def retile(ref, ntile, place):
            top = sub < 4
            nrep = ref.shape[1] // (8 * ntile)

            def body(a, carry):
                v = [ref[a, 8 * n:8 * n + 8, :] for n in range(nrep * ntile)]
                for k in range(nrep):
                    for t in range(ntile):
                        lo = v[k * ntile + t // 2]
                        hi = v[k * ntile + (ntile + t) // 2]
                        if t % 2:
                            lo = pltpu.roll(lo, 4, 0)
                        if (ntile + t) % 2 == 0:
                            hi = pltpu.roll(hi, 4, 0)
                        r = 8 * place(k, t)
                        ref[a, r:r + 8, :] = jnp.where(top, lo, hi)
                return carry

            lax.fori_loop(0, ref.shape[0], body, 0)

        def k_rows(g, c):
            r = 8 * (c ^ (g // 2 % 4))
            return slice(r, r + 8)

        def k_ready(i):
            k_copy(i).wait()

            def body(a, carry):
                for g in range(2, 8):
                    ref = kbuf.at[i, a // 3, 8 * (a % 3) + g]
                    v = [ref[8 * c:8 * c + 8, :] for c in range(ncp)]
                    for c in range(ncp):
                        ref[k_rows(g, c), :] = v[c]
                return carry

            lax.fori_loop(0, NG // 8, body, 0)

        wq_copy.wait()
        retile(wq, H * DH // 128, lambda k, t: 2 * t + k)
        w1_copy.start()
        w3_copy.start()
        wo_copy.wait()
        retile(wo, D // 128, lambda k, t: t)
        for cp in w2_copies:
            cp.start()

        def expand_q(t, b):
            even = tab[8] == 0
            return [jnp.where(tab[9 + t] == 2 * var, y, jnp.uint32(0))
                    for y in (jnp.where(even, b >> 16, pltpu.roll(b, 8, 1)),
                              jnp.where(even, pltpu.roll(b, 120, 1) >> 16, b))
                    for var in range(2)]

        def q_stage(u, e, out, proj=None, expand=True):
            r0 = 96 * u
            if not isinstance(r0, int):
                r0 = pl.multiple_of(r0, 32)
            wref = wq.at[:, pl.ds(r0, 96), :]
            for t in range(3):
                r = 48 * e + 16 * t
                w = _as_bf16(wref[:, r:r + 16, :].reshape(D // 2, 128))
                q = proj(w) if proj else _dot(_as_bf16(zq[...]), w)[0:8]
                b = pltpu.bitcast(_round_bf16(q), u32)
                out.extend(expand_q(t, b) if expand else [b])
                yield 40, [(_as_f32(b), 7)]

        def fold_rows(x, op):
            x = op(x, pltpu.roll(x, 4, 0))
            return op(x, _gather_rows(x, tab[4]))

        def k_stage(i, ys, out):
            kref = kbuf.at[i]
            m = None
            for c in range(ncp):
                lhs = jnp.concatenate(
                    [ys(2 * n + c % 2) for n in range(6)], axis=1)
                w = jnp.concatenate(
                    [kref[g // GH, g % GH, k_rows(g, c), :]
                     for t in range(3) for e in range(2)
                     for g in range(16 * t + e, 16 * t + 16, 2)], axis=0)
                s = _dot(_as_bf16(lhs), _as_bf16(w))[0:8]
                if c % 2 == 0:
                    out.append(s)
                    yield 48, [(s, 6)]
                else:
                    out[-1] = out[-1] + s
                    m = out[-1] if m is None else jnp.maximum(m, out[-1])
                    if c == ncp - 1:
                        m = fold_rows(m, jnp.maximum)
                    yield 48, [(m, 12 if c == ncp - 1 else 8)]
            out.append(m)

        def k_first(qb, out_a, out):
            even, low = tab[8] == 0, tab[6] == 0
            b = qb[1]
            rot = {n: pltpu.roll(b, n, 1) for n in (8, 56, 64, 72, 120)}
            mix = (jnp.where(even, jnp.where(low, b, rot[56]) >> 16,
                             jnp.where(low, rot[8], rot[64])),
                   jnp.where(even, jnp.where(low, rot[64], rot[120]) >> 16,
                             jnp.where(low, rot[72], b)))
            tiles = []
            for par in range(2):
                ys = expand_q(2 * par, qb[2 * par])
                for e in range(2):
                    tiles.append((ys[2 * e:2 * e + 2],
                                  range(32 * par + e, 32 * par + 16, 2)))
                g0 = 16 + 8 * par
                tiles.append((
                    [jnp.where(tab[9 + 2 * par] == 2 * var, mix[par],
                               jnp.uint32(0)) for var in range(2)],
                    [*range(g0, g0 + 8, 2), *range(g0 + 1, g0 + 8, 2)]))

            def part(c, sel):
                lhs = jnp.concatenate([tiles[n][0][c % 2] for n in sel], axis=1)
                w = jnp.concatenate(
                    [kbuf[0, g // GH, g % GH, k_rows(g, c), :]
                     for n in sel for g in tiles[n][1]], axis=0)
                return _dot(_as_bf16(lhs), _as_bf16(w))[0:8]

            plan = [(c, (0, 1)) for c in range(4)] + [(c, (2,)) for c in range(4)]
            plan += [(c, (0, 1, 2)) for c in range(4, ncp)]
            acc = [None] * (ncp // 2)
            for c, sel in plan:
                s = part(c, sel)
                acc[c // 2] = s if acc[c // 2] is None else acc[c // 2] + s
                yield 8 * len(sel), []
            m = acc[0]
            for a in acc[1:]:
                m = jnp.maximum(m, a)
            out_a.extend(acc + [fold_rows(m, jnp.maximum)])
            m = None
            for j in range(ncp // 2):
                s = acc[j] + part(2 * j, (3, 4, 5)) + part(2 * j + 1, (3, 4, 5))
                out.append(s)
                m = s if m is None else jnp.maximum(m, s)
                if j == ncp // 2 - 1:
                    m = fold_rows(m, jnp.maximum)
                yield 48, [(m, 8)]
            out.append(m)

        def softmax_numerator(ss, sc=scale):
            m = jnp.max(ss[-1], axis=1, keepdims=True)
            return [jnp.exp((s - m) * sc) for s in ss[:-1]]

        def inverse_sum(ps):
            tot = ps[0]
            for p in ps[1:]:
                tot = tot + p
            lf = fold_rows(tot, jnp.add)
            l = jnp.sum(lf, axis=1, keepdims=True)
            return lf, jnp.broadcast_to(1.0 / l, (8, 128))

        def lane_sums(b, j):
            a = jnp.concatenate(
                [abuf[b, 16 * j:16 * j + 16, 8 * s:8 * s + 8, :].reshape(128, 128)
                 for s in range(2)], axis=1)
            return lax.dot_general(
                jnp.concatenate([ones[...]] * 2, axis=1), a,
                (((1,), (1,)), ((), ())), preferred_element_type=f32)

        def r_stage(b, out):
            for j in range(3):
                out.append(_packed(lane_sums(b, j) * lbuf[b, j]))
                yield 32, [(out[-1], 4)]

        def o_stage(i, ts):
            wref = wo.at[pl.ds(24 * i, 24)]
            t = _as_bf16(jnp.concatenate(ts, axis=1))
            for n in range(D // 128):
                cols = slice(128 * n, 128 * n + 128)
                w = wref[:, 8 * n:8 * n + 8, :].reshape(DH, 128)
                y = obuf[:, cols] + _dot(t, _as_bf16(w))[0:8]
                obuf[:, cols] = y
                yield 24, [(y, 4)]

        def o_tile(i, j, t):
            r0 = 24 * i + 8 * j
            w = jnp.concatenate(
                [wo[r0:r0 + 8, 8 * n:8 * n + 8, :].reshape(64, 128)
                 for n in range(D // 128)], axis=1)
            return _dot(_as_bf16(t), _as_bf16(w))[0:8]

        def trace_mxu(gens, links, latency, t=0.0):
            for gen in gens:
                for cost, res in gen:
                    t += cost
                    links.setdefault(t + latency, []).extend(res)
            return t

        def v_stage(first, i, b, getp, links, clock, hist, t_sum=None):
            never = zeros[...] != 0
            last = i is None
            for n, g in enumerate(range(NG) if last else order):
                par, gl = divmod(g, GH)
                if n % GH == 0:
                    ps = [getp(par, j) for j in range(nc // 4)]
                    idx = [tab[par], tab[2 + par]]
                    if len(hist) > 1 and getp is not from_pbuf:
                        dep = pltpu.bitcast(hist[-2][0], jnp.int32)
                        idx = [jnp.where(never, dep, ix) for ix in idx]
                    pv = [_gather_rows(ps[c // 2], idx[c % 2])
                          for c in range(ncp)]
                    clock[0] += 4
                    if par == 1 and not last:
                        lf, inv = inverse_sum(ps)
                        for val, at in zip((lf, inv), t_sum or ()):
                            links.setdefault(clock[0] + at, []).append((val, 14))
                        for j in range(3):
                            lbuf[b, j] = _gather_rows(inv, tab[5 + j])
                wide = last or gl >= GH - NW
                if last:
                    ref = vlast.at[:, par, gl]
                elif wide:
                    ref = vwide.at[i, :, par, gl - (GH - NW)]
                else:
                    ref = vbuf.at[i, par, gl]
                fast = wide and not first
                dur = T_GROUP * (T_WIDE if fast else 1.0)
                accs = [None, None]
                held = [None, None]
                pending = []
                for c in range(ncp):
                    for key in sorted(links):
                        if key < clock[0] + dur * (c + 1) / 16:
                            for val, ops in links.pop(key):
                                pending.append(val)
                                clock[0] += ops / 4
                    rs = slice(8 * c, 8 * c + 8)
                    if fast:
                        lo, hi = ref[0, rs, :], ref[1, rs, :]
                    else:
                        w = ref[1, rs, :] if wide else ref[rs, :]
                        lo = w << 16
                        hi = w & jnp.uint32(0xFFFF0000)
                        if wide:
                            ref[0, rs, :] = lo
                            ref[1, rs, :] = hi
                    p = pv[c]
                    if c == (6 if fast else 0) and hist and not last:
                        p = jnp.where(never, hist[-1][0] + hist[-1][1], p)
                    for a, t in enumerate((_as_f32(lo) * p, _as_f32(hi) * p)):
                        if accs[a] is None:
                            accs[a] = t
                            continue
                        if pending:
                            t = jnp.where(never, pending.pop(), t)
                        if c % 2 == 1 and c < ncp - 1:
                            held[a] = t
                        else:
                            if held[a] is not None:
                                t = held[a] + t
                                held[a] = None
                            accs[a] = accs[a] + t
                for a in range(2):
                    abuf[b, g, pl.ds(a, 8, stride=2), :] = accs[a]
                clock[0] += dur
                hist.append(accs)
                yield g

        def from_pbuf(par, j):
            return pbuf[par, j]

        def store_p(ps):
            for j, p in enumerate(ps):
                pbuf[0, j] = p
                pbuf[1, j] = p

        def two_pairs(first, it):
            i = 2 * it
            links, clock, hist = {}, [T_START], []
            s1, s2, ya, qb, t0, t1 = [], [], [], [], [], []
            y2 = [y for t in range(3) for y in expand_q(t, qbuf[t])]
            k2 = k_stage(i + 2, lambda n: y2[n], s2)
            t = trace_mxu([k_stage(i + 1, lambda n: ybuf[n], s1)],
                          links, T_RESULT)
            p1 = softmax_numerator(s1)
            t = trace_mxu([r_stage(1, t1), q_stage(it + 1, 1, ya),
                           o_stage(i - 1, t1), _take(k2, 4)],
                          links, T_RESULT, t)
            _run(v_stage(first, i, 0, from_pbuf, links, clock, hist, T_SUM))
            t = trace_mxu([r_stage(0, t0), k2], links, T_RESULT,
                          max(t, clock[0] - 64))
            p2 = softmax_numerator(s2)
            trace_mxu([o_stage(i, t0),
                       q_stage(jnp.minimum(it + 2, NP // 2 - 1), 0, qb,
                               expand=False)], links, T_RESULT, t)
            _run(v_stage(first, i + 1, 1, lambda par, j: p1[j], links, clock,
                         hist, T_SUM))
            for n in range(12):
                ybuf[n] = ya[n]
            for n in range(3):
                qbuf[n] = qb[n]
            store_p(p2)

        def first_pairs(first, xo, m, r):
            links, clock, hist = {}, [T_FIRST], []
            q0, y1, y2, sa, s0, s1, s2, ya, qb, t0 = ([] for _ in range(10))
            _run(q_stage(0, 0, q0, lambda w: _centered_dot(xo, w, m), False),
                 q_stage(0, 1, y1, lambda w: _centered_dot(xo, w, m) * r))
            t = trace_mxu([k_first(q0, sa, s0),
                           k_stage(1, lambda n: y1[n], s1),
                           q_stage(1, 0, y2), q_stage(1, 1, ya),
                           q_stage(2, 0, qb, expand=False)], links, T_RESULT1)
            for key in [key for key in links if key < T_FIRST + 30]:
                del links[key]
            pa = softmax_numerator(sa, r * scale)
            p0 = softmax_numerator(s0, r * scale)
            p1 = softmax_numerator(s1)
            _run(v_stage(first, 0, 0, lambda par, j: (pa, p0)[par][j], links,
                         clock, hist, T_SUM))
            trace_mxu([r_stage(0, t0), k_stage(2, lambda n: y2[n], s2),
                       o_stage(0, t0)], links, T_RESULT1,
                      max(t, clock[0] - 64))
            p2 = softmax_numerator(s2)
            _run(v_stage(first, 1, 1, lambda par, j: p1[j], links, clock,
                         hist, T_SUM))
            for n in range(12):
                ybuf[n] = ya[n]
            for n in range(3):
                qbuf[n] = qb[n]
            store_p(p2)

        def one_pair(first):
            i = NP - 2
            links = {}
            s1, t1 = [], []
            trace_mxu([r_stage(1, t1), k_stage(i + 1, lambda n: ybuf[n], s1),
                       o_stage(i - 1, t1)], links, T_RESULT1)
            _run(v_stage(first, i, 0, from_pbuf, links, [T_START], []))
            store_p(softmax_numerator(s1))

        def last_pair(first):
            ts = [_packed(lane_sums(0, j) * lbuf[0, j]) for j in range(3)]
            lf, inv = inverse_sum([pbuf[1, j] for j in range(nc // 4)])
            tn = []
            for g in v_stage(first, None, 1, from_pbuf, {50: [(lf, 0)]},
                             [0.0], []):
                if g % 16 == 15:
                    j = g // 16
                    tn.append(_packed(
                        lane_sums(1, j) * _gather_rows(inv, tab[5 + j])))
            y = obuf[...]
            for j in range(3):
                y = y + o_tile(NP - 2, j, ts[j])
            for j in range(3):
                y = y + o_tile(NP - 1, j, tn[j])
            return y

        def attention(first, x):
            if first:
                k_ready(0)
                for i in range(2):
                    for cp in v_copies(i):
                        cp.wait()
                    k_ready(i + 1)
            m, c, r = _ln_stats(x)
            z = c * r
            xo = _with_ones(x)
            zq[...] = pltpu.bitcast(
                jnp.concatenate([z, z], axis=0).astype(bf16), u32)
            obuf[...] = jnp.zeros(obuf.shape, f32)
            first_pairs(first, xo, m, r)

            def body(it, count):
                if first:
                    for i in (2 * it, 2 * it + 1):
                        for cp in v_copies(i):
                            cp.wait()
                        k_ready(i + 1)
                two_pairs(first, it)
                return count + 1

            count = lax.fori_loop(1, NP // 2 - 1, body, 0)

            @pl.when(count > 0)
            def _():
                if first:
                    for cp in v_copies(NP - 2):
                        cp.wait()
                    k_ready(NP - 1)
                one_pair(first)

            if first:
                vlast_copy.wait()
            return last_pair(first)

        def ffn(first, x):
            if first:
                w1_copy.wait()
                w3_copy.wait()
            m, _, r = _ln_stats(x)
            xo = _with_ones(x)
            hids = []
            for n in range(0, FF, FCH):
                gate = _round_bf16(_centered_dot(xo, w1[:, n:n + FCH], m) * r)
                up = _round_bf16(_centered_dot(xo, w3[:, n:n + FCH], m) * r)
                hids.append(
                    (_round_bf16(gate * jax.nn.sigmoid(gate)) * up).astype(bf16))
            y = None
            starts = [a for a, _ in W2_SPLITS]
            for n, hid in enumerate(hids):
                if first and n in starts:
                    if y is not None:
                        obuf[...] = y
                    w2_copies[starts.index(n)].wait()
                    if y is not None:
                        y = obuf[...]
                t = _dot(hid, w2[n])
                y = t if y is None else y + t
            return y

        x_copy.wait()
        x = jnp.broadcast_to(xbuf[0].astype(f32), (8, D))
        for first in (True, False):
            x = _round_bf16(x + _round_bf16(attention(first, x)))
            x = _round_bf16(x + _round_bf16(ffn(first, x)))
        o_ref[0] = x[0:1].astype(bf16)

    return kernel


def _tiles(a, lead):
    r, c = a.shape
    t = a.reshape(r // 8, 8, c // 128, 128).transpose(0, 2, 1, 3)
    return t.reshape(lead + (-1, 128))


@jax.jit
def pallas_interleave_layers__sliding_block_cached__glu_gated_swiglu__decode_kernel(
    A_x: jax.Array,
    A_k_cache: jax.Array,
    A_v_cache: jax.Array,
    A_wq: jax.Array,
    A_wo: jax.Array,
    B_x: jax.Array,
    B_w1: jax.Array,
    B_w3: jax.Array,
    B_w2: jax.Array,
):
    del B_x
    sk = A_k_cache.shape[2]
    win = min(4096, max(256, sk // 4))
    wr = win // 32
    kt = _tiles(jnp.swapaxes(A_k_cache, 2, 3).reshape(H * DH, sk), (NP, 2, GH))
    vt = _tiles(jnp.swapaxes(A_v_cache, 2, 3).reshape(H * DH, sk), (NP, 2, GH))
    any_spec = pl.BlockSpec(memory_space=pl.ANY)
    return pl.pallas_call(
        _make_kernel(sk, win),
        out_shape=jax.ShapeDtypeStruct((1, 1, D), bf16),
        in_specs=[any_spec] * 8,
        out_specs=pl.BlockSpec(memory_space=pltpu.VMEM),
        scratch_shapes=[
            pltpu.VMEM((1, 1, D), bf16),
            pltpu.VMEM((NP, 2, GH, wr, 128), u32),
            pltpu.VMEM((NP - 1, 2, GH - NW, wr, 128), u32),
            pltpu.VMEM((NP - 1, 2, 2, NW, wr, 128), u32),
            pltpu.VMEM((2, 2, GH, wr, 128), u32),
            pltpu.VMEM((D // 32, H * DH // 8, 128), u32),
            pltpu.VMEM((H * DH // 16, D // 16, 128), u32),
            pltpu.VMEM((D, FF), bf16),
            pltpu.VMEM((D, FF), bf16),
            pltpu.VMEM((FF // FCH, FCH, D), bf16),
            pltpu.VMEM((8, D), u32),
            pltpu.VMEM((12, 8, 128), u32),
            pltpu.VMEM((3, 8, 128), u32),
            pltpu.VMEM((2, 8, 8, 128), f32),
            pltpu.VMEM((2, 3, 8, 128), f32),
            pltpu.VMEM((2, NG, 16, 128), f32),
            pltpu.VMEM((8, D), f32),
            pltpu.VMEM((8, 128), u32),
            pltpu.VMEM((8, 128), f32),
            pltpu.VMEM((12, 8, 128), jnp.int32),
            pltpu.SemaphoreType.DMA((NP,)),
            pltpu.SemaphoreType.DMA((2 * NP - 2,)),
            pltpu.SemaphoreType.DMA((8,)),
        ],
        compiler_params=pltpu.CompilerParams(
            vmem_limit_bytes=128 * 1024 * 1024,
            disable_semaphore_checks=True),
    )(A_x, kt, vt, _tiles(A_wq, (D // 32,)), _tiles(A_wo, (H * DH // 16,)),
      B_w1, B_w3, B_w2.reshape(FF // FCH, FCH, D))
```

```python
import jax
import jax.numpy as jnp
import numpy as np
from jax import lax
import jax.experimental.pallas as pl
import jax.experimental.pallas.tpu as pltpu

D = 640
H = 32
NP = H // 2
DH = 192
GH = DH // 8
NG = 2 * GH
FF = 1536
FCH = 256
EPS = 1e-5

NW = 3
W2_SPLITS = ((0, 5), (5, 6))

T_START = 20
T_GROUP = 24.0
T_WIDE = 0.69
T_RESULT = 175
T_RESULT1 = 190
T_FIRST = 740
T_SUM = (40, 200)

f32 = jnp.float32
bf16 = jnp.bfloat16
u32 = jnp.uint32


def _round_bf16(x):
    return x.astype(bf16).astype(f32)


def _as_bf16(x):
    return pltpu.bitcast(x, bf16)


def _as_f32(x):
    return pltpu.bitcast(x, f32)


def _dot(a, b):
    return jnp.dot(a, b, preferred_element_type=f32)


def _gather_rows(x, idx):
    dnums = lax.GatherDimensionNumbers(
        offset_dims=(), collapsed_slice_dims=(0,), start_index_map=(0,),
        operand_batching_dims=(1,), start_indices_batching_dims=(1,))
    return lax.gather(x, idx.reshape(8, 128, 1), dnums, slice_sizes=(1, 1),
                      mode=lax.GatherScatterMode.FILL_OR_DROP)


def _ln_stats(x):
    m = jnp.mean(x, axis=-1, keepdims=True)
    c = x - m
    v = jnp.mean(c * c, axis=-1, keepdims=True)
    return m, c, lax.rsqrt(v + EPS)


def _with_ones(x):
    return jnp.concatenate([x, jnp.ones_like(x)], axis=0).astype(bf16)


def _centered_dot(xo, w, m):
    y = _dot(xo, w)
    return y[0:8] - m * y[8:16]


def _packed(t):
    return _as_f32(jnp.concatenate([t, t], axis=0).astype(bf16))


def _unpack(w):
    return w << 16, w & jnp.uint32(0xFFFF0000)


def _run(*gens):
    for g in gens:
        for _ in g:
            pass


def _take(gen, n):
    for _ in range(n):
        yield next(gen)


def _group_order():
    order = []
    step = GH // NW
    for par in range(2):
        packed = list(range(GH * par, GH * par + GH - NW))
        wide = list(range(GH * par + GH - NW, GH * par + GH))
        order += [(wide if n % step == step // 2 else packed).pop(0)
                  for n in range(GH)]
    return order


def _make_kernel(sk, win):
    nc = win // 128
    ncp = nc // 2
    row0 = (sk - win) // 128 * 4
    assert nc == 32
    scale = float(np.asarray(DH ** -0.5, dtype=bf16))
    order = _group_order()

    def kernel(x_hbm, k_hbm, v_hbm, wq_hbm, wo_hbm, w1_hbm, w3_hbm, w2_hbm,
               o_ref,
               xbuf, kbuf, vbuf, vwide, vlast, wq, wo, w1, w3, w2,
               zq, ybuf, qbuf, pbuf, lbuf, abuf, obuf, zeros, ones, tab,
               ksem, vsem, wsem):
        k32 = k_hbm.bitcast(u32)
        v32 = v_hbm.bitcast(u32)
        window = pl.ds(row0, 4 * nc)

        def k_copy(i):
            return pltpu.make_async_copy(
                k32.at[i, :, :, window, :], kbuf.at[i], ksem.at[i])

        def v_copies(i):
            return (
                pltpu.make_async_copy(
                    v32.at[i, :, pl.ds(0, GH - NW), window, :], vbuf.at[i],
                    vsem.at[2 * i]),
                pltpu.make_async_copy(
                    v32.at[i, :, pl.ds(GH - NW, NW), window, :],
                    vwide.at[i, 1], vsem.at[2 * i + 1]))

        x_copy = pltpu.make_async_copy(x_hbm, xbuf, wsem.at[0])
        wq_copy = pltpu.make_async_copy(wq_hbm.bitcast(u32), wq, wsem.at[1])
        wo_copy = pltpu.make_async_copy(wo_hbm.bitcast(u32), wo, wsem.at[2])
        vlast_copy = pltpu.make_async_copy(
            v32.at[NP - 1, :, :, window, :], vlast.at[1], wsem.at[3])
        w1_copy = pltpu.make_async_copy(w1_hbm, w1, wsem.at[4])
        w3_copy = pltpu.make_async_copy(w3_hbm, w3, wsem.at[5])
        w2_copies = [
            pltpu.make_async_copy(w2_hbm.at[pl.ds(a, b - a)],
                                  w2.at[pl.ds(a, b - a)], wsem.at[6 + n])
            for n, (a, b) in enumerate(W2_SPLITS)]

        wq_copy.start()
        x_copy.start()
        wo_copy.start()
        k_copy(0).start()

        def start_kv(i, carry):
            for cp in v_copies(i):
                cp.start()
            k_copy(i + 1).start()
            return carry

        lax.fori_loop(0, NP - 1, start_kv, 0)
        vlast_copy.start()

        lane = lax.broadcasted_iota(jnp.int32, (8, 128), 1)
        sub = lax.broadcasted_iota(jnp.int32, (8, 128), 0)
        zeros[...] = jnp.zeros((8, 128), u32)
        ones[...] = jnp.ones((8, 128), f32)
        for n in range(4):
            tab[n] = 2 * n + (sub >> 2)
        tab[4] = sub ^ 1
        tab[5] = jnp.zeros_like(sub)
        tab[6] = jnp.where(lane < 64, 0, 2)
        tab[7] = jnp.full_like(sub, 2)
        tab[8] = lane & 8
        tab[9] = sub
        tab[10] = sub - jnp.where(lane < 64, 0, 1)
        tab[11] = sub - 1

        def retile(ref, ntile, place):
            top = sub < 4
            nrep = ref.shape[1] // (8 * ntile)

            def body(a, carry):
                v = [ref[a, 8 * n:8 * n + 8, :] for n in range(nrep * ntile)]
                for k in range(nrep):
                    for t in range(ntile):
                        lo = v[k * ntile + t // 2]
                        hi = v[k * ntile + (ntile + t) // 2]
                        if t % 2:
                            lo = pltpu.roll(lo, 4, 0)
                        if (ntile + t) % 2 == 0:
                            hi = pltpu.roll(hi, 4, 0)
                        r = 8 * place(k, t)
                        ref[a, r:r + 8, :] = jnp.where(top, lo, hi)
                return carry

            lax.fori_loop(0, ref.shape[0], body, 0)

        def k_rows(g, c):
            r = 8 * (c ^ (g // 2 % 4))
            return slice(r, r + 8)

        wq_copy.wait()
        retile(wq, H * DH // 128, lambda k, t: 2 * t + k)
        w1_copy.start()
        w3_copy.start()
        wo_copy.wait()
        retile(wo, D // 128, lambda k, t: t)
        for cp in w2_copies:
            cp.start()

        def expand_q(t, b):
            even = tab[8] == 0
            return [jnp.where(tab[9 + t] == 2 * var, y, jnp.uint32(0))
                    for y in (jnp.where(even, b >> 16, pltpu.roll(b, 8, 1)),
                              jnp.where(even, pltpu.roll(b, 120, 1) >> 16, b))
                    for var in range(2)]

        def q_stage(u, e, out, proj=None, expand=True):
            if e is None:
                wref, e = wq.at[:, pl.ds(pl.multiple_of(48 * u, 16), 48), :], 0
            elif isinstance(u, int):
                wref = wq.at[:, pl.ds(96 * u, 96), :]
            else:
                wref = wq.at[:, pl.ds(pl.multiple_of(96 * u, 32), 96), :]
            for t in range(3):
                r = 48 * e + 16 * t
                w = _as_bf16(wref[:, r:r + 16, :].reshape(D // 2, 128))
                q = proj(w) if proj else _dot(_as_bf16(zq[...]), w)[0:8]
                b = pltpu.bitcast(_round_bf16(q), u32)
                out.extend(expand_q(t, b) if expand else [b])
                yield 40, [(_as_f32(b), 7)]

        def fold_rows(x, op):
            x = op(x, pltpu.roll(x, 4, 0))
            return op(x, _gather_rows(x, tab[4]))

        def k_stage(i, ys, out):
            kref = kbuf.at[i]
            m = None
            for c in range(ncp):
                lhs = jnp.concatenate(
                    [ys(2 * n + c % 2) for n in range(6)], axis=1)
                w = jnp.concatenate(
                    [kref[g // GH, g % GH, k_rows(g, c), :]
                     for t in range(3) for e in range(2)
                     for g in range(16 * t + e, 16 * t + 16, 2)], axis=0)
                s = _dot(_as_bf16(lhs), _as_bf16(w))[0:8]
                if c % 2 == 0:
                    out.append(s)
                    yield 48, [(s, 6)]
                else:
                    out[-1] = out[-1] + s
                    m = out[-1] if m is None else jnp.maximum(m, out[-1])
                    if c == ncp - 1:
                        m = fold_rows(m, jnp.maximum)
                    yield 48, [(m, 12 if c == ncp - 1 else 8)]
            out.append(m)

        def k_first(qb, out_a, out):
            even, low = tab[8] == 0, tab[6] == 0
            b = qb[1]
            rot = {n: pltpu.roll(b, n, 1) for n in (8, 56, 64, 72, 120)}
            mix = (jnp.where(even, jnp.where(low, b, rot[56]) >> 16,
                             jnp.where(low, rot[8], rot[64])),
                   jnp.where(even, jnp.where(low, rot[64], rot[120]) >> 16,
                             jnp.where(low, rot[72], b)))
            tiles = []
            for par in range(2):
                ys = expand_q(2 * par, qb[2 * par])
                for e in range(2):
                    tiles.append((ys[2 * e:2 * e + 2],
                                  range(32 * par + e, 32 * par + 16, 2)))
                g0 = 16 + 8 * par
                tiles.append((
                    [jnp.where(tab[9 + 2 * par] == 2 * var, mix[par],
                               jnp.uint32(0)) for var in range(2)],
                    [*range(g0, g0 + 8, 2), *range(g0 + 1, g0 + 8, 2)]))

            def part(c, sel):
                lhs = jnp.concatenate([tiles[n][0][c % 2] for n in sel], axis=1)
                w = jnp.concatenate(
                    [kbuf[0, g // GH, g % GH, k_rows(g, c), :]
                     for n in sel for g in tiles[n][1]], axis=0)
                return _dot(_as_bf16(lhs), _as_bf16(w))[0:8]

            plan = [(c, (0, 1)) for c in range(4)] + [(c, (2,)) for c in range(4)]
            plan += [(c, (0, 1, 2)) for c in range(4, ncp)]
            acc = [None] * (ncp // 2)
            for c, sel in plan:
                s = part(c, sel)
                acc[c // 2] = s if acc[c // 2] is None else acc[c // 2] + s
                yield 8 * len(sel), []
            m = acc[0]
            for a in acc[1:]:
                m = jnp.maximum(m, a)
            out_a.extend(acc + [fold_rows(m, jnp.maximum)])
            m = None
            for j in range(ncp // 2):
                s = acc[j] + part(2 * j, (3, 4, 5)) + part(2 * j + 1, (3, 4, 5))
                out.append(s)
                m = s if m is None else jnp.maximum(m, s)
                if j == ncp // 2 - 1:
                    m = fold_rows(m, jnp.maximum)
                yield 48, [(m, 8)]
            out.append(m)

        def softmax_numerator(ss, sc=scale):
            m = jnp.max(ss[-1], axis=1, keepdims=True)
            return [jnp.exp((s - m) * sc) for s in ss[:-1]]

        def inverse_sum(ps):
            tot = ps[0]
            for p in ps[1:]:
                tot = tot + p
            lf = fold_rows(tot, jnp.add)
            l = jnp.sum(lf, axis=1, keepdims=True)
            return lf, jnp.broadcast_to(1.0 / l, (8, 128))

        def lane_sums(b, j):
            a = jnp.concatenate(
                [abuf[b, 16 * j:16 * j + 16, 8 * s:8 * s + 8, :].reshape(128, 128)
                 for s in range(2)], axis=1)
            return lax.dot_general(
                jnp.concatenate([ones[...]] * 2, axis=1), a,
                (((1,), (1,)), ((), ())), preferred_element_type=f32)

        def r_stage(b, out):
            for j in range(3):
                out.append(_packed(lane_sums(b, j) * lbuf[b, j]))
                yield 32, [(out[-1], 4)]

        def o_stage(i, ts):
            wref = wo.at[pl.ds(24 * i, 24)]
            t = _as_bf16(jnp.concatenate(ts, axis=1))
            for n in range(D // 128):
                cols = slice(128 * n, 128 * n + 128)
                w = wref[:, 8 * n:8 * n + 8, :].reshape(DH, 128)
                y = obuf[:, cols] + _dot(t, _as_bf16(w))[0:8]
                obuf[:, cols] = y
                yield 24, [(y, 4)]

        def o_tile(i, j, t):
            r0 = 24 * i + 8 * j
            w = jnp.concatenate(
                [wo[r0:r0 + 8, 8 * n:8 * n + 8, :].reshape(64, 128)
                 for n in range(D // 128)], axis=1)
            return _dot(_as_bf16(t), _as_bf16(w))[0:8]

        def trace_mxu(gens, links, latency, t=0.0):
            for gen in gens:
                for cost, res in gen:
                    t += cost
                    links.setdefault(t + latency, []).extend(res)
            return t

        def v_stage(i, b, getp, links, clock, hist, t_sum=None):
            never = zeros[...] != 0
            last = i is None
            for n, g in enumerate(range(NG) if last else order):
                par, gl = divmod(g, GH)
                if n % GH == 0:
                    ps = [getp(par, j) for j in range(nc // 4)]
                    idx = [tab[par], tab[2 + par]]
                    if len(hist) > 1 and getp is not from_pbuf:
                        dep = pltpu.bitcast(hist[-2][0], jnp.int32)
                        idx = [jnp.where(never, dep, ix) for ix in idx]
                    pv = [_gather_rows(ps[c // 2], idx[c % 2])
                          for c in range(ncp)]
                    clock[0] += 4
                    if par == 1 and not last:
                        lf, inv = inverse_sum(ps)
                        for val, at in zip((lf, inv), t_sum or ()):
                            links.setdefault(clock[0] + at, []).append((val, 14))
                        for j in range(3):
                            lbuf[b, j] = _gather_rows(inv, tab[5 + j])
                wide = last or gl >= GH - NW
                if last:
                    ref = vlast.at[:, par, gl]
                elif wide:
                    ref = vwide.at[i, :, par, gl - (GH - NW)]
                else:
                    ref = vbuf.at[i, par, gl]
                dur = T_GROUP * (T_WIDE if wide else 1.0)
                accs = [None, None]
                held = [None, None]
                pending = []
                for c in range(ncp):
                    for key in sorted(links):
                        if key < clock[0] + dur * (c + 1) / 16:
                            for val, ops in links.pop(key):
                                pending.append(val)
                                clock[0] += ops / 4
                    rs = slice(8 * c, 8 * c + 8)
                    if wide:
                        lo, hi = ref[0, rs, :], ref[1, rs, :]
                    else:
                        lo, hi = _unpack(ref[rs, :])
                    p = pv[c]
                    if c == (6 if wide else 0) and hist and not last:
                        p = jnp.where(never, hist[-1][0] + hist[-1][1], p)
                    for a, t in enumerate((_as_f32(lo) * p, _as_f32(hi) * p)):
                        if accs[a] is None:
                            accs[a] = t
                            continue
                        if pending:
                            t = jnp.where(never, pending.pop(), t)
                        if c % 2 == 1 and c < ncp - 1:
                            held[a] = t
                        else:
                            if held[a] is not None:
                                t = held[a] + t
                                held[a] = None
                            accs[a] = accs[a] + t
                for a in range(2):
                    abuf[b, g, pl.ds(a, 8, stride=2), :] = accs[a]
                clock[0] += dur
                hist.append(accs)
                yield g

        def from_pbuf(par, j):
            return pbuf[par, j]

        def store_p(ps):
            for j, p in enumerate(ps):
                pbuf[0, j] = p
                pbuf[1, j] = p

        def two_pairs(it):
            i = 2 * it
            links, clock, hist = {}, [T_START], []
            s1, s2, ya, qb, t0, t1 = [], [], [], [], [], []
            y2 = [y for t in range(3) for y in expand_q(t, qbuf[t])]
            k2 = k_stage(i + 2, lambda n: y2[n], s2)
            t = trace_mxu([k_stage(i + 1, lambda n: ybuf[n], s1)],
                          links, T_RESULT)
            p1 = softmax_numerator(s1)
            t = trace_mxu([r_stage(1, t1), q_stage(it + 1, 1, ya),
                           o_stage(i - 1, t1), _take(k2, 4)],
                          links, T_RESULT, t)
            _run(v_stage(i, 0, from_pbuf, links, clock, hist, T_SUM))
            t = trace_mxu([r_stage(0, t0), k2], links, T_RESULT,
                          max(t, clock[0] - 64))
            p2 = softmax_numerator(s2)
            trace_mxu([o_stage(i, t0),
                       q_stage(jnp.minimum(it + 2, NP // 2 - 1), 0, qb,
                               expand=False)], links, T_RESULT, t)
            _run(v_stage(i + 1, 1, lambda par, j: p1[j], links, clock,
                         hist, T_SUM))
            for n in range(12):
                ybuf[n] = ya[n]
            for n in range(3):
                qbuf[n] = qb[n]
            store_p(p2)

        def first_pairs(xo, m, r):
            links, clock, hist = {}, [T_FIRST], []
            q0, y1, y2, sa, s0, s1, s2, ya, qb, t0 = ([] for _ in range(10))
            _run(q_stage(0, 0, q0, lambda w: _centered_dot(xo, w, m), False),
                 q_stage(0, 1, y1, lambda w: _centered_dot(xo, w, m) * r))
            t = trace_mxu([k_first(q0, sa, s0),
                           k_stage(1, lambda n: y1[n], s1),
                           q_stage(1, 0, y2), q_stage(1, 1, ya),
                           q_stage(2, 0, qb, expand=False)], links, T_RESULT1)
            for key in [key for key in links if key < T_FIRST + 30]:
                del links[key]
            pa = softmax_numerator(sa, r * scale)
            p0 = softmax_numerator(s0, r * scale)
            p1 = softmax_numerator(s1)
            _run(v_stage(0, 0, lambda par, j: (pa, p0)[par][j], links,
                         clock, hist, T_SUM))
            trace_mxu([r_stage(0, t0), k_stage(2, lambda n: y2[n], s2),
                       o_stage(0, t0)], links, T_RESULT1,
                      max(t, clock[0] - 64))
            p2 = softmax_numerator(s2)
            _run(v_stage(1, 1, lambda par, j: p1[j], links, clock,
                         hist, T_SUM))
            for n in range(12):
                ybuf[n] = ya[n]
            for n in range(3):
                qbuf[n] = qb[n]
            store_p(p2)

        def one_pair():
            i = NP - 2
            links = {}
            s1, t1 = [], []
            trace_mxu([r_stage(1, t1), k_stage(i + 1, lambda n: ybuf[n], s1),
                       o_stage(i - 1, t1)], links, T_RESULT1)
            _run(v_stage(i, 0, from_pbuf, links, [T_START], []))
            store_p(softmax_numerator(s1))

        def last_pair():
            ts = [_packed(lane_sums(0, j) * lbuf[0, j]) for j in range(3)]
            lf, inv = inverse_sum([pbuf[1, j] for j in range(nc // 4)])
            tn = []
            for g in v_stage(None, 1, from_pbuf, {50: [(lf, 0)]},
                             [0.0], []):
                if g % 16 == 15:
                    j = g // 16
                    tn.append(_packed(
                        lane_sums(1, j) * _gather_rows(inv, tab[5 + j])))
            y = obuf[...]
            for j in range(3):
                y = y + o_tile(NP - 2, j, ts[j])
            for j in range(3):
                y = y + o_tile(NP - 1, j, tn[j])
            return y

        def start_attention(x):
            m, c, r = _ln_stats(x)
            z = c * r
            zq[...] = pltpu.bitcast(
                jnp.concatenate([z, z], axis=0).astype(bf16), u32)
            obuf[...] = jnp.zeros(obuf.shape, f32)
            return m, r

        def attention(x):
            m, r = start_attention(x)
            first_pairs(_with_ones(x), m, r)

            def body(it, count):
                two_pairs(it)
                return count + 1

            count = lax.fori_loop(1, NP // 2 - 1, body, 0)
            pl.when(count > 0)(one_pair)
            return last_pair()

        def streamed_pair(i, u, e):
            last = isinstance(i, int)
            ys = []
            _run(q_stage(u, e, ys))
            lhs = [_as_bf16(jnp.concatenate(ys[var::2], axis=1))
                   for var in range(2)]
            k_copy(i).wait()
            ss = []
            for c in range(ncp):
                k = kbuf[i, :, :, 8 * c:8 * c + 8, :].reshape(3, 8, 2, 8, 128)
                w = jnp.concatenate(
                    [k[t, :, par].reshape(64, 128)
                     for t in range(3) for par in range(2)], axis=0)
                s = _dot(lhs[c % 2], _as_bf16(w))[0:8]
                if c % 2:
                    s = ss.pop() + s
                ss.append(s)
            m = ss[0]
            for s in ss[1:]:
                m = jnp.maximum(m, s)
            ps = softmax_numerator(ss + [fold_rows(m, jnp.maximum)])
            inv = inverse_sum(ps)[1]
            for j in range(3):
                lbuf[0, j] = _gather_rows(inv, tab[5 + j])

            def swizzle(a, carry):
                for g in range(2, 8):
                    ref = kbuf.at[i, a // 3, 8 * (a % 3) + g]
                    v = ref[...].reshape(4, 4, 8, 128)
                    v = jnp.concatenate(
                        [v[:, c ^ (g // 2):(c ^ (g // 2)) + 1] for c in range(4)],
                        axis=1)
                    ref[...] = v.reshape(128, 128)
                return carry

            lax.fori_loop(0, NG // 8, swizzle, 0)

            for cp in ((vlast_copy,) if last else v_copies(i)):
                cp.wait()
            for par in range(2):
                pv = jnp.concatenate(
                    [_gather_rows(ps[c // 2], tab[2 * (c % 2) + par])
                     for c in range(ncp)], axis=0)

                def group(g, w):
                    for a, half in enumerate(_unpack(w)):
                        acc = (_as_f32(half) * pv).reshape(ncp, 8, 128)
                        abuf[0, g, pl.ds(a, 8, stride=2), :] = jnp.sum(acc, axis=0)

                def packed_group(gl, carry):
                    group(GH * par + gl, vbuf[i, par, gl])
                    return carry

                def wide_group(gl, carry):
                    ref = (vlast.at[:, par, gl] if last
                           else vwide.at[i, :, par, gl - (GH - NW)])
                    w = ref[1]
                    ref[0], ref[1] = _unpack(w)
                    group(GH * par + gl, w)
                    return carry

                split = 0 if last else GH - NW
                if split:
                    lax.fori_loop(0, split, packed_group, 0)
                lax.fori_loop(split, GH, wide_group, 0)
            ts = []
            _run(r_stage(0, ts), o_stage(i, ts))

        def streamed_attention(x):
            start_attention(x)

            def body(i, carry):
                streamed_pair(i, i, None)
                return carry

            lax.fori_loop(0, NP - 1, body, 0)
            streamed_pair(NP - 1, NP // 2 - 1, 1)
            return obuf[...]

        def ffn(first, x):
            if first:
                w1_copy.wait()
                w3_copy.wait()
            m, _, r = _ln_stats(x)
            xo = _with_ones(x)
            hids = []
            for n in range(0, FF, FCH):
                gate = _round_bf16(_centered_dot(xo, w1[:, n:n + FCH], m) * r)
                up = _round_bf16(_centered_dot(xo, w3[:, n:n + FCH], m) * r)
                hids.append(
                    (_round_bf16(gate * jax.nn.sigmoid(gate)) * up).astype(bf16))
            y = None
            starts = [a for a, _ in W2_SPLITS]
            for n, hid in enumerate(hids):
                if first and n in starts:
                    if y is not None:
                        obuf[...] = y
                    w2_copies[starts.index(n)].wait()
                    if y is not None:
                        y = obuf[...]
                t = _dot(hid, w2[n])
                y = t if y is None else y + t
            return y

        x_copy.wait()
        x = jnp.broadcast_to(xbuf[0].astype(f32), (8, D))
        x = _round_bf16(x + _round_bf16(streamed_attention(x)))
        x = _round_bf16(x + _round_bf16(ffn(True, x)))
        x = _round_bf16(x + _round_bf16(attention(x)))
        x = _round_bf16(x + _round_bf16(ffn(False, x)))
        o_ref[0] = x[0:1].astype(bf16)

    return kernel


def _tiles(a, lead):
    r, c = a.shape
    t = a.reshape(r // 8, 8, c // 128, 128).transpose(0, 2, 1, 3)
    return t.reshape(lead + (-1, 128))


@jax.jit
def pallas_interleave_layers__sliding_block_cached__glu_gated_swiglu__decode_kernel(
    A_x: jax.Array,
    A_k_cache: jax.Array,
    A_v_cache: jax.Array,
    A_wq: jax.Array,
    A_wo: jax.Array,
    B_x: jax.Array,
    B_w1: jax.Array,
    B_w3: jax.Array,
    B_w2: jax.Array,
):
    del B_x
    sk = A_k_cache.shape[2]
    win = min(4096, max(256, sk // 4))
    wr = win // 32
    kt = _tiles(jnp.swapaxes(A_k_cache, 2, 3).reshape(H * DH, sk), (NP, 2, GH))
    vt = _tiles(jnp.swapaxes(A_v_cache, 2, 3).reshape(H * DH, sk), (NP, 2, GH))
    any_spec = pl.BlockSpec(memory_space=pl.ANY)
    return pl.pallas_call(
        _make_kernel(sk, win),
        out_shape=jax.ShapeDtypeStruct((1, 1, D), bf16),
        in_specs=[any_spec] * 8,
        out_specs=pl.BlockSpec(memory_space=pltpu.VMEM),
        scratch_shapes=[
            pltpu.VMEM((1, 1, D), bf16),
            pltpu.VMEM((NP, 2, GH, wr, 128), u32),
            pltpu.VMEM((NP - 1, 2, GH - NW, wr, 128), u32),
            pltpu.VMEM((NP - 1, 2, 2, NW, wr, 128), u32),
            pltpu.VMEM((2, 2, GH, wr, 128), u32),
            pltpu.VMEM((D // 32, H * DH // 8, 128), u32),
            pltpu.VMEM((H * DH // 16, D // 16, 128), u32),
            pltpu.VMEM((D, FF), bf16),
            pltpu.VMEM((D, FF), bf16),
            pltpu.VMEM((FF // FCH, FCH, D), bf16),
            pltpu.VMEM((8, D), u32),
            pltpu.VMEM((12, 8, 128), u32),
            pltpu.VMEM((3, 8, 128), u32),
            pltpu.VMEM((2, 8, 8, 128), f32),
            pltpu.VMEM((2, 3, 8, 128), f32),
            pltpu.VMEM((2, NG, 16, 128), f32),
            pltpu.VMEM((8, D), f32),
            pltpu.VMEM((8, 128), u32),
            pltpu.VMEM((8, 128), f32),
            pltpu.VMEM((12, 8, 128), jnp.int32),
            pltpu.SemaphoreType.DMA((NP,)),
            pltpu.SemaphoreType.DMA((2 * NP - 2,)),
            pltpu.SemaphoreType.DMA((8,)),
        ],
        compiler_params=pltpu.CompilerParams(
            vmem_limit_bytes=128 * 1024 * 1024,
            disable_semaphore_checks=True),
    )(A_x, kt, vt, _tiles(A_wq, (D // 32,)), _tiles(A_wo, (H * DH // 16,)),
      B_w1, B_w3, B_w2.reshape(FF // FCH, FCH, D))
```

```python
import jax
import jax.numpy as jnp
import numpy as np
from jax import lax
import jax.experimental.pallas as pl
import jax.experimental.pallas.tpu as pltpu

D = 640
H = 32
NP = H // 2
DH = 192
GH = DH // 8
NG = 2 * GH
FF = 1536
FCH = 256
EPS = 1e-5

NT = 7
NW = 3
W2_SPLITS = ((0, 5), (5, 6))

T_START = 20
T_GROUP = 24.0
T_WIDE = 0.69
T_RESULT = 175
T_RESULT1 = 190
T_FIRST = 740
T_SUM = (40, 200)
T_LAST = 12.0

f32 = jnp.float32
bf16 = jnp.bfloat16
u32 = jnp.uint32


def _round_bf16(x):
    return x.astype(bf16).astype(f32)


def _as_bf16(x):
    return pltpu.bitcast(x, bf16)


def _as_f32(x):
    return pltpu.bitcast(x, f32)


def _dot(a, b):
    return jnp.dot(a, b, preferred_element_type=f32)


def _gather_rows(x, idx):
    dnums = lax.GatherDimensionNumbers(
        offset_dims=(), collapsed_slice_dims=(0,), start_index_map=(0,),
        operand_batching_dims=(1,), start_indices_batching_dims=(1,))
    return lax.gather(x, idx.reshape(8, 128, 1), dnums, slice_sizes=(1, 1),
                      mode=lax.GatherScatterMode.FILL_OR_DROP)


def _ln_stats(x):
    m = jnp.mean(x, axis=-1, keepdims=True)
    c = x - m
    v = jnp.mean(c * c, axis=-1, keepdims=True)
    return m, c, lax.rsqrt(v + EPS)


def _with_ones(x):
    return jnp.concatenate([x, jnp.ones_like(x)], axis=0).astype(bf16)


def _centered_dot(xo, w, m):
    y = _dot(xo, w)
    return y[0:8] - m * y[8:16]


def _packed(t):
    return _as_f32(jnp.concatenate([t, t], axis=0).astype(bf16))


def _unpack(w):
    return w << 16, w & jnp.uint32(0xFFFF0000)


def _run(*gens):
    for g in gens:
        for _ in g:
            pass


def _take(gen, n):
    for _ in range(n):
        yield next(gen)


def _group_order():
    order = []
    step = GH // NW
    for par in range(2):
        packed = list(range(GH * par, GH * par + GH - NW))
        wide = list(range(GH * par + GH - NW, GH * par + GH))
        order += [(wide if n % step == step // 2 else packed).pop(0)
                  for n in range(GH)]
    return order


def _make_kernel(sk, win):
    nc = win // 128
    ncp = nc // 2
    row0 = (sk - win) // 128 * 4
    assert nc == 32
    scale = float(np.asarray(DH ** -0.5, dtype=bf16)) * float(np.log2(np.e))
    order = _group_order()

    def kernel(x_hbm, k_hbm, v_hbm, wq_hbm, wo_hbm, w1_hbm, w3_hbm, w2_hbm,
               o_ref,
               xbuf, kbuf, vbuf, vwide, vlast, wq, wo, w1, w3, w2,
               zq, ybuf, qbuf, pbuf, lbuf, abuf, obuf, zeros, ones, tab,
               ksem, vsem, wsem):
        k32 = k_hbm.bitcast(u32)
        v32 = v_hbm.bitcast(u32)
        window = pl.ds(row0, 4 * nc)

        def k_copy(i):
            return pltpu.make_async_copy(
                k32.at[i, :, :, window, :], kbuf.at[i], ksem.at[i])

        def v_copies(i):
            return (
                pltpu.make_async_copy(
                    v32.at[i, :, pl.ds(0, GH - NW), window, :], vbuf.at[i],
                    vsem.at[2 * i]),
                pltpu.make_async_copy(
                    v32.at[i, :, pl.ds(GH - NW, NW), window, :],
                    vwide.at[i, 1], vsem.at[2 * i + 1]))

        x_copy = pltpu.make_async_copy(x_hbm, xbuf, wsem.at[0])
        wq_copy = pltpu.make_async_copy(wq_hbm.bitcast(u32), wq, wsem.at[1])
        wo_copy = pltpu.make_async_copy(wo_hbm.bitcast(u32), wo, wsem.at[2])
        vlast_copy = pltpu.make_async_copy(
            v32.at[NP - 1, :, :, window, :], vlast.at[1], wsem.at[3])
        w1_copy = pltpu.make_async_copy(w1_hbm, w1, wsem.at[4])
        w3_copy = pltpu.make_async_copy(w3_hbm, w3, wsem.at[5])
        w2_copies = [
            pltpu.make_async_copy(w2_hbm.at[pl.ds(a, b - a)],
                                  w2.at[pl.ds(a, b - a)], wsem.at[6 + n])
            for n, (a, b) in enumerate(W2_SPLITS)]

        wq_copy.start()
        x_copy.start()
        wo_copy.start()
        k_copy(0).start()

        def start_kv(i, carry):
            for cp in v_copies(i):
                cp.start()
            k_copy(i + 1).start()
            return carry

        lax.fori_loop(0, NP - 1, start_kv, 0)
        vlast_copy.start()

        lane = lax.broadcasted_iota(jnp.int32, (8, 128), 1)
        sub = lax.broadcasted_iota(jnp.int32, (8, 128), 0)
        zeros[...] = jnp.zeros((8, 128), u32)
        ones[...] = jnp.ones((8, 128), f32)
        for n in range(4):
            tab[n] = 2 * n + (sub >> 2)
        tab[4] = sub ^ 1
        tab[5] = jnp.zeros_like(sub)
        tab[6] = jnp.where(lane < 64, 0, 2)
        tab[7] = jnp.full_like(sub, 2)
        tab[8] = lane & 8
        tab[9] = sub
        tab[10] = sub - jnp.where(lane < 64, 0, 1)
        tab[11] = sub - 1
        for n in range(4):
            tab[12 + n] = jnp.where((sub >> 1) == n // 2,
                                    -65536 if n % 2 else 65535, 0)

        def retile(ref, ntile, place):
            top = sub < 4
            nrep = ref.shape[1] // (8 * ntile)

            def body(a, carry):
                v = [ref[a, 8 * n:8 * n + 8, :] for n in range(nrep * ntile)]
                for k in range(nrep):
                    for t in range(ntile):
                        lo = v[k * ntile + t // 2]
                        hi = v[k * ntile + (ntile + t) // 2]
                        if t % 2:
                            lo = pltpu.roll(lo, 4, 0)
                        if (ntile + t) % 2 == 0:
                            hi = pltpu.roll(hi, 4, 0)
                        r = 8 * place(k, t)
                        ref[a, r:r + 8, :] = jnp.where(top, lo, hi)
                return carry

            lax.fori_loop(0, ref.shape[0], body, 0)

        def k_rows(g, c):
            r = 8 * (c ^ (g // 2 % 4))
            return slice(r, r + 8)

        wq_copy.wait()
        retile(wq, H * DH // 128, lambda k, t: 2 * t + k)
        w1_copy.start()
        w3_copy.start()
        wo_copy.wait()
        retile(wo, D // 128, lambda k, t: t)
        for cp in w2_copies:
            cp.start()

        def expand_q(t, b):
            even = tab[8] == 0
            return [jnp.where(tab[9 + t] == 2 * var, y, jnp.uint32(0))
                    for y in (jnp.where(even, b >> 16, pltpu.roll(b, 8, 1)),
                              jnp.where(even, pltpu.roll(b, 120, 1) >> 16, b))
                    for var in range(2)]

        def q_stage(u, e, out, proj=None, expand=True):
            if e is None:
                wref, e = wq.at[:, pl.ds(pl.multiple_of(48 * u, 16), 48), :], 0
            elif isinstance(u, int):
                wref = wq.at[:, pl.ds(96 * u, 96), :]
            else:
                wref = wq.at[:, pl.ds(pl.multiple_of(96 * u, 32), 96), :]
            for t in range(3):
                r = 48 * e + 16 * t
                w = _as_bf16(wref[:, r:r + 16, :].reshape(D // 2, 128))
                q = proj(w) if proj else _dot(_as_bf16(zq[...]), w)[0:8]
                b = pltpu.bitcast(_round_bf16(q), u32)
                out.extend(expand_q(t, b) if expand else [b])
                yield 40, [(_as_f32(b), 7)]

        def fold_rows(x, op):
            x = op(x, pltpu.roll(x, 4, 0))
            return op(x, _gather_rows(x, tab[4]))

        def k_stage(i, ys, out):
            kref = kbuf.at[i]
            m = None
            for c in range(ncp):
                lhs = jnp.concatenate(
                    [ys(2 * n + c % 2) for n in range(6)], axis=1)
                w = jnp.concatenate(
                    [kref[g // GH, g % GH, k_rows(g, c), :]
                     for t in range(3) for e in range(2)
                     for g in range(16 * t + e, 16 * t + 16, 2)], axis=0)
                s = _dot(_as_bf16(lhs), _as_bf16(w))[0:8]
                if c % 2 == 0:
                    out.append(s)
                    yield 48, [(s, 6)]
                else:
                    out[-1] = out[-1] + s
                    m = out[-1] if m is None else jnp.maximum(m, out[-1])
                    if c == ncp - 1:
                        m = fold_rows(m, jnp.maximum)
                    yield 48, [(m, 12 if c == ncp - 1 else 8)]
            out.append(m)

        def k_first(qb, out_a, out):
            even, low = tab[8] == 0, tab[6] == 0
            b = qb[1]
            rot = {n: pltpu.roll(b, n, 1) for n in (8, 56, 64, 72, 120)}
            mix = (jnp.where(even, jnp.where(low, b, rot[56]) >> 16,
                             jnp.where(low, rot[8], rot[64])),
                   jnp.where(even, jnp.where(low, rot[64], rot[120]) >> 16,
                             jnp.where(low, rot[72], b)))
            tiles = []
            for par in range(2):
                ys = expand_q(2 * par, qb[2 * par])
                for e in range(2):
                    tiles.append((ys[2 * e:2 * e + 2],
                                  range(32 * par + e, 32 * par + 16, 2)))
                g0 = 16 + 8 * par
                tiles.append((
                    [jnp.where(tab[9 + 2 * par] == 2 * var, mix[par],
                               jnp.uint32(0)) for var in range(2)],
                    [*range(g0, g0 + 8, 2), *range(g0 + 1, g0 + 8, 2)]))

            def part(c, sel):
                lhs = jnp.concatenate([tiles[n][0][c % 2] for n in sel], axis=1)
                w = jnp.concatenate(
                    [kbuf[0, g // GH, g % GH, k_rows(g, c), :]
                     for n in sel for g in tiles[n][1]], axis=0)
                return _dot(_as_bf16(lhs), _as_bf16(w))[0:8]

            plan = [(c, (0, 1)) for c in range(4)] + [(c, (2,)) for c in range(4)]
            plan += [(c, (0, 1, 2)) for c in range(4, ncp)]
            acc = [None] * (ncp // 2)
            for c, sel in plan:
                s = part(c, sel)
                acc[c // 2] = s if acc[c // 2] is None else acc[c // 2] + s
                yield 8 * len(sel), []
            m = acc[0]
            for a in acc[1:]:
                m = jnp.maximum(m, a)
            out_a.extend(acc + [fold_rows(m, jnp.maximum)])
            m = None
            for j in range(ncp // 2):
                s = acc[j] + part(2 * j, (3, 4, 5)) + part(2 * j + 1, (3, 4, 5))
                out.append(s)
                m = s if m is None else jnp.maximum(m, s)
                if j == ncp // 2 - 1:
                    m = fold_rows(m, jnp.maximum)
                yield 48, [(m, 8)]
            out.append(m)

        def softmax_numerator(ss, sc=scale):
            m = jnp.max(ss[-1], axis=1, keepdims=True)
            return [jnp.exp2((s - m) * sc) for s in ss[:-1]]

        def inverse_sum(ps):
            tot = ps[0]
            for p in ps[1:]:
                tot = tot + p
            lf = fold_rows(tot, jnp.add)
            l = jnp.sum(lf, axis=1, keepdims=True)
            l = jnp.broadcast_to(l, (8, 128))
            y = pl.reciprocal(l, approx=True)
            return lf, y * (2.0 - l * y)

        def lane_sums(b, j):
            a = jnp.concatenate(
                [abuf[b, 16 * j:16 * j + 16, 8 * s:8 * s + 8, :].reshape(128, 128)
                 for s in range(2)], axis=1)
            return lax.dot_general(
                jnp.concatenate([ones[...]] * 2, axis=1), a,
                (((1,), (1,)), ((), ())), preferred_element_type=f32)

        def r_stage(b, out):
            for j in range(3):
                out.append(_packed(lane_sums(b, j) * lbuf[b, j]))
                yield 32, [(out[-1], 4)]

        def o_stage(i, ts):
            wref = wo.at[pl.ds(24 * i, 24)]
            t = _as_bf16(jnp.concatenate(ts, axis=1))
            for n in range(D // 128):
                cols = slice(128 * n, 128 * n + 128)
                w = wref[:, 8 * n:8 * n + 8, :].reshape(DH, 128)
                y = obuf[:, cols] + _dot(t, _as_bf16(w))[0:8]
                obuf[:, cols] = y
                yield 24, [(y, 4)]

        def o_tile(i, j, t):
            r0 = 24 * i + 8 * j
            w = jnp.concatenate(
                [wo[r0:r0 + 8, 8 * n:8 * n + 8, :].reshape(64, 128)
                 for n in range(D // 128)], axis=1)
            return _dot(_as_bf16(t), _as_bf16(w))[0:8]

        def trace_mxu(gens, links, latency, t=0.0):
            for gen in gens:
                for cost, res in gen:
                    t += cost
                    links.setdefault(t + latency, []).extend(res)
            return t

        def v_stage(i, b, getp, links, clock, hist, t_sum=None):
            never = zeros[...] != 0
            last = i is None
            for n, g in enumerate(range(NG) if last else order):
                par, gl = divmod(g, GH)
                if n % GH == 0:
                    ps = [getp(par, j) for j in range(nc // 4)]
                    idx = [tab[par], tab[2 + par]]
                    if len(hist) > 1 and getp is not from_pbuf:
                        dep = pltpu.bitcast(hist[-2][0], jnp.int32)
                        idx = [jnp.where(never, dep, ix) for ix in idx]
                    pv = [_gather_rows(ps[c // 2], idx[c % 2])
                          for c in range(ncp - NT if last else ncp)]
                    clock[0] += 4
                    if par == 1 and not last:
                        lf, inv = inverse_sum(ps)
                        for val, at in zip((lf, inv), t_sum or ()):
                            links.setdefault(clock[0] + at, []).append((val, 14))
                        for j in range(3):
                            lbuf[b, j] = _gather_rows(inv, tab[5 + j])
                wide = last or gl >= GH - NW
                if last:
                    ref = vlast.at[:, par, gl]
                elif wide:
                    ref = vwide.at[i, :, par, gl - (GH - NW)]
                else:
                    ref = vbuf.at[i, par, gl]
                dur = T_LAST if last else T_GROUP * (T_WIDE if wide else 1.0)
                accs = [None, None]
                held = [None, None]
                pending = []
                nsteps = ncp - NT if last else ncp
                for c in range(nsteps):
                    for key in sorted(links):
                        if key < clock[0] + dur * (c + 1) / nsteps:
                            for val, ops in links.pop(key):
                                pending.append(val)
                                clock[0] += ops / 4
                    rs = slice(8 * c, 8 * c + 8)
                    if wide:
                        lo, hi = ref[0, rs, :], ref[1, rs, :]
                    else:
                        lo, hi = _unpack(ref[rs, :])
                    p = pv[c]
                    if c == (8 if last else 6 if wide else 0) and hist:
                        p = jnp.where(never, hist[-1][0] + hist[-1][1], p)
                    for a, t in enumerate((_as_f32(lo) * p, _as_f32(hi) * p)):
                        if accs[a] is None:
                            accs[a] = t
                            continue
                        if pending:
                            t = jnp.where(never, pending.pop(), t)
                        if c % 2 == 1 and c < nsteps - 1:
                            held[a] = t
                        else:
                            if held[a] is not None:
                                t = held[a] + t
                                held[a] = None
                            accs[a] = accs[a] + t
                for a in range(2):
                    abuf[b, g, pl.ds(a, 8, stride=2), :] = accs[a]
                clock[0] += dur
                hist.append(accs)
                yield g

        def from_pbuf(par, j):
            return pbuf[par, j]

        def store_p(ps):
            for j, p in enumerate(ps):
                pbuf[0, j] = p
                pbuf[1, j] = p

        def two_pairs(it):
            i = 2 * it
            links, clock, hist = {}, [T_START], []
            s1, s2, ya, qb, t0, t1 = [], [], [], [], [], []
            y2 = [y for t in range(3) for y in expand_q(t, qbuf[t])]
            k2 = k_stage(i + 2, lambda n: y2[n], s2)
            t = trace_mxu([k_stage(i + 1, lambda n: ybuf[n], s1)],
                          links, T_RESULT)
            p1 = softmax_numerator(s1)
            t = trace_mxu([r_stage(1, t1), q_stage(it + 1, 1, ya),
                           o_stage(i - 1, t1), _take(k2, 4)],
                          links, T_RESULT, t)
            _run(v_stage(i, 0, from_pbuf, links, clock, hist, T_SUM))
            t = trace_mxu([r_stage(0, t0), k2], links, T_RESULT,
                          max(t, clock[0] - 64))
            p2 = softmax_numerator(s2)
            trace_mxu([o_stage(i, t0),
                       q_stage(jnp.minimum(it + 2, NP // 2 - 1), 0, qb,
                               expand=False)], links, T_RESULT, t)
            _run(v_stage(i + 1, 1, lambda par, j: p1[j], links, clock,
                         hist, T_SUM))
            for n in range(12):
                ybuf[n] = ya[n]
            for n in range(3):
                qbuf[n] = qb[n]
            store_p(p2)

        def first_pairs(xo, m, r):
            links, clock, hist = {}, [T_FIRST], []
            q0, y1, y2, sa, s0, s1, s2, ya, qb, t0 = ([] for _ in range(10))
            _run(q_stage(0, 0, q0, lambda w: _centered_dot(xo, w, m), False),
                 q_stage(0, 1, y1, lambda w: _centered_dot(xo, w, m) * r))
            t = trace_mxu([k_first(q0, sa, s0),
                           k_stage(1, lambda n: y1[n], s1),
                           q_stage(1, 0, y2), q_stage(1, 1, ya),
                           q_stage(2, 0, qb, expand=False)], links, T_RESULT1)
            for key in [key for key in links if key < T_FIRST + 30]:
                del links[key]
            pa = softmax_numerator(sa, r * scale)
            p0 = softmax_numerator(s0, r * scale)
            p1 = softmax_numerator(s1)
            _run(v_stage(0, 0, lambda par, j: (pa, p0)[par][j], links,
                         clock, hist, T_SUM))
            trace_mxu([r_stage(0, t0), k_stage(2, lambda n: y2[n], s2),
                       o_stage(0, t0)], links, T_RESULT1,
                      max(t, clock[0] - 64))
            p2 = softmax_numerator(s2)
            _run(v_stage(1, 1, lambda par, j: p1[j], links, clock,
                         hist, T_SUM))
            for n in range(12):
                ybuf[n] = ya[n]
            for n in range(3):
                qbuf[n] = qb[n]
            store_p(p2)

        def vt_slot(kc, j, n):
            g = 24 * (kc % 2) + 8 * j + n
            r = 8 * (kc // 2)
            return (0, g // GH, g % GH, slice(r, r + 8), slice(None))

        def last_pairs():
            i = NP - 2
            links, clock, hist = {}, [T_START], []
            s1, t0, t1, ts, part, rows = ([] for _ in range(6))
            tk = trace_mxu([k_stage(i + 1, lambda n: ybuf[n], s1)], links, 185)
            t = trace_mxu([r_stage(1, t1)], links, 185, tk)
            t = trace_mxu([o_stage(i - 1, t1)], links, 185, t + 60)
            ps = softmax_numerator(s1)
            chunks = range(nc - 2 * NT, nc)
            for kc in chunks:
                bits = pltpu.bitcast(_packed(ps[kc // 4]), u32)
                rows.append(bits & pltpu.bitcast(tab[12 + kc % 4], u32))
                links.setdefault(tk + 315, []).append((_as_f32(rows[-1]), 3))
            lhs = _as_bf16(jnp.concatenate(rows, axis=1))

            def p_stage():
                for j in range(3):
                    w = jnp.concatenate([vlast[vt_slot(kc, j, n)]
                                         for kc in chunks for n in range(8)],
                                        axis=0)
                    y = fold_rows(_dot(lhs, _as_bf16(w))[0:8], jnp.add)
                    part.append(_gather_rows(y, tab[5 + j]))
                    yield 16 * NT, [(part[j], 2 * NT + 5)]

            pg = p_stage()
            t = trace_mxu([_take(pg, 1)], links, 210, max(t, tk + 266))
            _run(v_stage(i, 0, from_pbuf, links, clock, hist))
            trace_mxu([r_stage(0, t0), _take(pg, 1), o_stage(i, t0), pg],
                      links, 210, max(t, clock[0] + 56))
            lf, inv = inverse_sum(ps)
            links.setdefault(clock[0] + 20, []).append((lf, 10))
            links.setdefault(clock[0] + 160, []).append((inv, 10))
            for g in v_stage(None, 1, lambda par, j: ps[j], links, clock, hist):
                if g % 16 == 15:
                    j = g // 16
                    ts.append(_packed((lane_sums(1, j) + part[j])
                                      * _gather_rows(inv, tab[5 + j])))
            y = obuf[...]
            for j in range(3):
                y = y + o_tile(NP - 1, j, ts[j])
            return y

        def start_attention(x):
            m, c, r = _ln_stats(x)
            z = c * r
            zq[...] = pltpu.bitcast(
                jnp.concatenate([z, z], axis=0).astype(bf16), u32)
            obuf[...] = jnp.zeros(obuf.shape, f32)
            return m, r

        def attention(x):
            m, r = start_attention(x)
            first_pairs(_with_ones(x), m, r)

            def body(it, carry):
                two_pairs(it)
                return carry

            lax.fori_loop(1, NP // 2 - 1, body, 0)
            return last_pairs()

        def streamed_pair(i, u, e):
            last = isinstance(i, int)
            ys = []
            _run(q_stage(u, e, ys))
            lhs = [_as_bf16(jnp.concatenate(ys[var::2], axis=1))
                   for var in range(2)]
            k_copy(i).wait()
            ss = []
            for c in range(ncp):
                k = kbuf[i, :, :, 8 * c:8 * c + 8, :].reshape(3, 8, 2, 8, 128)
                w = jnp.concatenate(
                    [k[t, :, par].reshape(64, 128)
                     for t in range(3) for par in range(2)], axis=0)
                s = _dot(lhs[c % 2], _as_bf16(w))[0:8]
                if c % 2:
                    s = ss.pop() + s
                ss.append(s)
            m = ss[0]
            for s in ss[1:]:
                m = jnp.maximum(m, s)
            ps = softmax_numerator(ss + [fold_rows(m, jnp.maximum)])
            inv = inverse_sum(ps)[1]
            for j in range(3):
                lbuf[0, j] = _gather_rows(inv, tab[5 + j])

            def swizzle(a, carry):
                for g in range(2, 8):
                    ref = kbuf.at[i, a // 3, 8 * (a % 3) + g]
                    v = ref[...].reshape(4, 4, 8, 128)
                    v = jnp.concatenate(
                        [v[:, c ^ (g // 2):(c ^ (g // 2)) + 1] for c in range(4)],
                        axis=1)
                    ref[...] = v.reshape(128, 128)
                return carry

            lax.fori_loop(0, NG // 8, swizzle, 0)

            for cp in ((vlast_copy,) if last else v_copies(i)):
                cp.wait()
            for par in range(2):
                pv = jnp.concatenate(
                    [_gather_rows(ps[c // 2], tab[2 * (c % 2) + par])
                     for c in range(ncp)], axis=0)

                def group(g, w):
                    for a, half in enumerate(_unpack(w)):
                        acc = (_as_f32(half) * pv).reshape(ncp, 8, 128)
                        abuf[0, g, pl.ds(a, 8, stride=2), :] = jnp.sum(acc, axis=0)

                def packed_group(gl, carry):
                    group(GH * par + gl, vbuf[i, par, gl])
                    return carry

                def wide_group(gl, carry):
                    ref = (vlast.at[:, par, gl] if last
                           else vwide.at[i, :, par, gl - (GH - NW)])
                    w = ref[1]
                    keep = slice(0, 8 * (ncp - NT) if last else 8 * ncp)
                    ref[0, keep, :], ref[1, keep, :] = _unpack(w[keep])
                    group(GH * par + gl, w)
                    return carry

                split = 0 if last else GH - NW
                if split:
                    lax.fori_loop(0, split, packed_group, 0)
                lax.fori_loop(split, GH, wide_group, 0)
            ts = []
            _run(r_stage(0, ts), o_stage(i, ts))

        def transpose_last():
            for c in range(ncp - NT, ncp):
                v = _as_bf16(vlast[1, :, :, 8 * c:8 * c + 8, :].reshape(
                    8 * NG, 128)).astype(f32).reshape(NG, 16, 128)
                for s in range(2):
                    for j in range(3):
                        t = v[16 * j:16 * j + 16, 8 * s:8 * s + 8].reshape(128, 128)
                        t = pltpu.bitcast(t.T.astype(bf16), u32)
                        for n in range(8):
                            vlast[vt_slot(2 * c + s, j, n)] = t[8 * n:8 * n + 8]

        def streamed_attention(x):
            start_attention(x)

            def body(i, carry):
                streamed_pair(i, i, None)
                return carry

            lax.fori_loop(0, NP - 1, body, 0)
            streamed_pair(NP - 1, NP // 2 - 1, 1)
            transpose_last()
            return obuf[...]

        def ffn(first, x):
            if first:
                w1_copy.wait()
                w3_copy.wait()
            m, _, r = _ln_stats(x)
            xo = _with_ones(x)
            hids = []
            for n in range(0, FF, FCH):
                gate = _round_bf16(_centered_dot(xo, w1[:, n:n + FCH], m) * r)
                up = _round_bf16(_centered_dot(xo, w3[:, n:n + FCH], m) * r)
                hids.append(
                    (_round_bf16(gate * jax.nn.sigmoid(gate)) * up).astype(bf16))
            y = None
            starts = [a for a, _ in W2_SPLITS]
            for n, hid in enumerate(hids):
                if first and n in starts:
                    if y is not None:
                        obuf[...] = y
                    w2_copies[starts.index(n)].wait()
                    if y is not None:
                        y = obuf[...]
                t = _dot(hid, w2[n])
                y = t if y is None else y + t
            return y

        x_copy.wait()
        x = jnp.broadcast_to(xbuf[0].astype(f32), (8, D))
        x = _round_bf16(x + _round_bf16(streamed_attention(x)))
        x = _round_bf16(x + _round_bf16(ffn(True, x)))
        x = _round_bf16(x + _round_bf16(attention(x)))
        x = _round_bf16(x + _round_bf16(ffn(False, x)))
        o_ref[0] = x[0:1].astype(bf16)

    return kernel


def _tiles(a, lead):
    r, c = a.shape
    t = a.reshape(r // 8, 8, c // 128, 128).transpose(0, 2, 1, 3)
    return t.reshape(lead + (-1, 128))


@jax.jit
def pallas_interleave_layers__sliding_block_cached__glu_gated_swiglu__decode_kernel(
    A_x: jax.Array,
    A_k_cache: jax.Array,
    A_v_cache: jax.Array,
    A_wq: jax.Array,
    A_wo: jax.Array,
    B_x: jax.Array,
    B_w1: jax.Array,
    B_w3: jax.Array,
    B_w2: jax.Array,
):
    del B_x
    sk = A_k_cache.shape[2]
    win = min(4096, max(256, sk // 4))
    wr = win // 32
    kt = _tiles(jnp.swapaxes(A_k_cache, 2, 3).reshape(H * DH, sk), (NP, 2, GH))
    vt = _tiles(jnp.swapaxes(A_v_cache, 2, 3).reshape(H * DH, sk), (NP, 2, GH))
    any_spec = pl.BlockSpec(memory_space=pl.ANY)
    return pl.pallas_call(
        _make_kernel(sk, win),
        out_shape=jax.ShapeDtypeStruct((1, 1, D), bf16),
        in_specs=[any_spec] * 8,
        out_specs=pl.BlockSpec(memory_space=pltpu.VMEM),
        scratch_shapes=[
            pltpu.VMEM((1, 1, D), bf16),
            pltpu.VMEM((NP, 2, GH, wr, 128), u32),
            pltpu.VMEM((NP - 1, 2, GH - NW, wr, 128), u32),
            pltpu.VMEM((NP - 1, 2, 2, NW, wr, 128), u32),
            pltpu.VMEM((2, 2, GH, wr, 128), u32),
            pltpu.VMEM((D // 32, H * DH // 8, 128), u32),
            pltpu.VMEM((H * DH // 16, D // 16, 128), u32),
            pltpu.VMEM((D, FF), bf16),
            pltpu.VMEM((D, FF), bf16),
            pltpu.VMEM((FF // FCH, FCH, D), bf16),
            pltpu.VMEM((8, D), u32),
            pltpu.VMEM((12, 8, 128), u32),
            pltpu.VMEM((3, 8, 128), u32),
            pltpu.VMEM((2, 8, 8, 128), f32),
            pltpu.VMEM((2, 3, 8, 128), f32),
            pltpu.VMEM((2, NG, 16, 128), f32),
            pltpu.VMEM((8, D), f32),
            pltpu.VMEM((8, 128), u32),
            pltpu.VMEM((8, 128), f32),
            pltpu.VMEM((16, 8, 128), jnp.int32),
            pltpu.SemaphoreType.DMA((NP,)),
            pltpu.SemaphoreType.DMA((2 * NP - 2,)),
            pltpu.SemaphoreType.DMA((8,)),
        ],
        compiler_params=pltpu.CompilerParams(
            vmem_limit_bytes=128 * 1024 * 1024,
            disable_semaphore_checks=True),
    )(A_x, kt, vt, _tiles(A_wq, (D // 32,)), _tiles(A_wo, (H * DH // 16,)),
      B_w1, B_w3, B_w2.reshape(FF // FCH, FCH, D))
```

```python
import jax
import jax.numpy as jnp
import numpy as np
from jax import lax
import jax.experimental.pallas as pl
import jax.experimental.pallas.tpu as pltpu

D = 640
H = 32
NP = H // 2
DH = 192
GH = DH // 8
NG = 2 * GH
FF = 1536
FCH = 256
EPS = 1e-5

NT = 7
NW = 4
W2_SPLITS = ((0, 5), (5, 6))

T_GROUP = 24.1
T_LAST = 12.0
T_FIRST = 740
EDGE_PACE = (0.69, 6, (40, 200))
LOOP_PACE = (0.65, 8, (60, 240))
LOOP_MXU = (155, 0.985)

f32 = jnp.float32
bf16 = jnp.bfloat16
u32 = jnp.uint32


def _round_bf16(x):
    return x.astype(bf16).astype(f32)


def _as_bf16(x):
    return pltpu.bitcast(x, bf16)


def _as_f32(x):
    return pltpu.bitcast(x, f32)


def _dot(a, b):
    return jnp.dot(a, b, preferred_element_type=f32)


def _gather_rows(x, idx):
    dnums = lax.GatherDimensionNumbers(
        offset_dims=(), collapsed_slice_dims=(0,), start_index_map=(0,),
        operand_batching_dims=(1,), start_indices_batching_dims=(1,))
    return lax.gather(x, idx.reshape(8, 128, 1), dnums, slice_sizes=(1, 1),
                      mode=lax.GatherScatterMode.FILL_OR_DROP)


def _ln_stats(x):
    m = jnp.mean(x, axis=-1, keepdims=True)
    c = x - m
    v = jnp.mean(c * c, axis=-1, keepdims=True)
    return m, c, lax.rsqrt(v + EPS)


def _with_ones(x):
    return jnp.concatenate([x, jnp.ones_like(x)], axis=0).astype(bf16)


def _centered_dot(xo, w, m):
    y = _dot(xo, w)
    return y[0:8] - m * y[8:16]


def _packed(t):
    return _as_f32(jnp.concatenate([t, t], axis=0).astype(bf16))


def _unpack(w):
    return w << 16, w & jnp.uint32(0xFFFF0000)


def _run(*gens):
    for g in gens:
        for _ in g:
            pass


def _take(gen, n):
    for _ in range(n):
        yield next(gen)


def _group_order():
    order = []
    step = GH // NW
    for par in range(2):
        packed = list(range(GH * par, GH * par + GH - NW))
        wide = list(range(GH * par + GH - NW, GH * par + GH))
        order += [(wide if n % step == step // 2 else packed).pop(0)
                  for n in range(GH)]
    return order


def _make_kernel(sk, win):
    nc = win // 128
    ncp = nc // 2
    row0 = (sk - win) // 128 * 4
    assert nc == 32
    scale = float(np.asarray(DH ** -0.5, dtype=bf16)) * float(np.log2(np.e))
    order = _group_order()

    def kernel(x_hbm, k_hbm, v_hbm, wq_hbm, wo_hbm, w1_hbm, w3_hbm, w2_hbm,
               o_ref,
               xbuf, kbuf, vbuf, vwide, vlast, vlast_lo, wq, wo, w1, w3, w2,
               zq, ybuf, qbuf, pbuf, lbuf, abuf, obuf, zeros, ones, tab,
               ksem, vsem, wsem):
        k32 = k_hbm.bitcast(u32)
        v32 = v_hbm.bitcast(u32)
        window = pl.ds(row0, 4 * nc)

        def k_copy(i):
            return pltpu.make_async_copy(
                k32.at[i, :, :, window, :], kbuf.at[i], ksem.at[i])

        def v_copies(i):
            return (
                pltpu.make_async_copy(
                    v32.at[i, :, pl.ds(0, GH - NW), window, :], vbuf.at[i],
                    vsem.at[2 * i]),
                pltpu.make_async_copy(
                    v32.at[i, :, pl.ds(GH - NW, NW), window, :],
                    vwide.at[i, 1], vsem.at[2 * i + 1]))

        x_copy = pltpu.make_async_copy(x_hbm, xbuf, wsem.at[0])
        wq_copy = pltpu.make_async_copy(wq_hbm.bitcast(u32), wq, wsem.at[1])
        wo_copy = pltpu.make_async_copy(wo_hbm.bitcast(u32), wo, wsem.at[2])
        vlast_copy = pltpu.make_async_copy(
            v32.at[NP - 1, :, :, window, :], vlast, wsem.at[3])
        w1_copy = pltpu.make_async_copy(w1_hbm, w1, wsem.at[4])
        w3_copy = pltpu.make_async_copy(w3_hbm, w3, wsem.at[5])
        w2_copies = [
            pltpu.make_async_copy(w2_hbm.at[pl.ds(a, b - a)],
                                  w2.at[pl.ds(a, b - a)], wsem.at[6 + n])
            for n, (a, b) in enumerate(W2_SPLITS)]

        wq_copy.start()
        x_copy.start()
        wo_copy.start()
        k_copy(0).start()

        def start_kv(i, carry):
            for cp in v_copies(i):
                cp.start()
            k_copy(i + 1).start()
            return carry

        lax.fori_loop(0, NP - 1, start_kv, 0)
        vlast_copy.start()

        lane = lax.broadcasted_iota(jnp.int32, (8, 128), 1)
        sub = lax.broadcasted_iota(jnp.int32, (8, 128), 0)
        zeros[...] = jnp.zeros((8, 128), u32)
        ones[...] = jnp.ones((8, 128), f32)
        for n in range(4):
            tab[n] = 2 * n + (sub >> 2)
        tab[4] = sub ^ 1
        tab[5] = jnp.zeros_like(sub)
        tab[6] = jnp.where(lane < 64, 0, 2)
        tab[7] = jnp.full_like(sub, 2)
        tab[8] = lane & 8
        tab[9] = sub
        tab[10] = sub - jnp.where(lane < 64, 0, 1)
        tab[11] = sub - 1
        for n in range(4):
            tab[12 + n] = jnp.where((sub >> 1) == n // 2,
                                    -65536 if n % 2 else 65535, 0)

        def retile(ref, ntile, place):
            top = sub < 4
            nrep = ref.shape[1] // (8 * ntile)

            def body(a, carry):
                v = [ref[a, 8 * n:8 * n + 8, :] for n in range(nrep * ntile)]
                for k in range(nrep):
                    for t in range(ntile):
                        lo = v[k * ntile + t // 2]
                        hi = v[k * ntile + (ntile + t) // 2]
                        if t % 2:
                            lo = pltpu.roll(lo, 4, 0)
                        if (ntile + t) % 2 == 0:
                            hi = pltpu.roll(hi, 4, 0)
                        r = 8 * place(k, t)
                        ref[a, r:r + 8, :] = jnp.where(top, lo, hi)
                return carry

            lax.fori_loop(0, ref.shape[0], body, 0)

        def k_rows(g, c):
            r = 8 * (c ^ (g // 2 % 4))
            return slice(r, r + 8)

        wq_copy.wait()
        retile(wq, H * DH // 128, lambda k, t: 2 * t + k)
        w1_copy.start()
        w3_copy.start()
        wo_copy.wait()
        retile(wo, D // 128, lambda k, t: t)
        for cp in w2_copies:
            cp.start()

        def expand_q(t, b):
            even = tab[8] == 0
            return [jnp.where(tab[9 + t] == 2 * var, y, jnp.uint32(0))
                    for y in (jnp.where(even, b >> 16, pltpu.roll(b, 8, 1)),
                              jnp.where(even, pltpu.roll(b, 120, 1) >> 16, b))
                    for var in range(2)]

        def q_stage(u, e, out, proj=None, expand=True):
            if e is None:
                wref, e = wq.at[:, pl.ds(pl.multiple_of(48 * u, 16), 48), :], 0
            elif isinstance(u, int):
                wref = wq.at[:, pl.ds(96 * u, 96), :]
            else:
                wref = wq.at[:, pl.ds(pl.multiple_of(96 * u, 32), 96), :]
            for t in range(3):
                r = 48 * e + 16 * t
                w = _as_bf16(wref[:, r:r + 16, :].reshape(D // 2, 128))
                q = proj(w) if proj else _dot(_as_bf16(zq[...]), w)[0:8]
                b = pltpu.bitcast(_round_bf16(q), u32)
                out.extend(expand_q(t, b) if expand else [b])
                yield 40, [(_as_f32(b), 7)]

        def fold_rows(x, op):
            x = op(x, pltpu.roll(x, 4, 0))
            return op(x, _gather_rows(x, tab[4]))

        def k_stage(i, ys, out):
            kref = kbuf.at[i]
            m = None
            for c in range(ncp):
                lhs = jnp.concatenate(
                    [ys(2 * n + c % 2) for n in range(6)], axis=1)
                w = jnp.concatenate(
                    [kref[g // GH, g % GH, k_rows(g, c), :]
                     for t in range(3) for e in range(2)
                     for g in range(16 * t + e, 16 * t + 16, 2)], axis=0)
                s = _dot(_as_bf16(lhs), _as_bf16(w))[0:8]
                if c % 2 == 0:
                    out.append(s)
                    yield 48, [(s, 6)]
                else:
                    out[-1] = out[-1] + s
                    m = out[-1] if m is None else jnp.maximum(m, out[-1])
                    if c == ncp - 1:
                        m = fold_rows(m, jnp.maximum)
                    yield 48, [(m, 12 if c == ncp - 1 else 8)]
            out.append(m)

        def k_first(qb, out_a, out):
            even, low = tab[8] == 0, tab[6] == 0
            b = qb[1]
            rot = {n: pltpu.roll(b, n, 1) for n in (8, 56, 64, 72, 120)}
            mix = (jnp.where(even, jnp.where(low, b, rot[56]) >> 16,
                             jnp.where(low, rot[8], rot[64])),
                   jnp.where(even, jnp.where(low, rot[64], rot[120]) >> 16,
                             jnp.where(low, rot[72], b)))
            tiles = []
            for par in range(2):
                ys = expand_q(2 * par, qb[2 * par])
                for e in range(2):
                    tiles.append((ys[2 * e:2 * e + 2],
                                  range(32 * par + e, 32 * par + 16, 2)))
                g0 = 16 + 8 * par
                tiles.append((
                    [jnp.where(tab[9 + 2 * par] == 2 * var, mix[par],
                               jnp.uint32(0)) for var in range(2)],
                    [*range(g0, g0 + 8, 2), *range(g0 + 1, g0 + 8, 2)]))

            def part(c, sel):
                lhs = jnp.concatenate([tiles[n][0][c % 2] for n in sel], axis=1)
                w = jnp.concatenate(
                    [kbuf[0, g // GH, g % GH, k_rows(g, c), :]
                     for n in sel for g in tiles[n][1]], axis=0)
                return _dot(_as_bf16(lhs), _as_bf16(w))[0:8]

            plan = [(c, (0, 1)) for c in range(4)] + [(c, (2,)) for c in range(4)]
            plan += [(c, (0, 1, 2)) for c in range(4, ncp)]
            acc = [None] * (ncp // 2)
            for c, sel in plan:
                s = part(c, sel)
                acc[c // 2] = s if acc[c // 2] is None else acc[c // 2] + s
                yield 8 * len(sel), []
            m = acc[0]
            for a in acc[1:]:
                m = jnp.maximum(m, a)
            out_a.extend(acc + [fold_rows(m, jnp.maximum)])
            m = None
            for j in range(ncp // 2):
                s = acc[j] + part(2 * j, (3, 4, 5)) + part(2 * j + 1, (3, 4, 5))
                out.append(s)
                m = s if m is None else jnp.maximum(m, s)
                if j == ncp // 2 - 1:
                    m = fold_rows(m, jnp.maximum)
                yield 48, [(m, 8)]
            out.append(m)

        def softmax_numerator(ss, sc=scale):
            m = jnp.max(ss[-1], axis=1, keepdims=True)
            return [jnp.exp2((s - m) * sc) for s in ss[:-1]]

        def inverse_sum(ps):
            tot = ps[0]
            for p in ps[1:]:
                tot = tot + p
            lf = fold_rows(tot, jnp.add)
            l = jnp.sum(lf, axis=1, keepdims=True)
            l = jnp.broadcast_to(l, (8, 128))
            y = pl.reciprocal(l, approx=True)
            return lf, y * (2.0 - l * y)

        def lane_sums(b, j):
            a = jnp.concatenate(
                [abuf[b, 16 * j:16 * j + 16, 8 * s:8 * s + 8, :].reshape(128, 128)
                 for s in range(2)], axis=1)
            return lax.dot_general(
                jnp.concatenate([ones[...]] * 2, axis=1), a,
                (((1,), (1,)), ((), ())), preferred_element_type=f32)

        def r_stage(b, out):
            for j in range(3):
                out.append(_packed(lane_sums(b, j) * lbuf[b, j]))
                yield 32, [(out[-1], 4)]

        def o_stage(i, ts):
            wref = wo.at[pl.ds(24 * i, 24)]
            t = _as_bf16(jnp.concatenate(ts, axis=1))
            for n in range(D // 128):
                cols = slice(128 * n, 128 * n + 128)
                w = wref[:, 8 * n:8 * n + 8, :].reshape(DH, 128)
                y = obuf[:, cols] + _dot(t, _as_bf16(w))[0:8]
                obuf[:, cols] = y
                yield 24, [(y, 4)]

        def o_tile(i, j, t):
            r0 = 24 * i + 8 * j
            w = jnp.concatenate(
                [wo[r0:r0 + 8, 8 * n:8 * n + 8, :].reshape(64, 128)
                 for n in range(D // 128)], axis=1)
            return _dot(_as_bf16(t), _as_bf16(w))[0:8]

        def trace_mxu(gens, links, latency, t=0.0, rate=1.0):
            for gen in gens:
                for cost, res in gen:
                    t += cost / rate
                    links.setdefault(t + latency, []).extend(res)
            return t

        def v_stage(i, b, getp, links, clock, hist, pace):
            never = zeros[...] != 0
            last = i is None
            for n, g in enumerate(range(NG) if last else order):
                par, gl = divmod(g, GH)
                if n % GH == 0:
                    ps = [getp(par, j) for j in range(nc // 4)]
                    idx = [tab[par], tab[2 + par]]
                    if len(hist) > 1 and getp is not from_pbuf:
                        dep = pltpu.bitcast(hist[-2][0], jnp.int32)
                        idx = [jnp.where(never, dep, ix) for ix in idx]
                    pv = [_gather_rows(ps[c // 2], idx[c % 2])
                          for c in range(ncp - NT if last else ncp)]
                    clock[0] += 4
                    if par == 1 and not last:
                        lf, inv = inverse_sum(ps)
                        for val, at in zip((lf, inv), pace[2]):
                            links.setdefault(clock[0] + at, []).append((val, 14))
                        for j in range(3):
                            lbuf[b, j] = _gather_rows(inv, tab[5 + j])
                wide = last or gl >= GH - NW
                if last:
                    refs = vlast_lo.at[par, gl], vlast.at[par, gl]
                elif wide:
                    ref = vwide.at[i, :, par, gl - (GH - NW)]
                    refs = ref.at[0], ref.at[1]
                else:
                    ref = vbuf.at[i, par, gl]
                dur = T_LAST if last else T_GROUP * (pace[0] if wide else 1.0)
                accs = [None, None]
                held = [None, None]
                pending = []
                nsteps = ncp - NT if last else ncp
                for c in range(nsteps):
                    for key in sorted(links):
                        if key < clock[0] + dur * (c + 1) / nsteps:
                            for val, ops in links.pop(key):
                                pending.append(val)
                                clock[0] += ops / 4
                    rs = slice(8 * c, 8 * c + 8)
                    if wide:
                        lo, hi = refs[0][rs, :], refs[1][rs, :]
                    else:
                        lo, hi = _unpack(ref[rs, :])
                    p = pv[c]
                    if c == (8 if last else pace[1] if wide else 0) and hist:
                        p = jnp.where(never, hist[-1][0] + hist[-1][1], p)
                    for a, t in enumerate((_as_f32(lo) * p, _as_f32(hi) * p)):
                        if accs[a] is None:
                            accs[a] = t
                            continue
                        if pending:
                            t = jnp.where(never, pending.pop(), t)
                        if c % 2 == 1 and c < nsteps - 1:
                            held[a] = t
                        else:
                            if held[a] is not None:
                                t = held[a] + t
                                held[a] = None
                            accs[a] = accs[a] + t
                for a in range(2):
                    abuf[b, g, pl.ds(a, 8, stride=2), :] = accs[a]
                clock[0] += dur
                hist.append(accs)
                yield g

        def from_pbuf(par, j):
            return pbuf[par, j]

        def values(ps):
            return lambda par, j: ps[j]

        def store_state(ya, qb, ps):
            for n in range(12):
                ybuf[n] = ya[n]
            for n in range(3):
                qbuf[n] = qb[n]
            for j, p in enumerate(ps):
                pbuf[0, j] = p
                pbuf[1, j] = p

        def four_pairs(u0):
            links, clock, hist = {}, [10], []
            getq, getp = (lambda n: qbuf[n]), from_pbuf
            s1 = []
            k1 = k_stage(2 * u0 + 1, lambda n: ybuf[n], s1)
            t = 0.0

            def mxu(gens, t):
                return trace_mxu(gens, links, LOOP_MXU[0], t, LOOP_MXU[1])

            for half in range(2):
                u = u0 + half
                i = 2 * u
                s2, ya, qb, t0, t1 = [], [], [], [], []
                y2 = [y for n in range(3) for y in expand_q(n, getq(n))]
                k2 = k_stage(i + 2, y2.__getitem__, s2)
                t = mxu([k1], t)
                p1 = softmax_numerator(s1)
                t = mxu([r_stage(1, t1), q_stage(u + 1, 1, ya),
                         o_stage(i - 1, t1), _take(k2, 4 + 4 * half)], t)
                _run(v_stage(i, 0, getp, links, clock, hist, LOOP_PACE))
                t = mxu([r_stage(0, t0), k2], max(t, clock[0] - 64))
                p2 = softmax_numerator(s2)
                t = mxu([o_stage(i, t0),
                         q_stage(jnp.minimum(u + 2, NP // 2 - 1), 0, qb,
                                 expand=False)], t)
                if half == 0:
                    s1 = []
                    k1 = k_stage(i + 3, ya.__getitem__, s1)
                    t = mxu([_take(k1, 3)], t)
                _run(v_stage(i + 1, 1, values(p1), links, clock, hist,
                             LOOP_PACE))
                getq, getp = qb.__getitem__, values(p2)
            store_state(ya, qb, p2)

        def first_pairs(xo, m, r):
            links, clock, hist = {}, [T_FIRST], []
            q0, y1, y2, sa, s0, s1, s2, ya, qb, t0 = ([] for _ in range(10))
            _run(q_stage(0, 0, q0, lambda w: _centered_dot(xo, w, m), False),
                 q_stage(0, 1, y1, lambda w: _centered_dot(xo, w, m) * r))
            t = trace_mxu([k_first(q0, sa, s0),
                           k_stage(1, lambda n: y1[n], s1),
                           q_stage(1, 0, y2), q_stage(1, 1, ya),
                           q_stage(2, 0, qb, expand=False)], links, 190)
            for key in [key for key in links if key < T_FIRST + 30]:
                del links[key]
            pa = softmax_numerator(sa, r * scale)
            p0 = softmax_numerator(s0, r * scale)
            p1 = softmax_numerator(s1)
            _run(v_stage(0, 0, lambda par, j: (pa, p0)[par][j], links,
                         clock, hist, EDGE_PACE))
            trace_mxu([r_stage(0, t0), k_stage(2, lambda n: y2[n], s2),
                       o_stage(0, t0)], links, 190,
                      max(t, clock[0] - 64))
            p2 = softmax_numerator(s2)
            _run(v_stage(1, 1, values(p1), links, clock,
                         hist, EDGE_PACE))
            store_state(ya, qb, p2)

        def vt_slot(kc, j, n):
            g = 24 * (kc % 2) + 8 * j + n
            r = 8 * (kc // 2)
            return (g // GH, g % GH, slice(r, r + 8), slice(None))

        def last_pairs():
            i = NP - 2
            links, clock, hist = {}, [20], []
            s1, t0, t1, ts, part, rows = ([] for _ in range(6))
            tk = trace_mxu([k_stage(i + 1, lambda n: ybuf[n], s1)], links, 185)
            t = trace_mxu([r_stage(1, t1)], links, 185, tk)
            t = trace_mxu([o_stage(i - 1, t1)], links, 185, t + 60)
            ps = softmax_numerator(s1)
            chunks = range(nc - 2 * NT, nc)
            for kc in chunks:
                bits = pltpu.bitcast(_packed(ps[kc // 4]), u32)
                rows.append(bits & pltpu.bitcast(tab[12 + kc % 4], u32))
                links.setdefault(tk + 315, []).append((_as_f32(rows[-1]), 3))
            lhs = _as_bf16(jnp.concatenate(rows, axis=1))

            def p_stage():
                for j in range(3):
                    w = jnp.concatenate([vlast[vt_slot(kc, j, n)]
                                         for kc in chunks for n in range(8)],
                                        axis=0)
                    y = fold_rows(_dot(lhs, _as_bf16(w))[0:8], jnp.add)
                    part.append(_gather_rows(y, tab[5 + j]))
                    yield 16 * NT, [(part[j], 2 * NT + 5)]

            pg = p_stage()
            t = trace_mxu([_take(pg, 1)], links, 210, max(t, tk + 266))
            _run(v_stage(i, 0, from_pbuf, links, clock, hist,
                         EDGE_PACE[:2] + ((),)))
            trace_mxu([r_stage(0, t0), _take(pg, 1), o_stage(i, t0), pg],
                      links, 210, max(t, clock[0] + 56))
            lf, inv = inverse_sum(ps)
            links.setdefault(clock[0] + 20, []).append((lf, 10))
            links.setdefault(clock[0] + 160, []).append((inv, 10))
            for g in v_stage(None, 1, values(ps), links, clock, hist,
                             EDGE_PACE):
                if g % 16 == 15:
                    j = g // 16
                    ts.append(_packed((lane_sums(1, j) + part[j])
                                      * _gather_rows(inv, tab[5 + j])))
            y = obuf[...]
            for j in range(3):
                y = y + o_tile(NP - 1, j, ts[j])
            return y

        def start_attention(x):
            m, c, r = _ln_stats(x)
            z = c * r
            zq[...] = pltpu.bitcast(
                jnp.concatenate([z, z], axis=0).astype(bf16), u32)
            obuf[...] = jnp.zeros(obuf.shape, f32)
            return m, r

        def attention(x):
            m, r = start_attention(x)
            first_pairs(_with_ones(x), m, r)

            def body(it, carry):
                four_pairs(1 + 2 * it)
                return carry

            lax.fori_loop(0, (NP - 4) // 4, body, 0)
            return last_pairs()

        def streamed_pair(i, u, e):
            last = isinstance(i, int)
            ys = []
            _run(q_stage(u, e, ys))
            lhs = [_as_bf16(jnp.concatenate(ys[var::2], axis=1))
                   for var in range(2)]
            k_copy(i).wait()
            ss = []
            for c in range(ncp):
                k = kbuf[i, :, :, 8 * c:8 * c + 8, :].reshape(3, 8, 2, 8, 128)
                w = jnp.concatenate(
                    [k[t, :, par].reshape(64, 128)
                     for t in range(3) for par in range(2)], axis=0)
                s = _dot(lhs[c % 2], _as_bf16(w))[0:8]
                if c % 2:
                    s = ss.pop() + s
                ss.append(s)
            m = ss[0]
            for s in ss[1:]:
                m = jnp.maximum(m, s)
            ps = softmax_numerator(ss + [fold_rows(m, jnp.maximum)])
            inv = inverse_sum(ps)[1]
            for j in range(3):
                lbuf[0, j] = _gather_rows(inv, tab[5 + j])

            def swizzle(a, carry):
                for g in range(2, 8):
                    ref = kbuf.at[i, a // 3, 8 * (a % 3) + g]
                    v = ref[...].reshape(4, 4, 8, 128)
                    v = jnp.concatenate(
                        [v[:, c ^ (g // 2):(c ^ (g // 2)) + 1] for c in range(4)],
                        axis=1)
                    ref[...] = v.reshape(128, 128)
                return carry

            lax.fori_loop(0, NG // 8, swizzle, 0)

            for cp in ((vlast_copy,) if last else v_copies(i)):
                cp.wait()
            for par in range(2):
                pv = jnp.concatenate(
                    [_gather_rows(ps[c // 2], tab[2 * (c % 2) + par])
                     for c in range(ncp)], axis=0)

                def group(g, w):
                    for a, half in enumerate(_unpack(w)):
                        acc = (_as_f32(half) * pv).reshape(ncp, 8, 128)
                        abuf[0, g, pl.ds(a, 8, stride=2), :] = jnp.sum(acc, axis=0)

                def packed_group(gl, carry):
                    group(GH * par + gl, vbuf[i, par, gl])
                    return carry

                def wide_group(gl, carry):
                    if last:
                        w = vlast[par, gl]
                        keep = slice(0, 8 * (ncp - NT))
                        vlast_lo[par, gl], vlast[par, gl, keep, :] = _unpack(w[keep])
                    else:
                        ref = vwide.at[i, :, par, gl - (GH - NW)]
                        w = ref[1]
                        ref[0], ref[1] = _unpack(w)
                    group(GH * par + gl, w)
                    return carry

                split = 0 if last else GH - NW
                if split:
                    lax.fori_loop(0, split, packed_group, 0)
                lax.fori_loop(split, GH, wide_group, 0)
            ts = []
            _run(r_stage(0, ts), o_stage(i, ts))

        def transpose_last():
            for c in range(ncp - NT, ncp):
                v = _as_bf16(vlast[:, :, 8 * c:8 * c + 8, :].reshape(
                    8 * NG, 128)).astype(f32).reshape(NG, 16, 128)
                for s in range(2):
                    for j in range(3):
                        t = v[16 * j:16 * j + 16, 8 * s:8 * s + 8].reshape(128, 128)
                        t = pltpu.bitcast(t.T.astype(bf16), u32)
                        for n in range(8):
                            vlast[vt_slot(2 * c + s, j, n)] = t[8 * n:8 * n + 8]

        def streamed_attention(x):
            start_attention(x)

            def body(i, carry):
                streamed_pair(i, i, None)
                return carry

            lax.fori_loop(0, NP - 1, body, 0)
            streamed_pair(NP - 1, NP // 2 - 1, 1)
            transpose_last()
            return obuf[...]

        def ffn(first, x):
            if first:
                w1_copy.wait()
                w3_copy.wait()
            m, _, r = _ln_stats(x)
            xo = _with_ones(x)
            hids = []
            for n in range(0, FF, FCH):
                gate = _round_bf16(_centered_dot(xo, w1[:, n:n + FCH], m) * r)
                up = _round_bf16(_centered_dot(xo, w3[:, n:n + FCH], m) * r)
                hids.append(
                    (_round_bf16(gate * jax.nn.sigmoid(gate)) * up).astype(bf16))
            y = None
            starts = [a for a, _ in W2_SPLITS]
            for n, hid in enumerate(hids):
                if first and n in starts:
                    if y is not None:
                        obuf[...] = y
                    w2_copies[starts.index(n)].wait()
                    if y is not None:
                        y = obuf[...]
                t = _dot(hid, w2[n])
                y = t if y is None else y + t
            return y

        x_copy.wait()
        x = jnp.broadcast_to(xbuf[0].astype(f32), (8, D))
        x = _round_bf16(x + _round_bf16(streamed_attention(x)))
        x = _round_bf16(x + _round_bf16(ffn(True, x)))
        x = _round_bf16(x + _round_bf16(attention(x)))
        x = _round_bf16(x + _round_bf16(ffn(False, x)))
        o_ref[0] = x[0:1].astype(bf16)

    return kernel


def _tiles(a, lead):
    r, c = a.shape
    t = a.reshape(r // 8, 8, c // 128, 128).transpose(0, 2, 1, 3)
    return t.reshape(lead + (-1, 128))


@jax.jit
def pallas_interleave_layers__sliding_block_cached__glu_gated_swiglu__decode_kernel(
    A_x: jax.Array,
    A_k_cache: jax.Array,
    A_v_cache: jax.Array,
    A_wq: jax.Array,
    A_wo: jax.Array,
    B_x: jax.Array,
    B_w1: jax.Array,
    B_w3: jax.Array,
    B_w2: jax.Array,
):
    del B_x
    sk = A_k_cache.shape[2]
    win = min(4096, max(256, sk // 4))
    wr = win // 32
    kt = _tiles(jnp.swapaxes(A_k_cache, 2, 3).reshape(H * DH, sk), (NP, 2, GH))
    vt = _tiles(jnp.swapaxes(A_v_cache, 2, 3).reshape(H * DH, sk), (NP, 2, GH))
    any_spec = pl.BlockSpec(memory_space=pl.ANY)
    return pl.pallas_call(
        _make_kernel(sk, win),
        out_shape=jax.ShapeDtypeStruct((1, 1, D), bf16),
        in_specs=[any_spec] * 8,
        out_specs=pl.BlockSpec(memory_space=pltpu.VMEM),
        scratch_shapes=[
            pltpu.VMEM((1, 1, D), bf16),
            pltpu.VMEM((NP, 2, GH, wr, 128), u32),
            pltpu.VMEM((NP - 1, 2, GH - NW, wr, 128), u32),
            pltpu.VMEM((NP - 1, 2, 2, NW, wr, 128), u32),
            pltpu.VMEM((2, GH, wr, 128), u32),
            pltpu.VMEM((2, GH, wr - 8 * NT, 128), u32),
            pltpu.VMEM((D // 32, H * DH // 8, 128), u32),
            pltpu.VMEM((H * DH // 16, D // 16, 128), u32),
            pltpu.VMEM((D, FF), bf16),
            pltpu.VMEM((D, FF), bf16),
            pltpu.VMEM((FF // FCH, FCH, D), bf16),
            pltpu.VMEM((8, D), u32),
            pltpu.VMEM((12, 8, 128), u32),
            pltpu.VMEM((3, 8, 128), u32),
            pltpu.VMEM((2, 8, 8, 128), f32),
            pltpu.VMEM((2, 3, 8, 128), f32),
            pltpu.VMEM((2, NG, 16, 128), f32),
            pltpu.VMEM((8, D), f32),
            pltpu.VMEM((8, 128), u32),
            pltpu.VMEM((8, 128), f32),
            pltpu.VMEM((16, 8, 128), jnp.int32),
            pltpu.SemaphoreType.DMA((NP,)),
            pltpu.SemaphoreType.DMA((2 * NP - 2,)),
            pltpu.SemaphoreType.DMA((8,)),
        ],
        compiler_params=pltpu.CompilerParams(
            vmem_limit_bytes=128 * 1024 * 1024,
            disable_semaphore_checks=True),
    )(A_x, kt, vt, _tiles(A_wq, (D // 32,)), _tiles(A_wo, (H * DH // 16,)),
      B_w1, B_w3, B_w2.reshape(FF // FCH, FCH, D))
```

```python
import jax
import jax.numpy as jnp
import numpy as np
from jax import lax
import jax.experimental.pallas as pl
import jax.experimental.pallas.tpu as pltpu

D = 640
H = 32
NP = H // 2
DH = 192
GH = DH // 8
NG = 2 * GH
FF = 1536
FCH = 128
EPS = 1e-5

NT = 7
NKV = 6
NFV = 6
NW = 4
W2_SPLITS = ((0, 10), (10, 12))

T_GROUP = 24.1
T_LAST = 12.0
T_FIRST = 620
EDGE_PACE = (0.69, 6, (40, 200))
LOOP_PACE = (0.65, 8, (60, 240))
LOOP_MXU = (155, 0.985)

f32 = jnp.float32
bf16 = jnp.bfloat16
u32 = jnp.uint32


def _round_bf16(x):
    return x.astype(bf16).astype(f32)


def _as_bf16(x):
    return pltpu.bitcast(x, bf16)


def _as_f32(x):
    return pltpu.bitcast(x, f32)


def _dot(a, b):
    return jnp.dot(a, b, preferred_element_type=f32)


def _gather_rows(x, idx):
    dnums = lax.GatherDimensionNumbers(
        offset_dims=(), collapsed_slice_dims=(0,), start_index_map=(0,),
        operand_batching_dims=(1,), start_indices_batching_dims=(1,))
    return lax.gather(x, idx.reshape(8, 128, 1), dnums, slice_sizes=(1, 1),
                      mode=lax.GatherScatterMode.FILL_OR_DROP)


def _ln_stats(x):
    m = jnp.mean(x, axis=-1, keepdims=True)
    c = x - m
    v = jnp.mean(c * c, axis=-1, keepdims=True)
    return m, c, lax.rsqrt(v + EPS)


def _with_ones(x):
    return jnp.concatenate([x, jnp.ones_like(x)], axis=0).astype(bf16)


def _centered_dot(xo, w, m):
    y = _dot(xo, w)
    return y[0:8] - m * y[8:16]


def _packed(t):
    return _as_f32(jnp.concatenate([t, t], axis=0).astype(bf16))


def _columns(row):
    col = jnp.concatenate([row] * 16, axis=0).T
    return [col[8 * a:8 * a + 8] for a in range(16)]


def _unpack(w):
    return w << 16, w & jnp.uint32(0xFFFF0000)


def _run(*gens):
    for g in gens:
        for _ in g:
            pass


def _take(gen, n):
    for _ in range(n):
        yield next(gen)


def _group_order():
    order = []
    step = GH // NW
    for par in range(2):
        packed = list(range(GH * par, GH * par + GH - NW))
        wide = list(range(GH * par + GH - NW, GH * par + GH))
        order += [(wide if n % step == step // 2 else packed).pop(0)
                  for n in range(GH)]
    return order


def _make_kernel(sk, win):
    nc = win // 128
    ncp = nc // 2
    row0 = (sk - win) // 128 * 4
    assert nc == 32
    scale = float(np.asarray(DH ** -0.5, dtype=bf16)) * float(np.log2(np.e))
    order = _group_order()

    def kernel(x_hbm, k_hbm, v_hbm, wq_hbm, wo_hbm, w1_hbm, w3_hbm, w2_hbm,
               o_ref,
               xbuf, kbuf, vbuf, vwide, vlast, vlast_lo, wq, wo, w1, w3, w2,
               zq, ybuf, qbuf, pbuf, lbuf, abuf, obuf, zeros, ones, tab,
               ksem, vsem, wsem):
        k32 = k_hbm.bitcast(u32)
        v32 = v_hbm.bitcast(u32)
        window = pl.ds(row0, 4 * nc)

        def k_copy(i):
            return pltpu.make_async_copy(
                k32.at[i, :, :, window, :], kbuf.at[i], ksem.at[i])

        def v_copies(i):
            return (
                pltpu.make_async_copy(
                    v32.at[i, :, pl.ds(0, GH - NW), window, :], vbuf.at[i],
                    vsem.at[2 * i]),
                pltpu.make_async_copy(
                    v32.at[i, :, pl.ds(GH - NW, NW), window, :],
                    vwide.at[i, 1], vsem.at[2 * i + 1]))

        x_copy = pltpu.make_async_copy(x_hbm, xbuf, wsem.at[0])
        wq_copy = pltpu.make_async_copy(wq_hbm.bitcast(u32), wq, wsem.at[1])
        wo_copy = pltpu.make_async_copy(wo_hbm.bitcast(u32), wo, wsem.at[2])
        vlast_copy = pltpu.make_async_copy(
            v32.at[NP - 1, :, :, window, :], vlast, wsem.at[3])
        w1_copy = pltpu.make_async_copy(w1_hbm, w1, wsem.at[4])
        w3_copy = pltpu.make_async_copy(w3_hbm, w3, wsem.at[5])
        w2_copies = [
            pltpu.make_async_copy(w2_hbm.at[pl.ds(a, b - a)],
                                  w2.at[pl.ds(a, b - a)], wsem.at[6 + n])
            for n, (a, b) in enumerate(W2_SPLITS)]

        wq_copy.start()
        x_copy.start()
        wo_copy.start()
        k_copy(0).start()

        def start_kv(i, carry):
            for cp in v_copies(i):
                cp.start()
            k_copy(i + 1).start()
            return carry

        lax.fori_loop(0, NP - 1, start_kv, 0)
        vlast_copy.start()

        lane = lax.broadcasted_iota(jnp.int32, (8, 128), 1)
        sub = lax.broadcasted_iota(jnp.int32, (8, 128), 0)
        zeros[...] = jnp.zeros((8, 128), u32)
        ones[...] = jnp.ones((8, 128), f32)
        for n in range(4):
            tab[n] = 2 * n + (sub >> 2)
        tab[4] = sub ^ 1
        tab[5] = jnp.zeros_like(sub)
        tab[6] = jnp.where(lane < 64, 0, 2)
        tab[7] = jnp.full_like(sub, 2)
        tab[8] = lane & 8
        tab[9] = sub
        tab[10] = sub - jnp.where(lane < 64, 0, 1)
        tab[11] = sub - 1
        for n in range(4):
            tab[12 + n] = jnp.where((sub >> 1) == n // 2,
                                    -65536 if n % 2 else 65535, 0)

        def retile(ref, ntile, place):
            top = sub < 4
            nrep = ref.shape[1] // (8 * ntile)

            def body(a, carry):
                v = [ref[a, 8 * n:8 * n + 8, :] for n in range(nrep * ntile)]
                for k in range(nrep):
                    for t in range(ntile):
                        lo = v[k * ntile + t // 2]
                        hi = v[k * ntile + (ntile + t) // 2]
                        if t % 2:
                            lo = pltpu.roll(lo, 4, 0)
                        if (ntile + t) % 2 == 0:
                            hi = pltpu.roll(hi, 4, 0)
                        r = 8 * place(k, t)
                        ref[a, r:r + 8, :] = jnp.where(top, lo, hi)
                return carry

            lax.fori_loop(0, ref.shape[0], body, 0)

        def k_rows(g, c):
            r = 8 * (c ^ (g // 2 % 4))
            return slice(r, r + 8)

        wq_copy.wait()
        retile(wq, H * DH // 128, lambda k, t: 2 * t + k)
        w1_copy.start()
        w3_copy.start()
        wo_copy.wait()
        retile(wo, D // 128, lambda k, t: t)
        for cp in w2_copies:
            cp.start()

        def expand_q(t, b):
            even = tab[8] == 0
            return [jnp.where(tab[9 + t] == 2 * var, y, jnp.uint32(0))
                    for y in (jnp.where(even, b >> 16, pltpu.roll(b, 8, 1)),
                              jnp.where(even, pltpu.roll(b, 120, 1) >> 16, b))
                    for var in range(2)]

        def q_stage(u, e, out, proj=None, expand=True):
            if e is None:
                wref, e = wq.at[:, pl.ds(pl.multiple_of(48 * u, 16), 48), :], 0
            elif isinstance(u, int):
                wref = wq.at[:, pl.ds(96 * u, 96), :]
            else:
                wref = wq.at[:, pl.ds(pl.multiple_of(96 * u, 32), 96), :]
            for t in range(3):
                r = 48 * e + 16 * t
                w = _as_bf16(wref[:, r:r + 16, :].reshape(D // 2, 128))
                q = proj(w) if proj else _dot(_as_bf16(zq[...]), w)[0:8]
                b = pltpu.bitcast(_round_bf16(q), u32)
                out.extend(expand_q(t, b) if expand else [b])
                yield 40, [(_as_f32(b), 7)]

        def fold_rows(x, op):
            x = op(x, pltpu.roll(x, 4, 0))
            return op(x, _gather_rows(x, tab[4]))

        def k_stage(i, ys, out):
            kref = kbuf.at[i]
            m = None
            for c in range(ncp):
                lhs = jnp.concatenate(
                    [ys(2 * n + c % 2) for n in range(6)], axis=1)
                w = jnp.concatenate(
                    [kref[g // GH, g % GH, k_rows(g, c), :]
                     for t in range(3) for e in range(2)
                     for g in range(16 * t + e, 16 * t + 16, 2)], axis=0)
                s = _dot(_as_bf16(lhs), _as_bf16(w))[0:8]
                if c % 2 == 0:
                    out.append(s)
                    yield 48, [(s, 6)]
                else:
                    out[-1] = out[-1] + s
                    m = out[-1] if m is None else jnp.maximum(m, out[-1])
                    if c == ncp - 1:
                        m = fold_rows(m, jnp.maximum)
                    yield 48, [(m, 12 if c == ncp - 1 else 8)]
            out.append(m)

        def k_first(qb, out_a, out):
            even, low = tab[8] == 0, tab[6] == 0
            b = qb[1]
            rot = {n: pltpu.roll(b, n, 1) for n in (8, 56, 64, 72, 120)}
            mix = (jnp.where(even, jnp.where(low, b, rot[56]) >> 16,
                             jnp.where(low, rot[8], rot[64])),
                   jnp.where(even, jnp.where(low, rot[64], rot[120]) >> 16,
                             jnp.where(low, rot[72], b)))
            tiles = []
            for par in range(2):
                ys = expand_q(2 * par, qb[2 * par])
                for e in range(2):
                    tiles.append((ys[2 * e:2 * e + 2],
                                  range(32 * par + e, 32 * par + 16, 2)))
                g0 = 16 + 8 * par
                tiles.append((
                    [jnp.where(tab[9 + 2 * par] == 2 * var, mix[par],
                               jnp.uint32(0)) for var in range(2)],
                    [*range(g0, g0 + 8, 2), *range(g0 + 1, g0 + 8, 2)]))

            def part(c, sel):
                lhs = jnp.concatenate([tiles[n][0][c % 2] for n in sel], axis=1)
                w = jnp.concatenate(
                    [kbuf[0, g // GH, g % GH, k_rows(g, c), :]
                     for n in sel for g in tiles[n][1]], axis=0)
                return _dot(_as_bf16(lhs), _as_bf16(w))[0:8]

            plan = [(c, (0, 1)) for c in range(4)] + [(c, (2,)) for c in range(4)]
            plan += [(c, (0, 1, 2)) for c in range(4, ncp - NKV)]
            acc = [None] * (ncp // 2)
            cols = _columns(_as_f32(qb[0])) + _columns(_as_f32(qb[1]))[:8]
            vacc = [None] * (2 * NKV)
            for g in range(GH):
                for n, c in enumerate(range(ncp - NKV, ncp)):
                    k = _as_bf16(kbuf[0, 0, g, k_rows(g, c), :]).astype(f32)
                    for e in range(2):
                        t = k[8 * e:8 * e + 8] * cols[g]
                        vacc[2 * n + e] = t if g == 0 else vacc[2 * n + e] + t
            for n, t in enumerate(vacc):
                for sh in (4, 2, 1):
                    t = t + pltpu.roll(t, sh, 0)
                c = ncp - NKV + n // 2
                prev = 0.0 if acc[c // 2] is None else acc[c // 2]
                acc[c // 2] = jnp.where(tab[9] == 4 * (c % 2) + n % 2, t, prev)
            for c, sel in plan:
                s = part(c, sel)
                acc[c // 2] = s if acc[c // 2] is None else acc[c // 2] + s
                yield 8 * len(sel), []
            m = acc[0]
            for a in acc[1:]:
                m = jnp.maximum(m, a)
            out_a.extend(acc + [fold_rows(m, jnp.maximum)])
            m = None
            for j in range(ncp // 2):
                s = acc[j] + part(2 * j, (3, 4, 5)) + part(2 * j + 1, (3, 4, 5))
                out.append(s)
                m = s if m is None else jnp.maximum(m, s)
                if j == ncp // 2 - 1:
                    m = fold_rows(m, jnp.maximum)
                yield 48, [(m, 8)]
            out.append(m)

        def softmax_numerator(ss, sc=scale):
            m = jnp.max(ss[-1], axis=1, keepdims=True)
            return [jnp.exp2((s - m) * sc) for s in ss[:-1]]

        def inverse_sum(ps):
            tot = ps[0]
            for p in ps[1:]:
                tot = tot + p
            lf = fold_rows(tot, jnp.add)
            l = jnp.sum(lf, axis=1, keepdims=True)
            l = jnp.broadcast_to(l, (8, 128))
            y = pl.reciprocal(l, approx=True)
            return lf, y * (2.0 - l * y)

        def lane_sums(b, j):
            a = jnp.concatenate(
                [abuf[b, 16 * j:16 * j + 16, 8 * s:8 * s + 8, :].reshape(128, 128)
                 for s in range(2)], axis=1)
            return lax.dot_general(
                jnp.concatenate([ones[...]] * 2, axis=1), a,
                (((1,), (1,)), ((), ())), preferred_element_type=f32)

        def r_stage(b, out):
            for j in range(3):
                out.append(_packed(lane_sums(b, j) * lbuf[b, j]))
                yield 32, [(out[-1], 4)]

        def o_stage(i, ts):
            wref = wo.at[pl.ds(24 * i, 24)]
            t = _as_bf16(jnp.concatenate(ts, axis=1))
            for n in range(D // 128):
                cols = slice(128 * n, 128 * n + 128)
                w = wref[:, 8 * n:8 * n + 8, :].reshape(DH, 128)
                y = obuf[:, cols] + _dot(t, _as_bf16(w))[0:8]
                obuf[:, cols] = y
                yield 24, [(y, 4)]

        def o_tile(i, j, t):
            r0 = 24 * i + 8 * j
            w = jnp.concatenate(
                [wo[r0:r0 + 8, 8 * n:8 * n + 8, :].reshape(64, 128)
                 for n in range(D // 128)], axis=1)
            return _dot(_as_bf16(t), _as_bf16(w))[0:8]

        def trace_mxu(gens, links, latency, t=0.0, rate=1.0):
            for gen in gens:
                for cost, res in gen:
                    t += cost / rate
                    links.setdefault(t + latency, []).extend(res)
            return t

        def v_stage(i, b, getp, links, clock, hist, pace):
            never = zeros[...] != 0
            last = i is None
            for n, g in enumerate(range(NG) if last else order):
                par, gl = divmod(g, GH)
                if n % GH == 0:
                    ps = [getp(par, j) for j in range(nc // 4)]
                    idx = [tab[par], tab[2 + par]]
                    if len(hist) > 1 and getp is not from_pbuf:
                        dep = pltpu.bitcast(hist[-2][0], jnp.int32)
                        idx = [jnp.where(never, dep, ix) for ix in idx]
                    pv = [_gather_rows(ps[c // 2], idx[c % 2])
                          for c in range(ncp - NT if last else ncp)]
                    clock[0] += 4
                    if par == 1 and not last:
                        lf, inv = inverse_sum(ps)
                        for val, at in zip((lf, inv), pace[2]):
                            links.setdefault(clock[0] + at, []).append((val, 14))
                        for j in range(3):
                            lbuf[b, j] = _gather_rows(inv, tab[5 + j])
                wide = last or gl >= GH - NW
                if last:
                    refs = vlast_lo.at[par, gl], vlast.at[par, gl]
                elif wide:
                    ref = vwide.at[i, :, par, gl - (GH - NW)]
                    refs = ref.at[0], ref.at[1]
                else:
                    ref = vbuf.at[i, par, gl]
                dur = T_LAST if last else T_GROUP * (pace[0] if wide else 1.0)
                accs = [None, None]
                held = [None, None]
                pending = []
                nsteps = ncp - NT if last else ncp
                for c in range(nsteps):
                    for key in sorted(links):
                        if key < clock[0] + dur * (c + 1) / nsteps:
                            for val, ops in links.pop(key):
                                pending.append(val)
                                clock[0] += ops / 4
                    rs = slice(8 * c, 8 * c + 8)
                    if wide:
                        lo, hi = refs[0][rs, :], refs[1][rs, :]
                    else:
                        lo, hi = _unpack(ref[rs, :])
                    p = pv[c]
                    if c == (8 if last else pace[1] if wide else 0) and hist:
                        p = jnp.where(never, hist[-1][0] + hist[-1][1], p)
                    for a, t in enumerate((_as_f32(lo) * p, _as_f32(hi) * p)):
                        if accs[a] is None:
                            accs[a] = t
                            continue
                        if pending:
                            t = jnp.where(never, pending.pop(), t)
                        if c % 2 == 1 and c < nsteps - 1:
                            held[a] = t
                        else:
                            if held[a] is not None:
                                t = held[a] + t
                                held[a] = None
                            accs[a] = accs[a] + t
                for a in range(2):
                    abuf[b, g, pl.ds(a, 8, stride=2), :] = accs[a]
                clock[0] += dur
                hist.append(accs)
                yield g

        def from_pbuf(par, j):
            return pbuf[par, j]

        def values(ps):
            return lambda par, j: ps[j]

        def store_state(ya, qb, ps):
            for n in range(12):
                ybuf[n] = ya[n]
            for n in range(3):
                qbuf[n] = qb[n]
            for j, p in enumerate(ps):
                pbuf[0, j] = p
                pbuf[1, j] = p

        def four_pairs(u0):
            links, clock, hist = {}, [10], []
            getq, getp = (lambda n: qbuf[n]), from_pbuf
            s1 = []
            k1 = k_stage(2 * u0 + 1, lambda n: ybuf[n], s1)
            t = 0.0

            def mxu(gens, t):
                return trace_mxu(gens, links, LOOP_MXU[0], t, LOOP_MXU[1])

            for half in range(2):
                u = u0 + half
                i = 2 * u
                s2, ya, qb, t0, t1 = [], [], [], [], []
                y2 = [y for n in range(3) for y in expand_q(n, getq(n))]
                k2 = k_stage(i + 2, y2.__getitem__, s2)
                t = mxu([k1], t)
                p1 = softmax_numerator(s1)
                t = mxu([r_stage(1, t1), q_stage(u + 1, 1, ya),
                         o_stage(i - 1, t1), _take(k2, 4 + 4 * half)], t)
                _run(v_stage(i, 0, getp, links, clock, hist, LOOP_PACE))
                t = mxu([r_stage(0, t0), k2], max(t, clock[0] - 64))
                p2 = softmax_numerator(s2)
                t = mxu([o_stage(i, t0),
                         q_stage(jnp.minimum(u + 2, NP // 2 - 1), 0, qb,
                                 expand=False)], t)
                if half == 0:
                    s1 = []
                    k1 = k_stage(i + 3, ya.__getitem__, s1)
                    t = mxu([_take(k1, 3)], t)
                _run(v_stage(i + 1, 1, values(p1), links, clock, hist,
                             LOOP_PACE))
                getq, getp = qb.__getitem__, values(p2)
            store_state(ya, qb, p2)

        def first_pairs(xo, m, r):
            links, clock, hist = {}, [T_FIRST], []
            q0, y1, y2, sa, s0, s1, s2, ya, qb, t0 = ([] for _ in range(10))
            _run(q_stage(0, 0, q0, lambda w: _centered_dot(xo, w, m), False),
                 q_stage(0, 1, y1, lambda w: _centered_dot(xo, w, m) * r))
            t = trace_mxu([k_first(q0, sa, s0),
                           k_stage(1, lambda n: y1[n], s1),
                           q_stage(1, 0, y2), q_stage(1, 1, ya),
                           q_stage(2, 0, qb, expand=False)], links, 190)
            for key in [key for key in links if key < T_FIRST + 30]:
                del links[key]
            pa = softmax_numerator(sa, r * scale)
            p0 = softmax_numerator(s0, r * scale)
            p1 = softmax_numerator(s1)
            _run(v_stage(0, 0, lambda par, j: (pa, p0)[par][j], links,
                         clock, hist, EDGE_PACE))
            trace_mxu([r_stage(0, t0), k_stage(2, lambda n: y2[n], s2),
                       o_stage(0, t0)], links, 190,
                      max(t, clock[0] - 64))
            p2 = softmax_numerator(s2)
            _run(v_stage(1, 1, values(p1), links, clock,
                         hist, EDGE_PACE))
            store_state(ya, qb, p2)

        def vt_slot(kc, j, n):
            g = 24 * (kc % 2) + 8 * j + n
            r = 8 * (kc // 2)
            return (g // GH, g % GH, slice(r, r + 8), slice(None))

        def last_pairs():
            i = NP - 2
            links, clock, hist = {}, [20], []
            s1, t0, t1, ts, part, rows = ([] for _ in range(6))
            tk = trace_mxu([k_stage(i + 1, lambda n: ybuf[n], s1)], links, 185)
            t = trace_mxu([r_stage(1, t1)], links, 185, tk)
            t = trace_mxu([o_stage(i - 1, t1)], links, 185, t + 60)
            ps = softmax_numerator(s1)
            chunks = range(nc - 2 * NT, nc)
            for kc in chunks:
                bits = pltpu.bitcast(_packed(ps[kc // 4]), u32)
                rows.append(bits & pltpu.bitcast(tab[12 + kc % 4], u32))
                links.setdefault(tk + 315, []).append((_as_f32(rows[-1]), 3))
            lhs = _as_bf16(jnp.concatenate(rows, axis=1))

            def p_stage():
                for j in range(3):
                    w = jnp.concatenate([vlast[vt_slot(kc, j, n)]
                                         for kc in chunks for n in range(8)],
                                        axis=0)
                    y = fold_rows(_dot(lhs, _as_bf16(w))[0:8], jnp.add)
                    part.append(_gather_rows(y, tab[5 + j]))
                    yield 16 * NT, [(part[j], 2 * NT + 5)]

            pg = p_stage()
            t = trace_mxu([_take(pg, 1)], links, 210, max(t, tk + 266))
            _run(v_stage(i, 0, from_pbuf, links, clock, hist,
                         EDGE_PACE[:2] + ((),)))
            trace_mxu([r_stage(0, t0), _take(pg, 1), o_stage(i, t0), pg],
                      links, 210, max(t, clock[0] + 56))
            lf, inv = inverse_sum(ps)
            links.setdefault(clock[0] + 20, []).append((lf, 10))
            links.setdefault(clock[0] + 160, []).append((inv, 10))
            for g in v_stage(None, 1, values(ps), links, clock, hist,
                             EDGE_PACE):
                if g % 16 == 15:
                    j = g // 16
                    ts.append(_packed((lane_sums(1, j) + part[j])
                                      * _gather_rows(inv, tab[5 + j])))
            y = obuf[...]
            for j in range(3):
                y = y + o_tile(NP - 1, j, ts[j])
            return y

        def start_attention(x):
            m, c, r = _ln_stats(x)
            z = c * r
            zq[...] = pltpu.bitcast(
                jnp.concatenate([z, z], axis=0).astype(bf16), u32)
            obuf[...] = jnp.zeros(obuf.shape, f32)
            return m, r

        def attention(x):
            m, r = start_attention(x)
            first_pairs(_with_ones(x), m, r)

            def body(it, carry):
                four_pairs(1 + 2 * it)
                return carry

            lax.fori_loop(0, (NP - 4) // 4, body, 0)
            return last_pairs()

        def streamed_pair(i, u, e):
            last = isinstance(i, int)
            ys = []
            _run(q_stage(u, e, ys))
            lhs = [_as_bf16(jnp.concatenate(ys[var::2], axis=1))
                   for var in range(2)]
            k_copy(i).wait()
            ss = []
            for c in range(ncp):
                k = kbuf[i, :, :, 8 * c:8 * c + 8, :].reshape(3, 8, 2, 8, 128)
                w = jnp.concatenate(
                    [k[t, :, par].reshape(64, 128)
                     for t in range(3) for par in range(2)], axis=0)
                s = _dot(lhs[c % 2], _as_bf16(w))[0:8]
                if c % 2:
                    s = ss.pop() + s
                ss.append(s)
            m = ss[0]
            for s in ss[1:]:
                m = jnp.maximum(m, s)
            ps = softmax_numerator(ss + [fold_rows(m, jnp.maximum)])
            inv = inverse_sum(ps)[1]
            for j in range(3):
                lbuf[0, j] = _gather_rows(inv, tab[5 + j])

            def swizzle(a, carry):
                for g in range(2, 8):
                    ref = kbuf.at[i, a // 3, 8 * (a % 3) + g]
                    v = ref[...].reshape(4, 4, 8, 128)
                    v = jnp.concatenate(
                        [v[:, c ^ (g // 2):(c ^ (g // 2)) + 1] for c in range(4)],
                        axis=1)
                    ref[...] = v.reshape(128, 128)
                return carry

            lax.fori_loop(0, NG // 8, swizzle, 0)

            for cp in ((vlast_copy,) if last else v_copies(i)):
                cp.wait()
            for par in range(2):
                pv = jnp.concatenate(
                    [_gather_rows(ps[c // 2], tab[2 * (c % 2) + par])
                     for c in range(ncp)], axis=0)

                def group(g, w):
                    for a, half in enumerate(_unpack(w)):
                        acc = (_as_f32(half) * pv).reshape(ncp, 8, 128)
                        abuf[0, g, pl.ds(a, 8, stride=2), :] = jnp.sum(acc, axis=0)

                def packed_group(gl, carry):
                    group(GH * par + gl, vbuf[i, par, gl])
                    return carry

                def wide_group(gl, carry):
                    if last:
                        w = vlast[par, gl]
                        keep = slice(0, 8 * (ncp - NT))
                        vlast_lo[par, gl], vlast[par, gl, keep, :] = _unpack(w[keep])
                    else:
                        ref = vwide.at[i, :, par, gl - (GH - NW)]
                        w = ref[1]
                        ref[0], ref[1] = _unpack(w)
                    group(GH * par + gl, w)
                    return carry

                split = 0 if last else GH - NW
                if split:
                    lax.fori_loop(0, split, packed_group, 0)
                lax.fori_loop(split, GH, wide_group, 0)
            ts = []
            _run(r_stage(0, ts), o_stage(i, ts))

        def transpose_last():
            for c in range(ncp - NT, ncp):
                v = _as_bf16(vlast[:, :, 8 * c:8 * c + 8, :].reshape(
                    8 * NG, 128)).astype(f32).reshape(NG, 16, 128)
                for s in range(2):
                    for j in range(3):
                        t = v[16 * j:16 * j + 16, 8 * s:8 * s + 8].reshape(128, 128)
                        t = pltpu.bitcast(t.T.astype(bf16), u32)
                        for n in range(8):
                            vlast[vt_slot(2 * c + s, j, n)] = t[8 * n:8 * n + 8]

        def streamed_attention(x):
            start_attention(x)

            def body(i, carry):
                streamed_pair(i, i, None)
                return carry

            lax.fori_loop(0, NP - 1, body, 0)
            streamed_pair(NP - 1, NP // 2 - 1, 1)
            transpose_last()
            return obuf[...]

        def ffn(first, x):
            if first:
                w1_copy.wait()
                w3_copy.wait()
            m, _, r = _ln_stats(x)
            xo = _with_ones(x)
            hids = []
            for n in range(0, FF, FCH):
                gate = _round_bf16(_centered_dot(xo, w1[:, n:n + FCH], m) * r)
                up = _round_bf16(_centered_dot(xo, w3[:, n:n + FCH], m) * r)
                hids.append(
                    (_round_bf16(gate * jax.nn.sigmoid(gate)) * up).astype(bf16))
            y = None
            starts = [a for a, _ in W2_SPLITS]
            nv = 0 if first else NFV
            acc = [None] * (D // 128)
            for n in range(nv):
                for a, cv in enumerate(_columns(hids[n].astype(f32))):
                    if acc[0] is not None:
                        cv = jnp.where(zeros[...] != 0,
                                       acc[a % 5] + acc[(a + 2) % 5], cv)
                    for j in range(D // 128):
                        t = cv * w2[n, 8 * a:8 * a + 8,
                                    128 * j:128 * j + 128].astype(f32)
                        acc[j] = t if acc[j] is None else acc[j] + t
            if nv:
                y = jnp.sum(jnp.concatenate(acc, axis=1), axis=0, keepdims=True)
            for n in range(nv, len(hids)):
                if first and n in starts:
                    if y is not None:
                        obuf[...] = y
                    w2_copies[starts.index(n)].wait()
                    if y is not None:
                        y = obuf[...]
                t = _dot(hids[n], w2[n])
                y = t if y is None else y + t
            return y

        x_copy.wait()
        x = jnp.broadcast_to(xbuf[0].astype(f32), (8, D))
        x = _round_bf16(x + _round_bf16(streamed_attention(x)))
        x = _round_bf16(x + _round_bf16(ffn(True, x)))
        x = _round_bf16(x + _round_bf16(attention(x)))
        x = _round_bf16(x + _round_bf16(ffn(False, x)))
        o_ref[0] = x[0:1].astype(bf16)

    return kernel


def _tiles(a, lead):
    r, c = a.shape
    t = a.reshape(r // 8, 8, c // 128, 128).transpose(0, 2, 1, 3)
    return t.reshape(lead + (-1, 128))


@jax.jit
def pallas_interleave_layers__sliding_block_cached__glu_gated_swiglu__decode_kernel(
    A_x: jax.Array,
    A_k_cache: jax.Array,
    A_v_cache: jax.Array,
    A_wq: jax.Array,
    A_wo: jax.Array,
    B_x: jax.Array,
    B_w1: jax.Array,
    B_w3: jax.Array,
    B_w2: jax.Array,
):
    del B_x
    sk = A_k_cache.shape[2]
    win = min(4096, max(256, sk // 4))
    wr = win // 32
    kt = _tiles(jnp.swapaxes(A_k_cache, 2, 3).reshape(H * DH, sk), (NP, 2, GH))
    vt = _tiles(jnp.swapaxes(A_v_cache, 2, 3).reshape(H * DH, sk), (NP, 2, GH))
    any_spec = pl.BlockSpec(memory_space=pl.ANY)
    return pl.pallas_call(
        _make_kernel(sk, win),
        out_shape=jax.ShapeDtypeStruct((1, 1, D), bf16),
        in_specs=[any_spec] * 8,
        out_specs=pl.BlockSpec(memory_space=pltpu.VMEM),
        scratch_shapes=[
            pltpu.VMEM((1, 1, D), bf16),
            pltpu.VMEM((NP, 2, GH, wr, 128), u32),
            pltpu.VMEM((NP - 1, 2, GH - NW, wr, 128), u32),
            pltpu.VMEM((NP - 1, 2, 2, NW, wr, 128), u32),
            pltpu.VMEM((2, GH, wr, 128), u32),
            pltpu.VMEM((2, GH, wr - 8 * NT, 128), u32),
            pltpu.VMEM((D // 32, H * DH // 8, 128), u32),
            pltpu.VMEM((H * DH // 16, D // 16, 128), u32),
            pltpu.VMEM((D, FF), bf16),
            pltpu.VMEM((D, FF), bf16),
            pltpu.VMEM((FF // FCH, FCH, D), bf16),
            pltpu.VMEM((8, D), u32),
            pltpu.VMEM((12, 8, 128), u32),
            pltpu.VMEM((3, 8, 128), u32),
            pltpu.VMEM((2, 8, 8, 128), f32),
            pltpu.VMEM((2, 3, 8, 128), f32),
            pltpu.VMEM((2, NG, 16, 128), f32),
            pltpu.VMEM((8, D), f32),
            pltpu.VMEM((8, 128), u32),
            pltpu.VMEM((8, 128), f32),
            pltpu.VMEM((16, 8, 128), jnp.int32),
            pltpu.SemaphoreType.DMA((NP,)),
            pltpu.SemaphoreType.DMA((2 * NP - 2,)),
            pltpu.SemaphoreType.DMA((8,)),
        ],
        compiler_params=pltpu.CompilerParams(
            vmem_limit_bytes=128 * 1024 * 1024,
            disable_semaphore_checks=True),
    )(A_x, kt, vt, _tiles(A_wq, (D // 32,)), _tiles(A_wo, (H * DH // 16,)),
      B_w1, B_w3, B_w2.reshape(FF // FCH, FCH, D))
```

```python
import jax
import jax.numpy as jnp
import numpy as np
from jax import lax
import jax.experimental.pallas as pl
import jax.experimental.pallas.tpu as pltpu

D = 640
H = 32
NP = H // 2
DH = 192
GH = DH // 8
NG = 2 * GH
FF = 1536
FCH = 128
EPS = 1e-5

NT = 7
NKV = 6
NFV = 6
NR = 12
NW = 7
W2_SPLITS = ((0, 10), (10, 12))

T_GROUP = 24.1
T_LAST = 12.0
T_FIRST = 610
EDGE_PACE = (0.8, 6, (40, 200))
LOOP_PACE = (0.8, 5, (30, 180))
LOOP_MXU = (175, 0.99)

f32 = jnp.float32
bf16 = jnp.bfloat16
u32 = jnp.uint32


def _round_bf16(x):
    return x.astype(bf16).astype(f32)


def _as_bf16(x):
    return pltpu.bitcast(x, bf16)


def _as_f32(x):
    return pltpu.bitcast(x, f32)


def _dot(a, b):
    return jnp.dot(a, b, preferred_element_type=f32)


def _gather_rows(x, idx):
    dnums = lax.GatherDimensionNumbers(
        offset_dims=(), collapsed_slice_dims=(0,), start_index_map=(0,),
        operand_batching_dims=(1,), start_indices_batching_dims=(1,))
    return lax.gather(x, idx.reshape(8, 128, 1), dnums, slice_sizes=(1, 1),
                      mode=lax.GatherScatterMode.FILL_OR_DROP)


def _ln_stats(x):
    m = jnp.mean(x, axis=-1, keepdims=True)
    c = x - m
    v = jnp.mean(c * c, axis=-1, keepdims=True)
    return m, c, lax.rsqrt(v + EPS)


def _with_ones(x):
    return jnp.concatenate([x, jnp.ones_like(x)], axis=0).astype(bf16)


def _centered_dot(xo, w, m):
    y = _dot(xo, w)
    return y[0:8] - m * y[8:16]


def _packed(t):
    return _as_f32(jnp.concatenate([t, t], axis=0).astype(bf16))


def _columns(row):
    col = jnp.concatenate([row] * 16, axis=0).T
    return [col[8 * a:8 * a + 8] for a in range(16)]


def _unpack(w):
    return w << 16, w & jnp.uint32(0xFFFF0000)


def _run(*gens):
    for g in gens:
        for _ in g:
            pass


def _take(gen, n):
    for _ in range(n):
        yield next(gen)


def _group_order():
    order = []
    spots = {int((n + 0.5) * GH / NW) for n in range(NW)}
    for par in range(2):
        packed = list(range(GH * par, GH * par + GH - NW))
        wide = list(range(GH * par + GH - NW, GH * par + GH))
        order += [(wide if n in spots else packed).pop(0) for n in range(GH)]
    return order


def _ring(i):
    if isinstance(i, int):
        return i % NR
    return jnp.where(i >= NR, i - NR, i)


def _make_kernel(sk, win):
    nc = win // 128
    ncp = nc // 2
    row0 = (sk - win) // 128 * 4
    assert nc == 32
    scale = float(np.asarray(DH ** -0.5, dtype=bf16)) * float(np.log2(np.e))
    order = _group_order()

    def kernel(x_hbm, k_hbm, v_hbm, wq_hbm, wo_hbm, w1_hbm, w3_hbm, w2_hbm,
               o_ref,
               xbuf, kbuf, vbuf, vwide, vlast, vlast_lo, wq, wo, w1, w3, w2,
               zq, ybuf, qbuf, pbuf, lbuf, abuf, obuf, zeros, ones, tab,
               ksem, vsem, wsem):
        k32 = k_hbm.bitcast(u32)
        v32 = v_hbm.bitcast(u32)
        window = pl.ds(row0, 4 * nc)

        def k_copy(i):
            return pltpu.make_async_copy(
                k32.at[i, :, :, window, :], kbuf.at[i], ksem.at[i])

        def vp_copy(i, dst=None):
            return pltpu.make_async_copy(
                v32.at[i, :, pl.ds(0, GH - NW), window, :],
                vbuf.at[_ring(i)] if dst is None else dst, vsem.at[2 * i])

        def v_copies(i):
            return (vp_copy(i), pltpu.make_async_copy(
                v32.at[i, :, pl.ds(GH - NW, NW), window, :],
                vwide.at[i, 1], vsem.at[2 * i + 1]))

        def visit(n):
            spare = NP - 1 - NR
            return jnp.where(n < spare, n + NR, jnp.where(n >= NR, n - NR, n))

        def start_pair(n, carry=None):
            k_copy(visit(n)).start()
            for cp in v_copies(visit(n)):
                cp.start()
            return carry

        v14 = kbuf.at[0, :, pl.ds(0, GH - NW)]
        x_copy = pltpu.make_async_copy(x_hbm, xbuf, wsem.at[0])
        wq_copy = pltpu.make_async_copy(wq_hbm.bitcast(u32), wq, wsem.at[1])
        wo_copy = pltpu.make_async_copy(wo_hbm.bitcast(u32), wo, wsem.at[2])
        vlast_copy = pltpu.make_async_copy(
            v32.at[NP - 1, :, :, window, :], vlast, wsem.at[3])
        w1_copy = pltpu.make_async_copy(w1_hbm, w1, wsem.at[4])
        w3_copy = pltpu.make_async_copy(w3_hbm, w3, wsem.at[5])
        w2_copies = [
            pltpu.make_async_copy(w2_hbm.at[pl.ds(a, b - a)],
                                  w2.at[pl.ds(a, b - a)], wsem.at[6 + n])
            for n, (a, b) in enumerate(W2_SPLITS)]

        wq_copy.start()
        x_copy.start()
        wo_copy.start()
        lax.fori_loop(0, NR, start_pair, 0)

        lane = lax.broadcasted_iota(jnp.int32, (8, 128), 1)
        sub = lax.broadcasted_iota(jnp.int32, (8, 128), 0)
        zeros[...] = jnp.zeros((8, 128), u32)
        ones[...] = jnp.ones((8, 128), f32)
        for n in range(4):
            tab[n] = 2 * n + (sub >> 2)
        tab[4] = sub ^ 1
        tab[5] = jnp.zeros_like(sub)
        tab[6] = jnp.where(lane < 64, 0, 2)
        tab[7] = jnp.full_like(sub, 2)
        tab[8] = lane & 8
        tab[9] = sub
        tab[10] = sub - jnp.where(lane < 64, 0, 1)
        tab[11] = sub - 1
        for n in range(4):
            tab[12 + n] = jnp.where((sub >> 1) == n // 2,
                                    -65536 if n % 2 else 65535, 0)

        def retile(ref, ntile, place):
            top = sub < 4
            nrep = ref.shape[1] // (8 * ntile)

            def body(a, carry):
                v = [ref[a, 8 * n:8 * n + 8, :] for n in range(nrep * ntile)]
                for k in range(nrep):
                    for t in range(ntile):
                        lo = v[k * ntile + t // 2]
                        hi = v[k * ntile + (ntile + t) // 2]
                        if t % 2:
                            lo = pltpu.roll(lo, 4, 0)
                        if (ntile + t) % 2 == 0:
                            hi = pltpu.roll(hi, 4, 0)
                        r = 8 * place(k, t)
                        ref[a, r:r + 8, :] = jnp.where(top, lo, hi)
                return carry

            lax.fori_loop(0, ref.shape[0], body, 0)

        def k_rows(g, c):
            r = 8 * (c ^ (g // 2 % 4))
            return slice(r, r + 8)

        wq_copy.wait()
        retile(wq, H * DH // 128, lambda k, t: 2 * t + k)
        wo_copy.wait()
        retile(wo, D // 128, lambda k, t: t)

        def expand_q(t, b):
            even = tab[8] == 0
            return [jnp.where(tab[9 + t] == 2 * var, y, jnp.uint32(0))
                    for y in (jnp.where(even, b >> 16, pltpu.roll(b, 8, 1)),
                              jnp.where(even, pltpu.roll(b, 120, 1) >> 16, b))
                    for var in range(2)]

        def q_stage(u, e, out, proj=None, expand=True):
            if e is None:
                wref, e = wq.at[:, pl.ds(pl.multiple_of(48 * u, 16), 48), :], 0
            elif isinstance(u, int):
                wref = wq.at[:, pl.ds(96 * u, 96), :]
            else:
                wref = wq.at[:, pl.ds(pl.multiple_of(96 * u, 32), 96), :]
            for t in range(3):
                r = 48 * e + 16 * t
                w = _as_bf16(wref[:, r:r + 16, :].reshape(D // 2, 128))
                q = proj(w) if proj else _dot(_as_bf16(zq[...]), w)[0:8]
                b = pltpu.bitcast(_round_bf16(q), u32)
                out.extend(expand_q(t, b) if expand else [b])
                yield 40, [(_as_f32(b), 7)]

        def fold_rows(x, op):
            x = op(x, pltpu.roll(x, 4, 0))
            return op(x, _gather_rows(x, tab[4]))

        def k_stage(i, ys, out):
            kref = kbuf.at[i]
            m = None
            for c in range(ncp):
                lhs = jnp.concatenate(
                    [ys(2 * n + c % 2) for n in range(6)], axis=1)
                w = jnp.concatenate(
                    [kref[g // GH, g % GH, k_rows(g, c), :]
                     for t in range(3) for e in range(2)
                     for g in range(16 * t + e, 16 * t + 16, 2)], axis=0)
                s = _dot(_as_bf16(lhs), _as_bf16(w))[0:8]
                if c % 2 == 0:
                    out.append(s)
                    yield 48, [(s, 6)]
                else:
                    out[-1] = out[-1] + s
                    m = out[-1] if m is None else jnp.maximum(m, out[-1])
                    if c == ncp - 1:
                        m = fold_rows(m, jnp.maximum)
                    yield 48, [(m, 12 if c == ncp - 1 else 8)]
            out.append(m)

        def k_first(qb, out_a, out):
            even, low = tab[8] == 0, tab[6] == 0
            b = qb[1]
            rot = {n: pltpu.roll(b, n, 1) for n in (8, 56, 64, 72, 120)}
            mix = (jnp.where(even, jnp.where(low, b, rot[56]) >> 16,
                             jnp.where(low, rot[8], rot[64])),
                   jnp.where(even, jnp.where(low, rot[64], rot[120]) >> 16,
                             jnp.where(low, rot[72], b)))
            tiles = []
            for par in range(2):
                ys = expand_q(2 * par, qb[2 * par])
                for e in range(2):
                    tiles.append((ys[2 * e:2 * e + 2],
                                  range(32 * par + e, 32 * par + 16, 2)))
                g0 = 16 + 8 * par
                tiles.append((
                    [jnp.where(tab[9 + 2 * par] == 2 * var, mix[par],
                               jnp.uint32(0)) for var in range(2)],
                    [*range(g0, g0 + 8, 2), *range(g0 + 1, g0 + 8, 2)]))

            def part(c, sel):
                lhs = jnp.concatenate([tiles[n][0][c % 2] for n in sel], axis=1)
                w = jnp.concatenate(
                    [kbuf[0, g // GH, g % GH, k_rows(g, c), :]
                     for n in sel for g in tiles[n][1]], axis=0)
                return _dot(_as_bf16(lhs), _as_bf16(w))[0:8]

            plan = [(c, (0, 1)) for c in range(4)] + [(c, (2,)) for c in range(4)]
            plan += [(c, (0, 1, 2)) for c in range(4, ncp - NKV)]
            acc = [None] * (ncp // 2)
            cols = _columns(_as_f32(qb[0])) + _columns(_as_f32(qb[1]))[:8]
            vacc = [None] * (2 * NKV)
            for g in range(GH):
                for n, c in enumerate(range(ncp - NKV, ncp)):
                    k = _as_bf16(kbuf[0, 0, g, k_rows(g, c), :]).astype(f32)
                    for e in range(2):
                        t = k[8 * e:8 * e + 8] * cols[g]
                        vacc[2 * n + e] = t if g == 0 else vacc[2 * n + e] + t
            for n, t in enumerate(vacc):
                for sh in (4, 2, 1):
                    t = t + pltpu.roll(t, sh, 0)
                c = ncp - NKV + n // 2
                prev = 0.0 if acc[c // 2] is None else acc[c // 2]
                acc[c // 2] = jnp.where(tab[9] == 4 * (c % 2) + n % 2, t, prev)
            for c, sel in plan:
                s = part(c, sel)
                acc[c // 2] = s if acc[c // 2] is None else acc[c // 2] + s
                yield 8 * len(sel), []
            m = acc[0]
            for a in acc[1:]:
                m = jnp.maximum(m, a)
            out_a.extend(acc + [fold_rows(m, jnp.maximum)])
            m = None
            for j in range(ncp // 2):
                s = acc[j] + part(2 * j, (3, 4, 5)) + part(2 * j + 1, (3, 4, 5))
                out.append(s)
                m = s if m is None else jnp.maximum(m, s)
                if j == ncp // 2 - 1:
                    m = fold_rows(m, jnp.maximum)
                yield 48, [(m, 8)]
            out.append(m)

        def softmax_numerator(ss, sc=scale):
            m = jnp.max(ss[-1], axis=1, keepdims=True)
            return [jnp.exp2((s - m) * sc) for s in ss[:-1]]

        def inverse_sum(ps):
            tot = ps[0]
            for p in ps[1:]:
                tot = tot + p
            lf = fold_rows(tot, jnp.add)
            l = jnp.sum(lf, axis=1, keepdims=True)
            l = jnp.broadcast_to(l, (8, 128))
            y = pl.reciprocal(l, approx=True)
            return lf, y * (2.0 - l * y)

        def lane_sums(b, j):
            a = jnp.concatenate(
                [abuf[b, 16 * j:16 * j + 16, 8 * s:8 * s + 8, :].reshape(128, 128)
                 for s in range(2)], axis=1)
            return lax.dot_general(
                jnp.concatenate([ones[...]] * 2, axis=1), a,
                (((1,), (1,)), ((), ())), preferred_element_type=f32)

        def r_stage(b, out):
            for j in range(3):
                out.append(_packed(lane_sums(b, j) * lbuf[b, j]))
                yield 32, [(out[-1], 4)]

        def o_stage(i, ts):
            wref = wo.at[pl.ds(24 * i, 24)]
            t = _as_bf16(jnp.concatenate(ts, axis=1))
            for n in range(D // 128):
                cols = slice(128 * n, 128 * n + 128)
                w = wref[:, 8 * n:8 * n + 8, :].reshape(DH, 128)
                y = obuf[:, cols] + _dot(t, _as_bf16(w))[0:8]
                obuf[:, cols] = y
                yield 24, [(y, 4)]

        def o_tile(i, j, t):
            r0 = 24 * i + 8 * j
            w = jnp.concatenate(
                [wo[r0:r0 + 8, 8 * n:8 * n + 8, :].reshape(64, 128)
                 for n in range(D // 128)], axis=1)
            return _dot(_as_bf16(t), _as_bf16(w))[0:8]

        def trace_mxu(gens, links, latency, t=0.0, rate=1.0):
            for gen in gens:
                for cost, res in gen:
                    t += cost / rate
                    links.setdefault(t + latency, []).extend(res)
            return t

        def v_stage(i, b, getp, links, clock, hist, pace):
            never = zeros[...] != 0
            last = i is None
            if not last:
                vp = (v14 if isinstance(i, int) and i == NP - 2
                      else vbuf.at[_ring(i)])
            for n, g in enumerate(range(NG) if last else order):
                par, gl = divmod(g, GH)
                if n % GH == 0:
                    ps = [getp(par, j) for j in range(nc // 4)]
                    idx = [tab[par], tab[2 + par]]
                    if len(hist) > 1 and getp is not from_pbuf:
                        dep = pltpu.bitcast(hist[-2][0], jnp.int32)
                        idx = [jnp.where(never, dep, ix) for ix in idx]
                    pv = [_gather_rows(ps[c // 2], idx[c % 2])
                          for c in range(ncp - NT if last else ncp)]
                    clock[0] += 4
                    if par == 1 and not last:
                        lf, inv = inverse_sum(ps)
                        for val, at in zip((lf, inv), pace[2]):
                            links.setdefault(clock[0] + at, []).append((val, 14))
                        for j in range(3):
                            lbuf[b, j] = _gather_rows(inv, tab[5 + j])
                wide = last or gl >= GH - NW
                if last:
                    refs = vlast_lo.at[par, gl], vlast.at[par, gl]
                elif wide:
                    ref = vwide.at[i, :, par, gl - (GH - NW)]
                    refs = ref.at[0], ref.at[1]
                else:
                    ref = vp.at[par, gl]
                dur = T_LAST if last else T_GROUP * (pace[0] if wide else 1.0)
                accs = [None, None]
                held = [None, None]
                pending = []
                nsteps = ncp - NT if last else ncp
                for c in range(nsteps):
                    for key in sorted(links):
                        if key < clock[0] + dur * (c + 1) / nsteps:
                            for val, ops in links.pop(key):
                                pending.append(val)
                                clock[0] += ops / 4
                    rs = slice(8 * c, 8 * c + 8)
                    if wide:
                        lo, hi = refs[0][rs, :], refs[1][rs, :]
                    else:
                        lo, hi = _unpack(ref[rs, :])
                    p = pv[c]
                    if c == (8 if last else pace[1] if wide else 0) and hist:
                        p = jnp.where(never, hist[-1][0] + hist[-1][1], p)
                    for a, t in enumerate((_as_f32(lo) * p, _as_f32(hi) * p)):
                        if accs[a] is None:
                            accs[a] = t
                            continue
                        if pending:
                            t = jnp.where(never, pending.pop(), t)
                        if c % 2 == 1 and c < nsteps - 1:
                            held[a] = t
                        else:
                            if held[a] is not None:
                                t = held[a] + t
                                held[a] = None
                            accs[a] = accs[a] + t
                for a in range(2):
                    abuf[b, g, pl.ds(a, 8, stride=2), :] = accs[a]
                clock[0] += dur
                hist.append(accs)
                yield g

        def from_pbuf(par, j):
            return pbuf[par, j]

        def values(ps):
            return lambda par, j: ps[j]

        def store_state(ya, qb, ps):
            for n in range(12):
                ybuf[n] = ya[n]
            for n in range(3):
                qbuf[n] = qb[n]
            for j, p in enumerate(ps):
                pbuf[0, j] = p
                pbuf[1, j] = p

        def four_pairs(u0):
            links, clock, hist = {}, [30], []
            getq, getp = (lambda n: qbuf[n]), from_pbuf
            s1 = []
            k1 = k_stage(2 * u0 + 1, lambda n: ybuf[n], s1)
            t = 0.0

            def mxu(gens, t):
                return trace_mxu(gens, links, LOOP_MXU[0], t, LOOP_MXU[1])

            for half in range(2):
                u = u0 + half
                i = 2 * u
                s2, ya, qb, t0, t1 = [], [], [], [], []
                y2 = [y for n in range(3) for y in expand_q(n, getq(n))]
                k2 = k_stage(i + 2, y2.__getitem__, s2)
                t = mxu([k1], t)
                p1 = softmax_numerator(s1)
                t = mxu([r_stage(1, t1), q_stage(u + 1, 1, ya),
                         o_stage(i - 1, t1), _take(k2, 4)], t)
                _run(v_stage(i, 0, getp, links, clock, hist, LOOP_PACE))
                t = mxu([r_stage(0, t0), k2], max(t, clock[0] - 64))
                p2 = softmax_numerator(s2)
                t = mxu([o_stage(i, t0),
                         q_stage(jnp.minimum(u + 2, NP // 2 - 1), 0, qb,
                                 expand=False)], t)
                if half == 0:
                    s1 = []
                    k1 = k_stage(i + 3, ya.__getitem__, s1)
                    t = mxu([_take(k1, 1)], t)
                _run(v_stage(i + 1, 1, values(p1), links, clock, hist,
                             LOOP_PACE))
                getq, getp = qb.__getitem__, values(p2)
            store_state(ya, qb, p2)

        def first_pairs(xo, m, r):
            links, clock, hist = {}, [T_FIRST], []
            q0, y1, y2, sa, s0, s1, s2, ya, qb, t0 = ([] for _ in range(10))
            _run(q_stage(0, 0, q0, lambda w: _centered_dot(xo, w, m), False),
                 q_stage(0, 1, y1, lambda w: _centered_dot(xo, w, m) * r))
            t = trace_mxu([k_first(q0, sa, s0),
                           k_stage(1, lambda n: y1[n], s1),
                           q_stage(1, 0, y2), q_stage(1, 1, ya),
                           q_stage(2, 0, qb, expand=False)], links, 190)
            for key in [key for key in links if key < T_FIRST + 30]:
                del links[key]
            pa = softmax_numerator(sa, r * scale)
            p0 = softmax_numerator(s0, r * scale)
            p1 = softmax_numerator(s1)
            _run(v_stage(0, 0, lambda par, j: (pa, p0)[par][j], links,
                         clock, hist, EDGE_PACE))
            vp_copy(NR).start()
            trace_mxu([r_stage(0, t0), k_stage(2, lambda n: y2[n], s2),
                       o_stage(0, t0)], links, 190,
                      max(t, clock[0] - 64))
            p2 = softmax_numerator(s2)
            _run(v_stage(1, 1, values(p1), links, clock,
                         hist, EDGE_PACE))
            store_state(ya, qb, p2)

        def vt_slot(kc, j, n):
            g = 24 * (kc % 2) + 8 * j + n
            r = 8 * (kc // 2)
            return (g // GH, g % GH, slice(r, r + 8), slice(None))

        def last_pairs():
            i = NP - 2
            links, clock, hist = {}, [20], []
            s1, t0, t1, ts, part, rows = ([] for _ in range(6))
            tk = trace_mxu([k_stage(i + 1, lambda n: ybuf[n], s1)], links, 170)
            t = trace_mxu([r_stage(1, t1)], links, 170, tk)
            t = trace_mxu([o_stage(i - 1, t1)], links, 170, t + 90)
            ps = softmax_numerator(s1)
            chunks = range(nc - 2 * NT, nc)
            for kc in chunks:
                bits = pltpu.bitcast(_packed(ps[kc // 4]), u32)
                rows.append(bits & pltpu.bitcast(tab[12 + kc % 4], u32))
                links.setdefault(tk + 315, []).append((_as_f32(rows[-1]), 3))
            lhs = _as_bf16(jnp.concatenate(rows, axis=1))

            def p_stage():
                for j in range(3):
                    w = jnp.concatenate([vlast[vt_slot(kc, j, n)]
                                         for kc in chunks for n in range(8)],
                                        axis=0)
                    y = fold_rows(_dot(lhs, _as_bf16(w))[0:8], jnp.add)
                    part.append(_gather_rows(y, tab[5 + j]))
                    yield 16 * NT, [(part[j], 2 * NT + 5)]

            pg = p_stage()
            t = trace_mxu([_take(pg, 1)], links, 160, max(t, tk + 300))
            _run(v_stage(i, 0, from_pbuf, links, clock, hist, EDGE_PACE))
            trace_mxu([r_stage(0, t0), _take(pg, 1), o_stage(i, t0), pg],
                      links, 160, max(t, clock[0] + 90))
            lf, inv = inverse_sum(ps)
            links.setdefault(clock[0] + 20, []).append((lf, 10))
            links.setdefault(clock[0] + 160, []).append((inv, 10))
            for g in v_stage(None, 1, values(ps), links, clock, hist,
                             EDGE_PACE):
                if g % 16 == 15:
                    j = g // 16
                    ts.append(_packed((lane_sums(1, j) + part[j])
                                      * _gather_rows(inv, tab[5 + j])))
            y = obuf[...]
            for j in range(3):
                y = y + o_tile(NP - 1, j, ts[j])
            return y

        def start_attention(x):
            m, c, r = _ln_stats(x)
            z = c * r
            zq[...] = pltpu.bitcast(
                jnp.concatenate([z, z], axis=0).astype(bf16), u32)
            obuf[...] = jnp.zeros(obuf.shape, f32)
            return m, r

        def attention(x):
            m, r = start_attention(x)
            first_pairs(_with_ones(x), m, r)
            vp_copy(NR + 1).start()
            vp_copy(NP - 2, v14).start()

            def body(it, carry):
                @pl.when(it == (NP - 4) // 4 - 1)
                def _():
                    for i in range(NR, NP - 2):
                        vp_copy(i).wait()

                four_pairs(1 + 2 * it)
                return carry

            lax.fori_loop(0, (NP - 4) // 4, body, 0)
            vp_copy(NP - 2, v14).wait()
            return last_pairs()

        def streamed_pair(i, u, e):
            last = isinstance(i, int)
            ys = []
            _run(q_stage(u, e, ys))
            lhs = [_as_bf16(jnp.concatenate(ys[var::2], axis=1))
                   for var in range(2)]
            k_copy(i).wait()
            ss = []
            for c in range(ncp):
                k = kbuf[i, :, :, 8 * c:8 * c + 8, :].reshape(3, 8, 2, 8, 128)
                w = jnp.concatenate(
                    [k[t, :, par].reshape(64, 128)
                     for t in range(3) for par in range(2)], axis=0)
                s = _dot(lhs[c % 2], _as_bf16(w))[0:8]
                if c % 2:
                    s = ss.pop() + s
                ss.append(s)
            m = ss[0]
            for s in ss[1:]:
                m = jnp.maximum(m, s)
            ps = softmax_numerator(ss + [fold_rows(m, jnp.maximum)])
            inv = inverse_sum(ps)[1]
            for j in range(3):
                lbuf[0, j] = _gather_rows(inv, tab[5 + j])

            def swizzle(a, carry):
                for g in range(2, 8):
                    ref = kbuf.at[i, a // 3, 8 * (a % 3) + g]
                    v = ref[...].reshape(4, 4, 8, 128)
                    v = jnp.concatenate(
                        [v[:, c ^ (g // 2):(c ^ (g // 2)) + 1] for c in range(4)],
                        axis=1)
                    ref[...] = v.reshape(128, 128)
                return carry

            lax.fori_loop(0, NG // 8, swizzle, 0)

            for cp in ((vlast_copy,) if last else v_copies(i)):
                cp.wait()
            for par in range(2):
                pv = jnp.concatenate(
                    [_gather_rows(ps[c // 2], tab[2 * (c % 2) + par])
                     for c in range(ncp)], axis=0)

                def group(g, w):
                    for a, half in enumerate(_unpack(w)):
                        acc = (_as_f32(half) * pv).reshape(ncp, 8, 128)
                        abuf[0, g, pl.ds(a, 8, stride=2), :] = jnp.sum(acc, axis=0)

                def packed_group(gl, carry):
                    group(GH * par + gl, vbuf[_ring(i), par, gl])
                    return carry

                def wide_group(gl, carry):
                    if last:
                        w = vlast[par, gl]
                        keep = slice(0, 8 * (ncp - NT))
                        vlast_lo[par, gl], vlast[par, gl, keep, :] = _unpack(w[keep])
                    else:
                        ref = vwide.at[i, :, par, gl - (GH - NW)]
                        w = ref[1]
                        ref[0], ref[1] = _unpack(w)
                    group(GH * par + gl, w)
                    return carry

                split = 0 if last else GH - NW
                if split:
                    lax.fori_loop(0, split, packed_group, 0)
                lax.fori_loop(split, GH, wide_group, 0)
            ts = []
            _run(r_stage(0, ts), o_stage(i, ts))

        def transpose_last():
            for c in range(ncp - NT, ncp):
                v = _as_bf16(vlast[:, :, 8 * c:8 * c + 8, :].reshape(
                    8 * NG, 128)).astype(f32).reshape(NG, 16, 128)
                for s in range(2):
                    for j in range(3):
                        t = v[16 * j:16 * j + 16, 8 * s:8 * s + 8].reshape(128, 128)
                        t = pltpu.bitcast(t.T.astype(bf16), u32)
                        for n in range(8):
                            vlast[vt_slot(2 * c + s, j, n)] = t[8 * n:8 * n + 8]

        def streamed_attention(x):
            start_attention(x)

            spare = NP - 1 - NR
            late = [[k_copy(NP - 1)], [vlast_copy], [w1_copy, w3_copy]]
            late += [[cp] for cp in w2_copies]

            def body(n, carry):
                @pl.when(jnp.logical_and(n >= spare, n < 2 * spare))
                def _():
                    start_pair(n + NR - spare)

                for k, cps in enumerate(late):
                    @pl.when(n == 2 * spare + k)
                    def _():
                        for cp in cps:
                            cp.start()

                streamed_pair(visit(n), visit(n), None)
                return carry

            lax.fori_loop(0, NP - 1, body, 0)
            streamed_pair(NP - 1, NP // 2 - 1, 1)
            transpose_last()
            return obuf[...]

        def ffn(first, x):
            if first:
                w1_copy.wait()
                w3_copy.wait()
            m, _, r = _ln_stats(x)
            xo = _with_ones(x)
            hids = []
            for n in range(0, FF, FCH):
                gate = _round_bf16(_centered_dot(xo, w1[:, n:n + FCH], m) * r)
                up = _round_bf16(_centered_dot(xo, w3[:, n:n + FCH], m) * r)
                hids.append(
                    (_round_bf16(gate * jax.nn.sigmoid(gate)) * up).astype(bf16))
            y = None
            starts = [a for a, _ in W2_SPLITS]
            nv = 0 if first else NFV
            acc = [None] * (D // 128)
            for n in range(nv):
                for a, cv in enumerate(_columns(hids[n].astype(f32))):
                    if acc[0] is not None:
                        cv = jnp.where(zeros[...] != 0,
                                       acc[a % 5] + acc[(a + 2) % 5], cv)
                    for j in range(D // 128):
                        t = cv * w2[n, 8 * a:8 * a + 8,
                                    128 * j:128 * j + 128].astype(f32)
                        acc[j] = t if acc[j] is None else acc[j] + t
            if nv:
                y = jnp.sum(jnp.concatenate(acc, axis=1), axis=0, keepdims=True)
            for n in range(nv, len(hids)):
                if first and n in starts:
                    if y is not None:
                        obuf[...] = y
                    w2_copies[starts.index(n)].wait()
                    if y is not None:
                        y = obuf[...]
                t = _dot(hids[n], w2[n])
                y = t if y is None else y + t
            return y

        x_copy.wait()
        x = jnp.broadcast_to(xbuf[0].astype(f32), (8, D))
        x = _round_bf16(x + _round_bf16(streamed_attention(x)))
        x = _round_bf16(x + _round_bf16(ffn(True, x)))
        x = _round_bf16(x + _round_bf16(attention(x)))
        x = _round_bf16(x + _round_bf16(ffn(False, x)))
        o_ref[0] = x[0:1].astype(bf16)

    return kernel


def _tiles(a, lead):
    r, c = a.shape
    t = a.reshape(r // 8, 8, c // 128, 128).transpose(0, 2, 1, 3)
    return t.reshape(lead + (-1, 128))


@jax.jit
def pallas_interleave_layers__sliding_block_cached__glu_gated_swiglu__decode_kernel(
    A_x: jax.Array,
    A_k_cache: jax.Array,
    A_v_cache: jax.Array,
    A_wq: jax.Array,
    A_wo: jax.Array,
    B_x: jax.Array,
    B_w1: jax.Array,
    B_w3: jax.Array,
    B_w2: jax.Array,
):
    del B_x
    sk = A_k_cache.shape[2]
    win = min(4096, max(256, sk // 4))
    wr = win // 32
    kt = _tiles(jnp.swapaxes(A_k_cache, 2, 3).reshape(H * DH, sk), (NP, 2, GH))
    vt = _tiles(jnp.swapaxes(A_v_cache, 2, 3).reshape(H * DH, sk), (NP, 2, GH))
    any_spec = pl.BlockSpec(memory_space=pl.ANY)
    return pl.pallas_call(
        _make_kernel(sk, win),
        out_shape=jax.ShapeDtypeStruct((1, 1, D), bf16),
        in_specs=[any_spec] * 8,
        out_specs=pl.BlockSpec(memory_space=pltpu.VMEM),
        scratch_shapes=[
            pltpu.VMEM((1, 1, D), bf16),
            pltpu.VMEM((NP, 2, GH, wr, 128), u32),
            pltpu.VMEM((NR, 2, GH - NW, wr, 128), u32),
            pltpu.VMEM((NP - 1, 2, 2, NW, wr, 128), u32),
            pltpu.VMEM((2, GH, wr, 128), u32),
            pltpu.VMEM((2, GH, wr - 8 * NT, 128), u32),
            pltpu.VMEM((D // 32, H * DH // 8, 128), u32),
            pltpu.VMEM((H * DH // 16, D // 16, 128), u32),
            pltpu.VMEM((D, FF), bf16),
            pltpu.VMEM((D, FF), bf16),
            pltpu.VMEM((FF // FCH, FCH, D), bf16),
            pltpu.VMEM((8, D), u32),
            pltpu.VMEM((12, 8, 128), u32),
            pltpu.VMEM((3, 8, 128), u32),
            pltpu.VMEM((2, 8, 8, 128), f32),
            pltpu.VMEM((2, 3, 8, 128), f32),
            pltpu.VMEM((2, NG, 16, 128), f32),
            pltpu.VMEM((8, D), f32),
            pltpu.VMEM((8, 128), u32),
            pltpu.VMEM((8, 128), f32),
            pltpu.VMEM((16, 8, 128), jnp.int32),
            pltpu.SemaphoreType.DMA((NP,)),
            pltpu.SemaphoreType.DMA((2 * NP - 2,)),
            pltpu.SemaphoreType.DMA((8,)),
        ],
        compiler_params=pltpu.CompilerParams(
            vmem_limit_bytes=128 * 1024 * 1024,
            disable_semaphore_checks=True),
    )(A_x, kt, vt, _tiles(A_wq, (D // 32,)), _tiles(A_wo, (H * DH // 16,)),
      B_w1, B_w3, B_w2.reshape(FF // FCH, FCH, D))
```

```python
import jax
import jax.numpy as jnp
import numpy as np
from jax import lax
import jax.experimental.pallas as pl
import jax.experimental.pallas.tpu as pltpu

D = 640
H = 32
NP = H // 2
DH = 192
GH = DH // 8
NG = 2 * GH
FF = 1536
FCH = 128
EPS = 1e-5

NT = 7
NKV = 6
NFV = 6
NR = 12
NW = 7
W2_SPLITS = ((0, 10), (10, 12))

T_GROUP = 24.1
T_LAST = 12.0
T_FIRST = 610
EDGE_PACE = (0.8, 6, (40, 200))
LOOP_PACE = (0.8, 5, (30, 180))
LAT_FIRST = (187, 191, 180, 183, 190, 198, 210, 183, 178, 170, 185, 163, 113)
LAT_LOOP = (152, 200, 185, 218, 185, 160, 180, 187, 195, 162, 170, 178, 203,
            199, 179, 179, 187, 187, 151)
LAT_LAST = (138, 155, 123, 155, 155, 128, 160, 147, 221)

f32 = jnp.float32
bf16 = jnp.bfloat16
u32 = jnp.uint32


def _round_bf16(x):
    return x.astype(bf16).astype(f32)


def _as_bf16(x):
    return pltpu.bitcast(x, bf16)


def _as_f32(x):
    return pltpu.bitcast(x, f32)


def _dot(a, b):
    return jnp.dot(a, b, preferred_element_type=f32)


def _gather_rows(x, idx):
    dnums = lax.GatherDimensionNumbers(
        offset_dims=(), collapsed_slice_dims=(0,), start_index_map=(0,),
        operand_batching_dims=(1,), start_indices_batching_dims=(1,))
    return lax.gather(x, idx.reshape(8, 128, 1), dnums, slice_sizes=(1, 1),
                      mode=lax.GatherScatterMode.FILL_OR_DROP)


def _ln_stats(x):
    m = jnp.mean(x, axis=-1, keepdims=True)
    c = x - m
    v = jnp.mean(c * c, axis=-1, keepdims=True)
    return m, c, lax.rsqrt(v + EPS)


def _with_ones(x):
    return jnp.concatenate([x, jnp.ones_like(x)], axis=0).astype(bf16)


def _centered_dot(xo, w, m):
    y = _dot(xo, w)
    return y[0:8] - m * y[8:16]


def _packed(t):
    return _as_f32(jnp.concatenate([t, t], axis=0).astype(bf16))


def _columns(row):
    col = jnp.concatenate([row] * 16, axis=0).T
    return [col[8 * a:8 * a + 8] for a in range(16)]


def _unpack(w):
    return w << 16, w & jnp.uint32(0xFFFF0000)


def _run(*gens):
    for g in gens:
        for _ in g:
            pass


def _take(gen, n):
    for _ in range(n):
        yield next(gen)


def _group_order():
    order = []
    spots = {int((n + 0.5) * GH / NW) for n in range(NW)}
    for par in range(2):
        packed = list(range(GH * par, GH * par + GH - NW))
        wide = list(range(GH * par + GH - NW, GH * par + GH))
        order += [(wide if n in spots else packed).pop(0) for n in range(GH)]
    return order


def _ring(i):
    if isinstance(i, int):
        return i % NR
    return jnp.where(i >= NR, i - NR, i)


def _make_kernel(sk, win):
    nc = win // 128
    ncp = nc // 2
    row0 = (sk - win) // 128 * 4
    assert nc == 32
    scale = float(np.asarray(DH ** -0.5, dtype=bf16)) * float(np.log2(np.e))
    order = _group_order()

    def kernel(x_hbm, k_hbm, v_hbm, wq_hbm, wo_hbm, w1_hbm, w3_hbm, w2_hbm,
               o_ref,
               xbuf, kbuf, vbuf, vwide, vlast, vlast_lo, wq, wo, w1, w3, w2,
               zq, ybuf, qbuf, pbuf, lbuf, abuf, obuf, zeros, ones, tab,
               ksem, vsem, wsem):
        k32 = k_hbm.bitcast(u32)
        v32 = v_hbm.bitcast(u32)
        window = pl.ds(row0, 4 * nc)

        def k_copy(i):
            return pltpu.make_async_copy(
                k32.at[i, :, :, window, :], kbuf.at[i], ksem.at[i])

        def vp_copy(i, dst=None):
            return pltpu.make_async_copy(
                v32.at[i, :, pl.ds(0, GH - NW), window, :],
                vbuf.at[_ring(i)] if dst is None else dst, vsem.at[2 * i])

        def v_copies(i):
            return (vp_copy(i), pltpu.make_async_copy(
                v32.at[i, :, pl.ds(GH - NW, NW), window, :],
                vwide.at[i, 1], vsem.at[2 * i + 1]))

        def visit(n):
            spare = NP - 1 - NR
            return jnp.where(n < spare, n + NR, jnp.where(n >= NR, n - NR, n))

        def start_pair(n, carry=None):
            k_copy(visit(n)).start()
            for cp in v_copies(visit(n)):
                cp.start()
            return carry

        v14 = kbuf.at[0, :, pl.ds(0, GH - NW)]
        x_copy = pltpu.make_async_copy(x_hbm, xbuf, wsem.at[0])
        wq_copy = pltpu.make_async_copy(wq_hbm.bitcast(u32), wq, wsem.at[1])
        wo_copy = pltpu.make_async_copy(wo_hbm.bitcast(u32), wo, wsem.at[2])
        vlast_copy = pltpu.make_async_copy(
            v32.at[NP - 1, :, :, window, :], vlast, wsem.at[3])
        w1_copy = pltpu.make_async_copy(w1_hbm, w1, wsem.at[4])
        w3_copy = pltpu.make_async_copy(w3_hbm, w3, wsem.at[5])
        w2_copies = [
            pltpu.make_async_copy(w2_hbm.at[pl.ds(a, b - a)],
                                  w2.at[pl.ds(a, b - a)], wsem.at[6 + n])
            for n, (a, b) in enumerate(W2_SPLITS)]

        wq_copy.start()
        x_copy.start()
        wo_copy.start()
        lax.fori_loop(0, NR, start_pair, 0)

        lane = lax.broadcasted_iota(jnp.int32, (8, 128), 1)
        sub = lax.broadcasted_iota(jnp.int32, (8, 128), 0)
        zeros[...] = jnp.zeros((8, 128), u32)
        ones[...] = jnp.ones((8, 128), f32)
        for n in range(4):
            tab[n] = 2 * n + (sub >> 2)
        tab[4] = sub ^ 1
        tab[5] = jnp.zeros_like(sub)
        tab[6] = jnp.where(lane < 64, 0, 2)
        tab[7] = jnp.full_like(sub, 2)
        tab[8] = lane & 8
        tab[9] = sub
        tab[10] = sub - jnp.where(lane < 64, 0, 1)
        tab[11] = sub - 1
        for n in range(4):
            tab[12 + n] = jnp.where((sub >> 1) == n // 2,
                                    -65536 if n % 2 else 65535, 0)

        def retile(ref, ntile, place):
            top = sub < 4
            nrep = ref.shape[1] // (8 * ntile)

            def body(a, carry):
                v = [ref[a, 8 * n:8 * n + 8, :] for n in range(nrep * ntile)]
                for k in range(nrep):
                    for t in range(ntile):
                        lo = v[k * ntile + t // 2]
                        hi = v[k * ntile + (ntile + t) // 2]
                        if t % 2:
                            lo = pltpu.roll(lo, 4, 0)
                        if (ntile + t) % 2 == 0:
                            hi = pltpu.roll(hi, 4, 0)
                        r = 8 * place(k, t)
                        ref[a, r:r + 8, :] = jnp.where(top, lo, hi)
                return carry

            lax.fori_loop(0, ref.shape[0], body, 0)

        def k_rows(g, c):
            r = 8 * (c ^ (g // 2 % 4))
            return slice(r, r + 8)

        wq_copy.wait()
        retile(wq, H * DH // 128, lambda k, t: 2 * t + k)
        wo_copy.wait()
        retile(wo, D // 128, lambda k, t: t)

        def expand_q(t, b):
            even = tab[8] == 0
            return [jnp.where(tab[9 + t] == 2 * var, y, jnp.uint32(0))
                    for y in (jnp.where(even, b >> 16, pltpu.roll(b, 8, 1)),
                              jnp.where(even, pltpu.roll(b, 120, 1) >> 16, b))
                    for var in range(2)]

        def q_stage(u, e, out, proj=None, expand=True):
            if e is None:
                wref, e = wq.at[:, pl.ds(pl.multiple_of(48 * u, 16), 48), :], 0
            elif isinstance(u, int):
                wref = wq.at[:, pl.ds(96 * u, 96), :]
            else:
                wref = wq.at[:, pl.ds(pl.multiple_of(96 * u, 32), 96), :]
            for t in range(3):
                r = 48 * e + 16 * t
                w = _as_bf16(wref[:, r:r + 16, :].reshape(D // 2, 128))
                q = proj(w) if proj else _dot(_as_bf16(zq[...]), w)[0:8]
                b = pltpu.bitcast(_round_bf16(q), u32)
                out.extend(expand_q(t, b) if expand else [b])
                yield 40, [(_as_f32(b), 7)]

        def fold_rows(x, op):
            x = op(x, pltpu.roll(x, 4, 0))
            return op(x, _gather_rows(x, tab[4]))

        def k_stage(i, ys, out):
            kref = kbuf.at[i]
            m = None
            for c in range(ncp):
                lhs = jnp.concatenate(
                    [ys(2 * n + c % 2) for n in range(6)], axis=1)
                w = jnp.concatenate(
                    [kref[g // GH, g % GH, k_rows(g, c), :]
                     for t in range(3) for e in range(2)
                     for g in range(16 * t + e, 16 * t + 16, 2)], axis=0)
                s = _dot(_as_bf16(lhs), _as_bf16(w))[0:8]
                if c % 2 == 0:
                    out.append(s)
                    yield 48, [(s, 6)]
                else:
                    out[-1] = out[-1] + s
                    m = out[-1] if m is None else jnp.maximum(m, out[-1])
                    if c == ncp - 1:
                        m = fold_rows(m, jnp.maximum)
                    yield 48, [(m, 12 if c == ncp - 1 else 8)]
            out.append(m)

        def k_first(qb, out_a, out):
            even, low = tab[8] == 0, tab[6] == 0
            b = qb[1]
            rot = {n: pltpu.roll(b, n, 1) for n in (8, 56, 64, 72, 120)}
            mix = (jnp.where(even, jnp.where(low, b, rot[56]) >> 16,
                             jnp.where(low, rot[8], rot[64])),
                   jnp.where(even, jnp.where(low, rot[64], rot[120]) >> 16,
                             jnp.where(low, rot[72], b)))
            tiles = []
            for par in range(2):
                ys = expand_q(2 * par, qb[2 * par])
                for e in range(2):
                    tiles.append((ys[2 * e:2 * e + 2],
                                  range(32 * par + e, 32 * par + 16, 2)))
                g0 = 16 + 8 * par
                tiles.append((
                    [jnp.where(tab[9 + 2 * par] == 2 * var, mix[par],
                               jnp.uint32(0)) for var in range(2)],
                    [*range(g0, g0 + 8, 2), *range(g0 + 1, g0 + 8, 2)]))

            def part(c, sel):
                lhs = jnp.concatenate([tiles[n][0][c % 2] for n in sel], axis=1)
                w = jnp.concatenate(
                    [kbuf[0, g // GH, g % GH, k_rows(g, c), :]
                     for n in sel for g in tiles[n][1]], axis=0)
                return _dot(_as_bf16(lhs), _as_bf16(w))[0:8]

            plan = [(c, (0, 1)) for c in range(4)] + [(c, (2,)) for c in range(4)]
            plan += [(c, (0, 1, 2)) for c in range(4, ncp - NKV)]
            acc = [None] * (ncp // 2)
            cols = _columns(_as_f32(qb[0])) + _columns(_as_f32(qb[1]))[:8]
            vacc = [None] * (2 * NKV)
            for g in range(GH):
                for n, c in enumerate(range(ncp - NKV, ncp)):
                    k = _as_bf16(kbuf[0, 0, g, k_rows(g, c), :]).astype(f32)
                    for e in range(2):
                        t = k[8 * e:8 * e + 8] * cols[g]
                        vacc[2 * n + e] = t if g == 0 else vacc[2 * n + e] + t
            for n, t in enumerate(vacc):
                for sh in (4, 2, 1):
                    t = t + pltpu.roll(t, sh, 0)
                c = ncp - NKV + n // 2
                prev = 0.0 if acc[c // 2] is None else acc[c // 2]
                acc[c // 2] = jnp.where(tab[9] == 4 * (c % 2) + n % 2, t, prev)
            for c, sel in plan:
                s = part(c, sel)
                acc[c // 2] = s if acc[c // 2] is None else acc[c // 2] + s
                yield 8 * len(sel), []
            m = acc[0]
            for a in acc[1:]:
                m = jnp.maximum(m, a)
            out_a.extend(acc + [fold_rows(m, jnp.maximum)])
            m = None
            for j in range(ncp // 2):
                s = acc[j] + part(2 * j, (3, 4, 5)) + part(2 * j + 1, (3, 4, 5))
                out.append(s)
                m = s if m is None else jnp.maximum(m, s)
                if j == ncp // 2 - 1:
                    m = fold_rows(m, jnp.maximum)
                yield 48, [(m, 8)]
            out.append(m)

        def softmax_numerator(ss, sc=scale):
            m = jnp.max(ss[-1], axis=1, keepdims=True)
            return [jnp.exp2((s - m) * sc) for s in ss[:-1]]

        def inverse_sum(ps):
            tot = ps[0]
            for p in ps[1:]:
                tot = tot + p
            lf = fold_rows(tot, jnp.add)
            l = jnp.sum(lf, axis=1, keepdims=True)
            l = jnp.broadcast_to(l, (8, 128))
            y = pl.reciprocal(l, approx=True)
            return lf, y * (2.0 - l * y)

        def lane_sums(b, j):
            a = jnp.concatenate(
                [abuf[b, 16 * j:16 * j + 16, 8 * s:8 * s + 8, :].reshape(128, 128)
                 for s in range(2)], axis=1)
            return lax.dot_general(
                jnp.concatenate([ones[...]] * 2, axis=1), a,
                (((1,), (1,)), ((), ())), preferred_element_type=f32)

        def r_stage(b, out):
            for j in range(3):
                out.append(_packed(lane_sums(b, j) * lbuf[b, j]))
                yield 32, [(out[-1], 4)]

        def o_stage(i, ts):
            wref = wo.at[pl.ds(24 * i, 24)]
            t = _as_bf16(jnp.concatenate(ts, axis=1))
            for n in range(D // 128):
                cols = slice(128 * n, 128 * n + 128)
                w = wref[:, 8 * n:8 * n + 8, :].reshape(DH, 128)
                y = obuf[:, cols] + _dot(t, _as_bf16(w))[0:8]
                obuf[:, cols] = y
                yield 24, [(y, 4)]

        def o_tile(i, j, t):
            r0 = 24 * i + 8 * j
            w = jnp.concatenate(
                [wo[r0:r0 + 8, 8 * n:8 * n + 8, :].reshape(64, 128)
                 for n in range(D // 128)], axis=1)
            return _dot(_as_bf16(t), _as_bf16(w))[0:8]

        def trace_mxu(gens, links, latency, t=0.0, rate=1.0):
            for gen in gens:
                for cost, res in gen:
                    t += cost / rate
                    lat = np.interp(t / 250, range(len(latency)), latency)
                    links.setdefault(t + float(lat), []).extend(res)
            return t

        def v_stage(i, b, getp, links, clock, hist, pace):
            never = zeros[...] != 0
            last = i is None
            if not last:
                vp = (v14 if isinstance(i, int) and i == NP - 2
                      else vbuf.at[_ring(i)])
            for n, g in enumerate(range(NG) if last else order):
                par, gl = divmod(g, GH)
                if n % GH == 0:
                    ps = [getp(par, j) for j in range(nc // 4)]
                    idx = [tab[par], tab[2 + par]]
                    if len(hist) > 1 and getp is not from_pbuf:
                        dep = pltpu.bitcast(hist[-2][0], jnp.int32)
                        idx = [jnp.where(never, dep, ix) for ix in idx]
                    pv = [_gather_rows(ps[c // 2], idx[c % 2])
                          for c in range(ncp - NT if last else ncp)]
                    clock[0] += 4
                    if par == 1 and not last:
                        lf, inv = inverse_sum(ps)
                        for val, at in zip((lf, inv), pace[2]):
                            links.setdefault(clock[0] + at, []).append((val, 14))
                        for j in range(3):
                            lbuf[b, j] = _gather_rows(inv, tab[5 + j])
                wide = last or gl >= GH - NW
                if last:
                    refs = vlast_lo.at[par, gl], vlast.at[par, gl]
                elif wide:
                    ref = vwide.at[i, :, par, gl - (GH - NW)]
                    refs = ref.at[0], ref.at[1]
                else:
                    ref = vp.at[par, gl]
                dur = T_LAST if last else T_GROUP * (pace[0] if wide else 1.0)
                accs = [None, None]
                held = [None, None]
                pending = []
                nsteps = ncp - NT if last else ncp
                for c in range(nsteps):
                    for key in sorted(links):
                        if key < clock[0] + dur * (c + 1) / nsteps:
                            for val, ops in links.pop(key):
                                pending.append(val)
                                clock[0] += ops / 4
                    rs = slice(8 * c, 8 * c + 8)
                    if wide:
                        lo, hi = refs[0][rs, :], refs[1][rs, :]
                    else:
                        lo, hi = _unpack(ref[rs, :])
                    p = pv[c]
                    if c == (8 if last else pace[1] if wide else 0) and hist:
                        p = jnp.where(never, hist[-1][0] + hist[-1][1], p)
                    for a, t in enumerate((_as_f32(lo) * p, _as_f32(hi) * p)):
                        if accs[a] is None:
                            accs[a] = t
                            continue
                        if pending:
                            t = jnp.where(never, pending.pop(), t)
                        if c % 2 == 1 and c < nsteps - 1:
                            held[a] = t
                        else:
                            if held[a] is not None:
                                t = held[a] + t
                                held[a] = None
                            accs[a] = accs[a] + t
                for a in range(2):
                    abuf[b, g, pl.ds(a, 8, stride=2), :] = accs[a]
                clock[0] += dur
                hist.append(accs)
                yield g

        def from_pbuf(par, j):
            return pbuf[par, j]

        def values(ps):
            return lambda par, j: ps[j]

        def store_state(ya, qb, ps):
            for n in range(12):
                ybuf[n] = ya[n]
            for n in range(3):
                qbuf[n] = qb[n]
            for j, p in enumerate(ps):
                pbuf[0, j] = p
                pbuf[1, j] = p

        def four_pairs(u0):
            links, clock, hist = {}, [30], []
            getq, getp = (lambda n: qbuf[n]), from_pbuf
            s1 = []
            k1 = k_stage(2 * u0 + 1, lambda n: ybuf[n], s1)
            t = 0.0

            def mxu(gens, t):
                return trace_mxu(gens, links, LAT_LOOP, t, 0.99)

            for half in range(2):
                u = u0 + half
                i = 2 * u
                s2, ya, qb, t0, t1 = [], [], [], [], []
                y2 = [y for n in range(3) for y in expand_q(n, getq(n))]
                k2 = k_stage(i + 2, y2.__getitem__, s2)
                t = mxu([k1], t)
                p1 = softmax_numerator(s1)
                t = mxu([r_stage(1, t1), q_stage(u + 1, 1, ya),
                         o_stage(i - 1, t1), _take(k2, 4)], t)
                _run(v_stage(i, 0, getp, links, clock, hist, LOOP_PACE))
                t = mxu([r_stage(0, t0), k2], max(t, clock[0] - 64))
                p2 = softmax_numerator(s2)
                t = mxu([o_stage(i, t0),
                         q_stage(jnp.minimum(u + 2, NP // 2 - 1), 0, qb,
                                 expand=False)], t)
                if half == 0:
                    s1 = []
                    k1 = k_stage(i + 3, ya.__getitem__, s1)
                    t = mxu([_take(k1, 1)], t)
                _run(v_stage(i + 1, 1, values(p1), links, clock, hist,
                             LOOP_PACE))
                getq, getp = qb.__getitem__, values(p2)
            store_state(ya, qb, p2)

        def first_pairs(xo, m, r):
            links, clock, hist = {}, [T_FIRST], []
            q0, y1, y2, sa, s0, s1, s2, ya, qb, t0 = ([] for _ in range(10))
            _run(q_stage(0, 0, q0, lambda w: _centered_dot(xo, w, m), False),
                 q_stage(0, 1, y1, lambda w: _centered_dot(xo, w, m) * r))
            t = trace_mxu([k_first(q0, sa, s0),
                           k_stage(1, lambda n: y1[n], s1),
                           q_stage(1, 0, y2), q_stage(1, 1, ya),
                           q_stage(2, 0, qb, expand=False)], links, LAT_FIRST)
            for key in [key for key in links if key < T_FIRST + 30]:
                del links[key]
            pa = softmax_numerator(sa, r * scale)
            p0 = softmax_numerator(s0, r * scale)
            p1 = softmax_numerator(s1)
            _run(v_stage(0, 0, lambda par, j: (pa, p0)[par][j], links,
                         clock, hist, EDGE_PACE))
            vp_copy(NR).start()
            trace_mxu([r_stage(0, t0), k_stage(2, lambda n: y2[n], s2),
                       o_stage(0, t0)], links, LAT_FIRST,
                      max(t, clock[0] - 64))
            p2 = softmax_numerator(s2)
            _run(v_stage(1, 1, values(p1), links, clock,
                         hist, EDGE_PACE))
            store_state(ya, qb, p2)

        def vt_slot(kc, j, n):
            g = 24 * (kc % 2) + 8 * j + n
            r = 8 * (kc // 2)
            return (g // GH, g % GH, slice(r, r + 8), slice(None))

        def last_pairs():
            i = NP - 2
            links, clock, hist = {}, [20], []
            s1, t0, t1, ts, part, rows = ([] for _ in range(6))
            tk = trace_mxu([k_stage(i + 1, lambda n: ybuf[n], s1)],
                           links, LAT_LAST)
            t = trace_mxu([r_stage(1, t1)], links, LAT_LAST, tk)
            t = trace_mxu([o_stage(i - 1, t1)], links, LAT_LAST, t + 90)
            ps = softmax_numerator(s1)
            chunks = range(nc - 2 * NT, nc)
            for kc in chunks:
                bits = pltpu.bitcast(_packed(ps[kc // 4]), u32)
                rows.append(bits & pltpu.bitcast(tab[12 + kc % 4], u32))
                links.setdefault(tk + 315, []).append((_as_f32(rows[-1]), 3))
            lhs = _as_bf16(jnp.concatenate(rows, axis=1))

            def p_stage():
                for j in range(3):
                    w = jnp.concatenate([vlast[vt_slot(kc, j, n)]
                                         for kc in chunks for n in range(8)],
                                        axis=0)
                    y = fold_rows(_dot(lhs, _as_bf16(w))[0:8], jnp.add)
                    part.append(_gather_rows(y, tab[5 + j]))
                    yield 16 * NT, [(part[j], 2 * NT + 5)]

            pg = p_stage()
            t = trace_mxu([_take(pg, 1)], links, LAT_LAST, max(t, tk + 300))
            _run(v_stage(i, 0, from_pbuf, links, clock, hist, EDGE_PACE))
            trace_mxu([r_stage(0, t0), _take(pg, 1), o_stage(i, t0), pg],
                      links, LAT_LAST, max(t, clock[0] + 90))
            lf, inv = inverse_sum(ps)
            links.setdefault(clock[0] + 20, []).append((lf, 10))
            links.setdefault(clock[0] + 160, []).append((inv, 10))
            for g in v_stage(None, 1, values(ps), links, clock, hist,
                             EDGE_PACE):
                if g % 16 == 15:
                    j = g // 16
                    ts.append(_packed((lane_sums(1, j) + part[j])
                                      * _gather_rows(inv, tab[5 + j])))
            y = obuf[...]
            for j in range(3):
                y = y + o_tile(NP - 1, j, ts[j])
            return y

        def start_attention(x):
            m, c, r = _ln_stats(x)
            z = c * r
            zq[...] = pltpu.bitcast(
                jnp.concatenate([z, z], axis=0).astype(bf16), u32)
            obuf[...] = jnp.zeros(obuf.shape, f32)
            return m, r

        def attention(x):
            m, r = start_attention(x)
            first_pairs(_with_ones(x), m, r)
            vp_copy(NR + 1).start()
            vp_copy(NP - 2, v14).start()

            def body(it, carry):
                @pl.when(it == (NP - 4) // 4 - 1)
                def _():
                    for i in range(NR, NP - 2):
                        vp_copy(i).wait()

                four_pairs(1 + 2 * it)
                return carry

            lax.fori_loop(0, (NP - 4) // 4, body, 0)
            vp_copy(NP - 2, v14).wait()
            return last_pairs()

        def streamed_pair(i, u, e):
            last = isinstance(i, int)
            ys = []
            _run(q_stage(u, e, ys))
            lhs = [_as_bf16(jnp.concatenate(ys[var::2], axis=1))
                   for var in range(2)]
            k_copy(i).wait()
            ss = []
            for c in range(ncp):
                k = kbuf[i, :, :, 8 * c:8 * c + 8, :].reshape(3, 8, 2, 8, 128)
                w = jnp.concatenate(
                    [k[t, :, par].reshape(64, 128)
                     for t in range(3) for par in range(2)], axis=0)
                s = _dot(lhs[c % 2], _as_bf16(w))[0:8]
                if c % 2:
                    s = ss.pop() + s
                ss.append(s)
            m = ss[0]
            for s in ss[1:]:
                m = jnp.maximum(m, s)
            ps = softmax_numerator(ss + [fold_rows(m, jnp.maximum)])
            inv = inverse_sum(ps)[1]
            for j in range(3):
                lbuf[0, j] = _gather_rows(inv, tab[5 + j])

            def swizzle(a, carry):
                for g in range(2, 8):
                    ref = kbuf.at[i, a // 3, 8 * (a % 3) + g]
                    v = ref[...].reshape(4, 4, 8, 128)
                    v = jnp.concatenate(
                        [v[:, c ^ (g // 2):(c ^ (g // 2)) + 1] for c in range(4)],
                        axis=1)
                    ref[...] = v.reshape(128, 128)
                return carry

            lax.fori_loop(0, NG // 8, swizzle, 0)

            for cp in ((vlast_copy,) if last else v_copies(i)):
                cp.wait()
            for par in range(2):
                pv = jnp.concatenate(
                    [_gather_rows(ps[c // 2], tab[2 * (c % 2) + par])
                     for c in range(ncp)], axis=0)

                def group(g, w):
                    for a, half in enumerate(_unpack(w)):
                        acc = (_as_f32(half) * pv).reshape(ncp, 8, 128)
                        abuf[0, g, pl.ds(a, 8, stride=2), :] = jnp.sum(acc, axis=0)

                def packed_group(gl, carry):
                    group(GH * par + gl, vbuf[_ring(i), par, gl])
                    return carry

                def wide_group(gl, carry):
                    if last:
                        w = vlast[par, gl]
                        keep = slice(0, 8 * (ncp - NT))
                        vlast_lo[par, gl], vlast[par, gl, keep, :] = _unpack(w[keep])
                    else:
                        ref = vwide.at[i, :, par, gl - (GH - NW)]
                        w = ref[1]
                        ref[0], ref[1] = _unpack(w)
                    group(GH * par + gl, w)
                    return carry

                split = 0 if last else GH - NW
                if split:
                    lax.fori_loop(0, split, packed_group, 0)
                lax.fori_loop(split, GH, wide_group, 0)
            ts = []
            _run(r_stage(0, ts), o_stage(i, ts))

        def transpose_last():
            for c in range(ncp - NT, ncp):
                v = _as_bf16(vlast[:, :, 8 * c:8 * c + 8, :].reshape(
                    8 * NG, 128)).astype(f32).reshape(NG, 16, 128)
                for s in range(2):
                    for j in range(3):
                        t = v[16 * j:16 * j + 16, 8 * s:8 * s + 8].reshape(128, 128)
                        t = pltpu.bitcast(t.T.astype(bf16), u32)
                        for n in range(8):
                            vlast[vt_slot(2 * c + s, j, n)] = t[8 * n:8 * n + 8]

        def streamed_attention(x):
            start_attention(x)

            spare = NP - 1 - NR
            late = [[k_copy(NP - 1)], [vlast_copy], [w1_copy, w3_copy]]
            late += [[cp] for cp in w2_copies]

            def body(n, carry):
                @pl.when(jnp.logical_and(n >= spare, n < 2 * spare))
                def _():
                    start_pair(n + NR - spare)

                for k, cps in enumerate(late):
                    @pl.when(n == 2 * spare + k)
                    def _():
                        for cp in cps:
                            cp.start()

                streamed_pair(visit(n), visit(n), None)
                return carry

            lax.fori_loop(0, NP - 1, body, 0)
            streamed_pair(NP - 1, NP // 2 - 1, 1)
            transpose_last()
            return obuf[...]

        def ffn(first, x):
            if first:
                w1_copy.wait()
                w3_copy.wait()
            m, _, r = _ln_stats(x)
            xo = _with_ones(x)
            hids = []
            for n in range(0, FF, FCH):
                gate = _round_bf16(_centered_dot(xo, w1[:, n:n + FCH], m) * r)
                up = _round_bf16(_centered_dot(xo, w3[:, n:n + FCH], m) * r)
                hids.append(
                    (_round_bf16(gate * jax.nn.sigmoid(gate)) * up).astype(bf16))
            y = None
            starts = [a for a, _ in W2_SPLITS]
            nv = 0 if first else NFV
            acc = [None] * (D // 128)
            for n in range(nv):
                for a, cv in enumerate(_columns(hids[n].astype(f32))):
                    if acc[0] is not None:
                        cv = jnp.where(zeros[...] != 0,
                                       acc[a % 5] + acc[(a + 2) % 5], cv)
                    for j in range(D // 128):
                        t = cv * w2[n, 8 * a:8 * a + 8,
                                    128 * j:128 * j + 128].astype(f32)
                        acc[j] = t if acc[j] is None else acc[j] + t
            if nv:
                y = jnp.sum(jnp.concatenate(acc, axis=1), axis=0, keepdims=True)
            for n in range(nv, len(hids)):
                if first and n in starts:
                    if y is not None:
                        obuf[...] = y
                    w2_copies[starts.index(n)].wait()
                    if y is not None:
                        y = obuf[...]
                t = _dot(hids[n], w2[n])
                y = t if y is None else y + t
            return y

        x_copy.wait()
        x = jnp.broadcast_to(xbuf[0].astype(f32), (8, D))
        x = _round_bf16(x + _round_bf16(streamed_attention(x)))
        x = _round_bf16(x + _round_bf16(ffn(True, x)))
        x = _round_bf16(x + _round_bf16(attention(x)))
        x = _round_bf16(x + _round_bf16(ffn(False, x)))
        o_ref[0] = x[0:1].astype(bf16)

    return kernel


def _tiles(a, lead):
    r, c = a.shape
    t = a.reshape(r // 8, 8, c // 128, 128).transpose(0, 2, 1, 3)
    return t.reshape(lead + (-1, 128))


@jax.jit
def pallas_interleave_layers__sliding_block_cached__glu_gated_swiglu__decode_kernel(
    A_x: jax.Array,
    A_k_cache: jax.Array,
    A_v_cache: jax.Array,
    A_wq: jax.Array,
    A_wo: jax.Array,
    B_x: jax.Array,
    B_w1: jax.Array,
    B_w3: jax.Array,
    B_w2: jax.Array,
):
    del B_x
    sk = A_k_cache.shape[2]
    win = min(4096, max(256, sk // 4))
    wr = win // 32
    kt = _tiles(jnp.swapaxes(A_k_cache, 2, 3).reshape(H * DH, sk), (NP, 2, GH))
    vt = _tiles(jnp.swapaxes(A_v_cache, 2, 3).reshape(H * DH, sk), (NP, 2, GH))
    any_spec = pl.BlockSpec(memory_space=pl.ANY)
    return pl.pallas_call(
        _make_kernel(sk, win),
        out_shape=jax.ShapeDtypeStruct((1, 1, D), bf16),
        in_specs=[any_spec] * 8,
        out_specs=pl.BlockSpec(memory_space=pltpu.VMEM),
        scratch_shapes=[
            pltpu.VMEM((1, 1, D), bf16),
            pltpu.VMEM((NP, 2, GH, wr, 128), u32),
            pltpu.VMEM((NR, 2, GH - NW, wr, 128), u32),
            pltpu.VMEM((NP - 1, 2, 2, NW, wr, 128), u32),
            pltpu.VMEM((2, GH, wr, 128), u32),
            pltpu.VMEM((2, GH, wr - 8 * NT, 128), u32),
            pltpu.VMEM((D // 32, H * DH // 8, 128), u32),
            pltpu.VMEM((H * DH // 16, D // 16, 128), u32),
            pltpu.VMEM((D, FF), bf16),
            pltpu.VMEM((D, FF), bf16),
            pltpu.VMEM((FF // FCH, FCH, D), bf16),
            pltpu.VMEM((8, D), u32),
            pltpu.VMEM((12, 8, 128), u32),
            pltpu.VMEM((3, 8, 128), u32),
            pltpu.VMEM((2, 8, 8, 128), f32),
            pltpu.VMEM((2, 3, 8, 128), f32),
            pltpu.VMEM((2, NG, 16, 128), f32),
            pltpu.VMEM((8, D), f32),
            pltpu.VMEM((8, 128), u32),
            pltpu.VMEM((8, 128), f32),
            pltpu.VMEM((16, 8, 128), jnp.int32),
            pltpu.SemaphoreType.DMA((NP,)),
            pltpu.SemaphoreType.DMA((2 * NP - 2,)),
            pltpu.SemaphoreType.DMA((8,)),
        ],
        compiler_params=pltpu.CompilerParams(
            vmem_limit_bytes=128 * 1024 * 1024,
            disable_semaphore_checks=True),
    )(A_x, kt, vt, _tiles(A_wq, (D // 32,)), _tiles(A_wo, (H * DH // 16,)),
      B_w1, B_w3, B_w2.reshape(FF // FCH, FCH, D))
```

```python
import jax
import jax.numpy as jnp
import numpy as np
from jax import lax
import jax.experimental.pallas as pl
import jax.experimental.pallas.tpu as pltpu

D = 640
H = 32
NP = H // 2
DH = 192
GH = DH // 8
NG = 2 * GH
FF = 1536
FCH = 128
EPS = 1e-5

NT = 7
NKV = 6
NFV = 6
NR = 12
NW = 7
W2_SPLITS = ((0, 8), (8, 11), (11, 12))

T_GROUP = 24.1
T_LAST = 12.0
T_FIRST = 610
EDGE_PACE = (0.8, 6, (40, 200))
LOOP_PACE = (0.8, 5, (30, 180))
LAT_FIRST = (187, 191, 180, 183, 190, 198, 210, 183, 178, 170, 185, 163, 113)
LAT_LOOP = (152, 200, 185, 218, 185, 160, 180, 187, 195, 162, 170, 178, 203,
            199, 179, 179, 187, 187, 151)
LAT_LAST = (138, 155, 123, 155, 155, 128, 160, 147, 221)

f32 = jnp.float32
bf16 = jnp.bfloat16
u32 = jnp.uint32


def _round_bf16(x):
    return x.astype(bf16).astype(f32)


def _as_bf16(x):
    return pltpu.bitcast(x, bf16)


def _as_f32(x):
    return pltpu.bitcast(x, f32)


def _dot(a, b):
    return jnp.dot(a, b, preferred_element_type=f32)


def _gather_rows(x, idx):
    dnums = lax.GatherDimensionNumbers(
        offset_dims=(), collapsed_slice_dims=(0,), start_index_map=(0,),
        operand_batching_dims=(1,), start_indices_batching_dims=(1,))
    return lax.gather(x, idx.reshape(8, 128, 1), dnums, slice_sizes=(1, 1),
                      mode=lax.GatherScatterMode.FILL_OR_DROP)


def _ln_stats(x):
    m = jnp.mean(x, axis=-1, keepdims=True)
    c = x - m
    v = jnp.mean(c * c, axis=-1, keepdims=True)
    return m, c, lax.rsqrt(v + EPS)


def _with_ones(x):
    return jnp.concatenate([x, jnp.ones_like(x)], axis=0).astype(bf16)


def _centered_dot(xo, w, m):
    y = _dot(xo, w)
    return y[0:8] - m * y[8:16]


def _packed(t):
    return _as_f32(jnp.concatenate([t, t], axis=0).astype(bf16))


def _columns(row):
    col = jnp.concatenate([row] * 16, axis=0).T
    return [col[8 * a:8 * a + 8] for a in range(16)]


def _unpack(w):
    return w << 16, w & jnp.uint32(0xFFFF0000)


def _run(*gens):
    for g in gens:
        for _ in g:
            pass


def _take(gen, n):
    for _ in range(n):
        yield next(gen)


def _group_order():
    order = []
    spots = {int((n + 0.5) * GH / NW) for n in range(NW)}
    for par in range(2):
        packed = list(range(GH * par, GH * par + GH - NW))
        wide = list(range(GH * par + GH - NW, GH * par + GH))
        order += [(wide if n in spots else packed).pop(0) for n in range(GH)]
    return order


def _ring(i):
    if isinstance(i, int):
        return i % NR
    return jnp.where(i >= NR, i - NR, i)


def _make_kernel(sk, win):
    nc = win // 128
    ncp = nc // 2
    row0 = (sk - win) // 128 * 4
    assert nc == 32
    scale = float(np.asarray(DH ** -0.5, dtype=bf16)) * float(np.log2(np.e))
    order = _group_order()

    def kernel(x_hbm, k_hbm, v_hbm, wq_hbm, wo_hbm, w1_hbm, w3_hbm, w2_hbm,
               o_ref,
               xbuf, kbuf, vbuf, vwide, vlast, vlast_lo, wq, wo, w1, w3, w2,
               zq, ybuf, qbuf, pbuf, lbuf, abuf, obuf, zeros, ones, tab,
               ksem, vsem, wsem):
        k32 = k_hbm.bitcast(u32)
        v32 = v_hbm.bitcast(u32)
        window = pl.ds(row0, 4 * nc)

        def k_copy(i):
            return pltpu.make_async_copy(
                k32.at[i, :, :, window, :], kbuf.at[i], ksem.at[i])

        def vp_copy(i, dst=None):
            return pltpu.make_async_copy(
                v32.at[i, :, pl.ds(0, GH - NW), window, :],
                vbuf.at[_ring(i)] if dst is None else dst, vsem.at[2 * i])

        def v_copies(i):
            return (vp_copy(i), pltpu.make_async_copy(
                v32.at[i, :, pl.ds(GH - NW, NW), window, :],
                vwide.at[i, 1], vsem.at[2 * i + 1]))

        def visit(n):
            spare = NP - 1 - NR
            return jnp.where(n < spare, n + NR, jnp.where(n >= NR, n - NR, n))

        def start_pair(n, carry=None):
            k_copy(visit(n)).start()
            for cp in v_copies(visit(n)):
                cp.start()
            return carry

        v14 = kbuf.at[0, :, pl.ds(0, GH - NW)]
        x_copy = pltpu.make_async_copy(x_hbm, xbuf, wsem.at[0])
        wq_copy = pltpu.make_async_copy(wq_hbm.bitcast(u32), wq, wsem.at[1])
        wo_copy = pltpu.make_async_copy(wo_hbm.bitcast(u32), wo, wsem.at[2])
        vlast_copy = pltpu.make_async_copy(
            v32.at[NP - 1, :, :, window, :], vlast, wsem.at[3])
        w1_copy = pltpu.make_async_copy(w1_hbm, w1, wsem.at[4])
        w3_copy = pltpu.make_async_copy(w3_hbm, w3, wsem.at[5])
        w2_copies = [
            pltpu.make_async_copy(w2_hbm.at[pl.ds(a, b - a)],
                                  w2.at[pl.ds(a, b - a)], wsem.at[6 + n])
            for n, (a, b) in enumerate(W2_SPLITS)]

        wq_copy.start()
        x_copy.start()
        wo_copy.start()
        lax.fori_loop(0, NR, start_pair, 0)

        lane = lax.broadcasted_iota(jnp.int32, (8, 128), 1)
        sub = lax.broadcasted_iota(jnp.int32, (8, 128), 0)
        zeros[...] = jnp.zeros((8, 128), u32)
        ones[...] = jnp.ones((8, 128), f32)
        for n in range(4):
            tab[n] = 2 * n + (sub >> 2)
        tab[4] = sub ^ 1
        tab[5] = jnp.zeros_like(sub)
        tab[6] = jnp.where(lane < 64, 0, 2)
        tab[7] = jnp.full_like(sub, 2)
        tab[8] = lane & 8
        tab[9] = sub
        tab[10] = sub - jnp.where(lane < 64, 0, 1)
        tab[11] = sub - 1
        for n in range(4):
            tab[12 + n] = jnp.where((sub >> 1) == n // 2,
                                    -65536 if n % 2 else 65535, 0)

        def retile(ref, ntile, place):
            top = sub < 4
            nrep = ref.shape[1] // (8 * ntile)

            def body(a, carry):
                v = [ref[a, 8 * n:8 * n + 8, :] for n in range(nrep * ntile)]
                for k in range(nrep):
                    for t in range(ntile):
                        lo = v[k * ntile + t // 2]
                        hi = v[k * ntile + (ntile + t) // 2]
                        if t % 2:
                            lo = pltpu.roll(lo, 4, 0)
                        if (ntile + t) % 2 == 0:
                            hi = pltpu.roll(hi, 4, 0)
                        r = 8 * place(k, t)
                        ref[a, r:r + 8, :] = jnp.where(top, lo, hi)
                return carry

            lax.fori_loop(0, ref.shape[0], body, 0)

        def k_rows(g, c):
            r = 8 * (c ^ (g // 2 % 4))
            return slice(r, r + 8)

        wq_copy.wait()
        retile(wq, H * DH // 128, lambda k, t: 2 * t + k)
        wo_copy.wait()
        retile(wo, D // 128, lambda k, t: t)

        def expand_q(t, b):
            even = tab[8] == 0
            return [jnp.where(tab[9 + t] == 2 * var, y, jnp.uint32(0))
                    for y in (jnp.where(even, b >> 16, pltpu.roll(b, 8, 1)),
                              jnp.where(even, pltpu.roll(b, 120, 1) >> 16, b))
                    for var in range(2)]

        def q_stage(u, e, out, proj=None, expand=True):
            if e is None:
                wref, e = wq.at[:, pl.ds(pl.multiple_of(48 * u, 16), 48), :], 0
            elif isinstance(u, int):
                wref = wq.at[:, pl.ds(96 * u, 96), :]
            else:
                wref = wq.at[:, pl.ds(pl.multiple_of(96 * u, 32), 96), :]
            for t in range(3):
                r = 48 * e + 16 * t
                w = _as_bf16(wref[:, r:r + 16, :].reshape(D // 2, 128))
                q = proj(w) if proj else _dot(_as_bf16(zq[...]), w)[0:8]
                b = pltpu.bitcast(_round_bf16(q), u32)
                out.extend(expand_q(t, b) if expand else [b])
                yield 40, [(_as_f32(b), 7)]

        def fold_rows(x, op):
            x = op(x, pltpu.roll(x, 4, 0))
            return op(x, _gather_rows(x, tab[4]))

        def k_stage(i, ys, out):
            kref = kbuf.at[i]
            m = None
            for c in range(ncp):
                lhs = jnp.concatenate(
                    [ys(2 * n + c % 2) for n in range(6)], axis=1)
                w = jnp.concatenate(
                    [kref[g // GH, g % GH, k_rows(g, c), :]
                     for t in range(3) for e in range(2)
                     for g in range(16 * t + e, 16 * t + 16, 2)], axis=0)
                s = _dot(_as_bf16(lhs), _as_bf16(w))[0:8]
                if c % 2 == 0:
                    out.append(s)
                    yield 48, [(s, 6)]
                else:
                    out[-1] = out[-1] + s
                    m = out[-1] if m is None else jnp.maximum(m, out[-1])
                    if c == ncp - 1:
                        m = fold_rows(m, jnp.maximum)
                    yield 48, [(m, 12 if c == ncp - 1 else 8)]
            out.append(m)

        def k_first(qb, out_a, out):
            even, low = tab[8] == 0, tab[6] == 0
            b = qb[1]
            rot = {n: pltpu.roll(b, n, 1) for n in (8, 56, 64, 72, 120)}
            mix = (jnp.where(even, jnp.where(low, b, rot[56]) >> 16,
                             jnp.where(low, rot[8], rot[64])),
                   jnp.where(even, jnp.where(low, rot[64], rot[120]) >> 16,
                             jnp.where(low, rot[72], b)))
            tiles = []
            for par in range(2):
                ys = expand_q(2 * par, qb[2 * par])
                for e in range(2):
                    tiles.append((ys[2 * e:2 * e + 2],
                                  range(32 * par + e, 32 * par + 16, 2)))
                g0 = 16 + 8 * par
                tiles.append((
                    [jnp.where(tab[9 + 2 * par] == 2 * var, mix[par],
                               jnp.uint32(0)) for var in range(2)],
                    [*range(g0, g0 + 8, 2), *range(g0 + 1, g0 + 8, 2)]))

            def part(c, sel):
                lhs = jnp.concatenate([tiles[n][0][c % 2] for n in sel], axis=1)
                w = jnp.concatenate(
                    [kbuf[0, g // GH, g % GH, k_rows(g, c), :]
                     for n in sel for g in tiles[n][1]], axis=0)
                return _dot(_as_bf16(lhs), _as_bf16(w))[0:8]

            plan = [(c, (0, 1)) for c in range(4)] + [(c, (2,)) for c in range(4)]
            plan += [(c, (0, 1, 2)) for c in range(4, ncp - NKV)]
            acc = [None] * (ncp // 2)
            cols = _columns(_as_f32(qb[0])) + _columns(_as_f32(qb[1]))[:8]
            vacc = [None] * (2 * NKV)
            for g in range(GH):
                for n, c in enumerate(range(ncp - NKV, ncp)):
                    k = _as_bf16(kbuf[0, 0, g, k_rows(g, c), :]).astype(f32)
                    for e in range(2):
                        t = k[8 * e:8 * e + 8] * cols[g]
                        vacc[2 * n + e] = t if g == 0 else vacc[2 * n + e] + t
            for n, t in enumerate(vacc):
                for sh in (4, 2, 1):
                    t = t + pltpu.roll(t, sh, 0)
                c = ncp - NKV + n // 2
                prev = 0.0 if acc[c // 2] is None else acc[c // 2]
                acc[c // 2] = jnp.where(tab[9] == 4 * (c % 2) + n % 2, t, prev)
            for c, sel in plan:
                s = part(c, sel)
                acc[c // 2] = s if acc[c // 2] is None else acc[c // 2] + s
                yield 8 * len(sel), []
            m = acc[0]
            for a in acc[1:]:
                m = jnp.maximum(m, a)
            out_a.extend(acc + [fold_rows(m, jnp.maximum)])
            m = None
            for j in range(ncp // 2):
                s = acc[j] + part(2 * j, (3, 4, 5)) + part(2 * j + 1, (3, 4, 5))
                out.append(s)
                m = s if m is None else jnp.maximum(m, s)
                if j == ncp // 2 - 1:
                    m = fold_rows(m, jnp.maximum)
                yield 48, [(m, 8)]
            out.append(m)

        def softmax_numerator(ss, sc=scale):
            m = jnp.max(ss[-1], axis=1, keepdims=True)
            return [jnp.exp2((s - m) * sc) for s in ss[:-1]]

        def inverse_sum(ps):
            tot = ps[0]
            for p in ps[1:]:
                tot = tot + p
            lf = fold_rows(tot, jnp.add)
            l = jnp.sum(lf, axis=1, keepdims=True)
            l = jnp.broadcast_to(l, (8, 128))
            y = pl.reciprocal(l, approx=True)
            return lf, y * (2.0 - l * y)

        def lane_sums(b, j):
            a = jnp.concatenate(
                [abuf[b, 16 * j:16 * j + 16, 8 * s:8 * s + 8, :].reshape(128, 128)
                 for s in range(2)], axis=1)
            return lax.dot_general(
                jnp.concatenate([ones[...]] * 2, axis=1), a,
                (((1,), (1,)), ((), ())), preferred_element_type=f32)

        def r_stage(b, out):
            for j in range(3):
                out.append(_packed(lane_sums(b, j) * lbuf[b, j]))
                yield 32, [(out[-1], 4)]

        def o_stage(i, ts):
            wref = wo.at[pl.ds(24 * i, 24)]
            t = _as_bf16(jnp.concatenate(ts, axis=1))
            for n in range(D // 128):
                cols = slice(128 * n, 128 * n + 128)
                w = wref[:, 8 * n:8 * n + 8, :].reshape(DH, 128)
                y = obuf[:, cols] + _dot(t, _as_bf16(w))[0:8]
                obuf[:, cols] = y
                yield 24, [(y, 4)]

        def o_tile(i, j, t):
            r0 = 24 * i + 8 * j
            w = jnp.concatenate(
                [wo[r0:r0 + 8, 8 * n:8 * n + 8, :].reshape(64, 128)
                 for n in range(D // 128)], axis=1)
            return _dot(_as_bf16(t), _as_bf16(w))[0:8]

        def trace_mxu(gens, links, latency, t=0.0, rate=1.0):
            for gen in gens:
                for cost, res in gen:
                    t += cost / rate
                    lat = np.interp(t / 250, range(len(latency)), latency)
                    links.setdefault(t + float(lat), []).extend(res)
            return t

        def v_stage(i, b, getp, links, clock, hist, pace):
            never = zeros[...] != 0
            last = i is None
            if not last:
                vp = (v14 if isinstance(i, int) and i == NP - 2
                      else vbuf.at[_ring(i)])
            for n, g in enumerate(range(NG) if last else order):
                par, gl = divmod(g, GH)
                if n % GH == 0:
                    ps = [getp(par, j) for j in range(nc // 4)]
                    idx = [tab[par], tab[2 + par]]
                    if len(hist) > 1 and getp is not from_pbuf:
                        dep = pltpu.bitcast(hist[-2][0], jnp.int32)
                        idx = [jnp.where(never, dep, ix) for ix in idx]
                    pv = [_gather_rows(ps[c // 2], idx[c % 2])
                          for c in range(ncp - NT if last else ncp)]
                    clock[0] += 4
                    if par == 1 and not last:
                        lf, inv = inverse_sum(ps)
                        for val, at in zip((lf, inv), pace[2]):
                            links.setdefault(clock[0] + at, []).append((val, 14))
                        for j in range(3):
                            lbuf[b, j] = _gather_rows(inv, tab[5 + j])
                wide = last or gl >= GH - NW
                if last:
                    refs = vlast_lo.at[par, gl], vlast.at[par, gl]
                elif wide:
                    ref = vwide.at[i, :, par, gl - (GH - NW)]
                    refs = ref.at[0], ref.at[1]
                else:
                    ref = vp.at[par, gl]
                dur = T_LAST if last else T_GROUP * (pace[0] if wide else 1.0)
                accs = [None, None]
                held = [None, None]
                pending = []
                nsteps = ncp - NT if last else ncp
                for c in range(nsteps):
                    for key in sorted(links):
                        if key < clock[0] + dur * (c + 1) / nsteps:
                            for val, ops in links.pop(key):
                                pending.append(val)
                                clock[0] += ops / 4
                    rs = slice(8 * c, 8 * c + 8)
                    if wide:
                        lo, hi = refs[0][rs, :], refs[1][rs, :]
                    else:
                        lo, hi = _unpack(ref[rs, :])
                    p = pv[c]
                    if c == (8 if last else pace[1] if wide else 0) and hist:
                        p = jnp.where(never, hist[-1][0] + hist[-1][1], p)
                    for a, t in enumerate((_as_f32(lo) * p, _as_f32(hi) * p)):
                        if accs[a] is None:
                            accs[a] = t
                            continue
                        if pending:
                            t = jnp.where(never, pending.pop(), t)
                        if c % 2 == 1 and c < nsteps - 1:
                            held[a] = t
                        else:
                            if held[a] is not None:
                                t = held[a] + t
                                held[a] = None
                            accs[a] = accs[a] + t
                for a in range(2):
                    abuf[b, g, pl.ds(a, 8, stride=2), :] = accs[a]
                clock[0] += dur
                hist.append(accs)
                yield g

        def from_pbuf(par, j):
            return pbuf[par, j]

        def values(ps):
            return lambda par, j: ps[j]

        def store_state(ya, qb, ps):
            for n in range(12):
                ybuf[n] = ya[n]
            for n in range(3):
                qbuf[n] = qb[n]
            for j, p in enumerate(ps):
                pbuf[0, j] = p
                pbuf[1, j] = p

        def four_pairs(u0):
            links, clock, hist = {}, [30], []
            getq, getp = (lambda n: qbuf[n]), from_pbuf
            s1 = []
            k1 = k_stage(2 * u0 + 1, lambda n: ybuf[n], s1)
            t = 0.0

            def mxu(gens, t):
                return trace_mxu(gens, links, LAT_LOOP, t, 0.99)

            for half in range(2):
                u = u0 + half
                i = 2 * u
                s2, ya, qb, t0, t1 = [], [], [], [], []
                y2 = [y for n in range(3) for y in expand_q(n, getq(n))]
                k2 = k_stage(i + 2, y2.__getitem__, s2)
                t = mxu([k1], t)
                p1 = softmax_numerator(s1)
                t = mxu([r_stage(1, t1), q_stage(u + 1, 1, ya),
                         o_stage(i - 1, t1), _take(k2, 4)], t)
                _run(v_stage(i, 0, getp, links, clock, hist, LOOP_PACE))
                t = mxu([r_stage(0, t0), k2], max(t, clock[0] - 64))
                p2 = softmax_numerator(s2)
                t = mxu([o_stage(i, t0),
                         q_stage(jnp.minimum(u + 2, NP // 2 - 1), 0, qb,
                                 expand=False)], t)
                if half == 0:
                    s1 = []
                    k1 = k_stage(i + 3, ya.__getitem__, s1)
                    t = mxu([_take(k1, 1)], t)
                _run(v_stage(i + 1, 1, values(p1), links, clock, hist,
                             LOOP_PACE))
                getq, getp = qb.__getitem__, values(p2)
            store_state(ya, qb, p2)

        def first_pairs(xo, m, r):
            links, clock, hist = {}, [T_FIRST], []
            q0, y1, y2, sa, s0, s1, s2, ya, qb, t0 = ([] for _ in range(10))
            _run(q_stage(0, 0, q0, lambda w: _centered_dot(xo, w, m), False),
                 q_stage(0, 1, y1, lambda w: _centered_dot(xo, w, m) * r))
            t = trace_mxu([k_first(q0, sa, s0),
                           k_stage(1, lambda n: y1[n], s1),
                           q_stage(1, 0, y2), q_stage(1, 1, ya),
                           q_stage(2, 0, qb, expand=False)], links, LAT_FIRST)
            for key in [key for key in links if key < T_FIRST + 30]:
                del links[key]
            pa = softmax_numerator(sa, r * scale)
            p0 = softmax_numerator(s0, r * scale)
            p1 = softmax_numerator(s1)
            _run(v_stage(0, 0, lambda par, j: (pa, p0)[par][j], links,
                         clock, hist, EDGE_PACE))
            vp_copy(NR).start()
            trace_mxu([r_stage(0, t0), k_stage(2, lambda n: y2[n], s2),
                       o_stage(0, t0)], links, LAT_FIRST,
                      max(t, clock[0] - 64))
            p2 = softmax_numerator(s2)
            _run(v_stage(1, 1, values(p1), links, clock,
                         hist, EDGE_PACE))
            store_state(ya, qb, p2)

        def vt_slot(kc, j, n):
            g = 24 * (kc % 2) + 8 * j + n
            r = 8 * (kc // 2)
            return (g // GH, g % GH, slice(r, r + 8), slice(None))

        def last_pairs():
            i = NP - 2
            links, clock, hist = {}, [20], []
            s1, t0, t1, ts, part, rows = ([] for _ in range(6))
            tk = trace_mxu([k_stage(i + 1, lambda n: ybuf[n], s1)],
                           links, LAT_LAST)
            t = trace_mxu([r_stage(1, t1)], links, LAT_LAST, tk)
            t = trace_mxu([o_stage(i - 1, t1)], links, LAT_LAST, t + 90)
            ps = softmax_numerator(s1)
            chunks = range(nc - 2 * NT, nc)
            for kc in chunks:
                bits = pltpu.bitcast(_packed(ps[kc // 4]), u32)
                rows.append(bits & pltpu.bitcast(tab[12 + kc % 4], u32))
                links.setdefault(tk + 315, []).append((_as_f32(rows[-1]), 3))
            lhs = _as_bf16(jnp.concatenate(rows, axis=1))

            def p_stage():
                for j in range(3):
                    w = jnp.concatenate([vlast[vt_slot(kc, j, n)]
                                         for kc in chunks for n in range(8)],
                                        axis=0)
                    y = fold_rows(_dot(lhs, _as_bf16(w))[0:8], jnp.add)
                    part.append(_gather_rows(y, tab[5 + j]))
                    yield 16 * NT, [(part[j], 2 * NT + 5)]

            pg = p_stage()
            t = trace_mxu([_take(pg, 1)], links, LAT_LAST, max(t, tk + 300))
            _run(v_stage(i, 0, from_pbuf, links, clock, hist, EDGE_PACE))
            trace_mxu([r_stage(0, t0), _take(pg, 1), o_stage(i, t0), pg],
                      links, LAT_LAST, max(t, clock[0] + 90))
            lf, inv = inverse_sum(ps)
            links.setdefault(clock[0] + 20, []).append((lf, 10))
            links.setdefault(clock[0] + 160, []).append((inv, 10))
            for g in v_stage(None, 1, values(ps), links, clock, hist,
                             EDGE_PACE):
                if g % 16 == 15:
                    j = g // 16
                    ts.append(_packed((lane_sums(1, j) + part[j])
                                      * _gather_rows(inv, tab[5 + j])))
            y = obuf[...]
            for j in range(3):
                y = y + o_tile(NP - 1, j, ts[j])
            return y

        def start_attention(x):
            m, c, r = _ln_stats(x)
            z = c * r
            zq[...] = pltpu.bitcast(
                jnp.concatenate([z, z], axis=0).astype(bf16), u32)
            obuf[...] = jnp.zeros(obuf.shape, f32)
            return m, r

        def attention(x):
            m, r = start_attention(x)
            first_pairs(_with_ones(x), m, r)
            vp_copy(NR + 1).start()
            vp_copy(NP - 2, v14).start()

            def body(it, carry):
                @pl.when(it == (NP - 4) // 4 - 1)
                def _():
                    for i in range(NR, NP - 2):
                        vp_copy(i).wait()

                four_pairs(1 + 2 * it)
                return carry

            lax.fori_loop(0, (NP - 4) // 4, body, 0)
            vp_copy(NP - 2, v14).wait()
            return last_pairs()

        def streamed_pair(i, u, e):
            last = isinstance(i, int)
            ys = []
            _run(q_stage(u, e, ys))
            lhs = [_as_bf16(jnp.concatenate(ys[var::2], axis=1))
                   for var in range(2)]
            k_copy(i).wait()
            ss = []
            for c in range(ncp):
                k = kbuf[i, :, :, 8 * c:8 * c + 8, :].reshape(3, 8, 2, 8, 128)
                w = jnp.concatenate(
                    [k[t, :, par].reshape(64, 128)
                     for t in range(3) for par in range(2)], axis=0)
                s = _dot(lhs[c % 2], _as_bf16(w))[0:8]
                if c % 2:
                    s = ss.pop() + s
                ss.append(s)
            m = ss[0]
            for s in ss[1:]:
                m = jnp.maximum(m, s)
            ps = softmax_numerator(ss + [fold_rows(m, jnp.maximum)])
            inv = inverse_sum(ps)[1]
            for j in range(3):
                lbuf[0, j] = _gather_rows(inv, tab[5 + j])

            def swizzle(a, carry):
                for g in range(2, 8):
                    ref = kbuf.at[i, a // 3, 8 * (a % 3) + g]
                    v = ref[...].reshape(4, 4, 8, 128)
                    v = jnp.concatenate(
                        [v[:, c ^ (g // 2):(c ^ (g // 2)) + 1] for c in range(4)],
                        axis=1)
                    ref[...] = v.reshape(128, 128)
                return carry

            lax.fori_loop(0, NG // 8, swizzle, 0)

            for cp in ((vlast_copy,) if last else v_copies(i)):
                cp.wait()
            for par in range(2):
                pv = jnp.concatenate(
                    [_gather_rows(ps[c // 2], tab[2 * (c % 2) + par])
                     for c in range(ncp)], axis=0)

                def group(g, w):
                    for a, half in enumerate(_unpack(w)):
                        acc = (_as_f32(half) * pv).reshape(ncp, 8, 128)
                        abuf[0, g, pl.ds(a, 8, stride=2), :] = jnp.sum(acc, axis=0)

                def packed_group(gl, carry):
                    group(GH * par + gl, vbuf[_ring(i), par, gl])
                    return carry

                def wide_group(gl, carry):
                    if last:
                        w = vlast[par, gl]
                        keep = slice(0, 8 * (ncp - NT))
                        vlast_lo[par, gl], vlast[par, gl, keep, :] = _unpack(w[keep])
                    else:
                        ref = vwide.at[i, :, par, gl - (GH - NW)]
                        w = ref[1]
                        ref[0], ref[1] = _unpack(w)
                    group(GH * par + gl, w)
                    return carry

                split = 0 if last else GH - NW
                if split:
                    lax.fori_loop(0, split, packed_group, 0)
                lax.fori_loop(split, GH, wide_group, 0)
            ts = []
            _run(r_stage(0, ts), o_stage(i, ts))

        def transpose_last():
            for c in range(ncp - NT, ncp):
                v = _as_bf16(vlast[:, :, 8 * c:8 * c + 8, :].reshape(
                    8 * NG, 128)).astype(f32).reshape(NG, 16, 128)
                for s in range(2):
                    for j in range(3):
                        t = v[16 * j:16 * j + 16, 8 * s:8 * s + 8].reshape(128, 128)
                        t = pltpu.bitcast(t.T.astype(bf16), u32)
                        for n in range(8):
                            vlast[vt_slot(2 * c + s, j, n)] = t[8 * n:8 * n + 8]

        def streamed_attention(x):
            start_attention(x)

            spare = NP - 1 - NR
            late = [[k_copy(NP - 1)], [vlast_copy], [w1_copy, w3_copy]]
            late += [[cp] for cp in w2_copies]

            def body(n, carry):
                @pl.when(jnp.logical_and(n >= spare, n < 2 * spare))
                def _():
                    start_pair(n + NR - spare)

                for k, cps in enumerate(late):
                    @pl.when(n == 2 * spare + k)
                    def _():
                        for cp in cps:
                            cp.start()

                streamed_pair(visit(n), visit(n), None)
                return carry

            lax.fori_loop(0, NP - 1, body, 0)
            streamed_pair(NP - 1, NP // 2 - 1, 1)
            transpose_last()
            return obuf[...]

        def ffn(first, x):
            if first:
                w1_copy.wait()
                w3_copy.wait()
            m, _, r = _ln_stats(x)
            xo = _with_ones(x)
            hids = []
            for n in range(0, FF, FCH):
                gate = _round_bf16(_centered_dot(xo, w1[:, n:n + FCH], m) * r)
                up = _round_bf16(_centered_dot(xo, w3[:, n:n + FCH], m) * r)
                hids.append(
                    (_round_bf16(gate * jax.nn.sigmoid(gate)) * up).astype(bf16))
            y = None
            starts = [a for a, _ in W2_SPLITS]
            nv = 0 if first else NFV
            acc = [None] * (D // 128)
            for n in range(nv):
                for a, cv in enumerate(_columns(hids[n].astype(f32))):
                    if acc[0] is not None:
                        cv = jnp.where(zeros[...] != 0,
                                       acc[a % 5] + acc[(a + 2) % 5], cv)
                    for j in range(D // 128):
                        t = cv * w2[n, 8 * a:8 * a + 8,
                                    128 * j:128 * j + 128].astype(f32)
                        acc[j] = t if acc[j] is None else acc[j] + t
            if nv:
                y = jnp.sum(jnp.concatenate(acc, axis=1), axis=0, keepdims=True)
            tail = range(starts[1], len(hids)) if first else ()

            def col(n, a):
                return (0, 8 * (n - tail[0]) + a // 2, pl.ds(8 * (a % 2), 8))

            for n in tail:
                for a, cv in enumerate(_columns(hids[n].astype(f32))):
                    abuf[col(n, a)] = cv
            for n in range(nv, len(hids)):
                if first and n in starts:
                    if y is not None:
                        obuf[...] = y
                    w2_copies[starts.index(n)].wait()
                    if y is not None:
                        y = obuf[...]
                if n in tail:
                    parts = []
                    for j in range(D // 128):
                        ts = [abuf[col(n, a)] * w2[n, 8 * a:8 * a + 8,
                                                   128 * j:128 * j + 128].astype(f32)
                              for a in range(16)]
                        while len(ts) > 1:
                            ts = [ts[k] + ts[k + 1] for k in range(0, len(ts), 2)]
                        t = ts[0]
                        for sh in (4, 2, 1):
                            t = t + pltpu.roll(t, sh, 0)
                        parts.append(t)
                    t = jnp.concatenate(parts, axis=1)
                else:
                    t = _dot(hids[n], w2[n])
                y = t if y is None else y + t
            return y

        x_copy.wait()
        x = jnp.broadcast_to(xbuf[0].astype(f32), (8, D))
        x = _round_bf16(x + _round_bf16(streamed_attention(x)))
        x = _round_bf16(x + _round_bf16(ffn(True, x)))
        x = _round_bf16(x + _round_bf16(attention(x)))
        x = _round_bf16(x + _round_bf16(ffn(False, x)))
        o_ref[0] = x[0:1].astype(bf16)

    return kernel


def _tiles(a, lead):
    r, c = a.shape
    t = a.reshape(r // 8, 8, c // 128, 128).transpose(0, 2, 1, 3)
    return t.reshape(lead + (-1, 128))


@jax.jit
def pallas_interleave_layers__sliding_block_cached__glu_gated_swiglu__decode_kernel(
    A_x: jax.Array,
    A_k_cache: jax.Array,
    A_v_cache: jax.Array,
    A_wq: jax.Array,
    A_wo: jax.Array,
    B_x: jax.Array,
    B_w1: jax.Array,
    B_w3: jax.Array,
    B_w2: jax.Array,
):
    del B_x
    sk = A_k_cache.shape[2]
    win = min(4096, max(256, sk // 4))
    wr = win // 32
    kt = _tiles(jnp.swapaxes(A_k_cache, 2, 3).reshape(H * DH, sk), (NP, 2, GH))
    vt = _tiles(jnp.swapaxes(A_v_cache, 2, 3).reshape(H * DH, sk), (NP, 2, GH))
    any_spec = pl.BlockSpec(memory_space=pl.ANY)
    return pl.pallas_call(
        _make_kernel(sk, win),
        out_shape=jax.ShapeDtypeStruct((1, 1, D), bf16),
        in_specs=[any_spec] * 8,
        out_specs=pl.BlockSpec(memory_space=pltpu.VMEM),
        scratch_shapes=[
            pltpu.VMEM((1, 1, D), bf16),
            pltpu.VMEM((NP, 2, GH, wr, 128), u32),
            pltpu.VMEM((NR, 2, GH - NW, wr, 128), u32),
            pltpu.VMEM((NP - 1, 2, 2, NW, wr, 128), u32),
            pltpu.VMEM((2, GH, wr, 128), u32),
            pltpu.VMEM((2, GH, wr - 8 * NT, 128), u32),
            pltpu.VMEM((D // 32, H * DH // 8, 128), u32),
            pltpu.VMEM((H * DH // 16, D // 16, 128), u32),
            pltpu.VMEM((D, FF), bf16),
            pltpu.VMEM((D, FF), bf16),
            pltpu.VMEM((FF // FCH, FCH, D), bf16),
            pltpu.VMEM((8, D), u32),
            pltpu.VMEM((12, 8, 128), u32),
            pltpu.VMEM((3, 8, 128), u32),
            pltpu.VMEM((2, 8, 8, 128), f32),
            pltpu.VMEM((2, 3, 8, 128), f32),
            pltpu.VMEM((2, NG, 16, 128), f32),
            pltpu.VMEM((8, D), f32),
            pltpu.VMEM((8, 128), u32),
            pltpu.VMEM((8, 128), f32),
            pltpu.VMEM((16, 8, 128), jnp.int32),
            pltpu.SemaphoreType.DMA((NP,)),
            pltpu.SemaphoreType.DMA((2 * NP - 2,)),
            pltpu.SemaphoreType.DMA((6 + len(W2_SPLITS),)),
        ],
        compiler_params=pltpu.CompilerParams(
            vmem_limit_bytes=128 * 1024 * 1024,
            disable_semaphore_checks=True),
    )(A_x, kt, vt, _tiles(A_wq, (D // 32,)), _tiles(A_wo, (H * DH // 16,)),
      B_w1, B_w3, B_w2.reshape(FF // FCH, FCH, D))
```
